```python
import os as _os
_os.environ.setdefault("JAX_PLATFORMS", "cpu")
import jax
import jax.numpy as jnp

def _softmax(x, axis=-1):
    return jax.nn.softmax(x, axis=axis)
def _gelu(x):
    return jax.nn.gelu(x, approximate=True)
def _silu(x):
    return jax.nn.silu(x)
def _sigmoid(x):
    return jax.nn.sigmoid(x)
def _layernorm(x, axis=-1, eps=1e-5):
    m = jnp.mean(x, axis=axis, keepdims=True)
    v = jnp.var(x, axis=axis, keepdims=True)
    return (x - m) / jnp.sqrt(v + eps)
def _scatter_add(tgt, idx, src, axis=0):
    return tgt.at[idx].add(src)
def _segment_sum(src, seg, n):
    return jax.ops.segment_sum(src, seg, n)
class _Rng:
    def __init__(self, key):
        self._k = key
    def _next(self):
        self._k, sub = jax.random.split(self._k)
        return sub
    def normal(self, shape):
        return jax.random.normal(self._next(), shape, dtype=jnp.bfloat16)
    def randint(self, lo, hi, shape):
        return jax.random.randint(self._next(), shape, lo, hi, dtype=jnp.int32)
    def uniform(self, shape, lo=0.0, hi=1.0):
        return jax.random.uniform(self._next(), shape, jnp.bfloat16, lo, hi)
    def permutation(self, n):
        return jax.random.permutation(self._next(), n)


kernel_name = 'sequential_preLN__linear_kernel_hedgehog__geglu_ffn__prompt'

def setup_inputs():
    _rng = _Rng(jax.random.key(int.from_bytes(__import__("os").urandom(4), "little")))
    _w = (lambda a: (lambda t: t.astype(jnp.bfloat16) if jnp.issubdtype(t.dtype, jnp.floating) else t)(jnp.asarray(a)))
    def _A_setup():
        B, S, D, H = 1, 2048, 640, 32
        Dh = D // H
        return {
            "x": _w((lambda *s: _rng.normal(s) * 0.05)(B, S, D)),
            "wqkv": _w((lambda *s: _rng.normal(s) * 0.2)(D, 3 * D)),
            "w_phi": _w((lambda *s: _rng.normal(s) * 0.2)(H, Dh, Dh) * (Dh ** -0.5)),
            "wo": _w((lambda *s: _rng.normal(s) * 0.05)(D, D)),
        }
    _A_in = _A_setup()

    def _B_setup():
        B, S, D, F = 1, 2048, 640, 1536
        return {
            "x": _w((lambda *s: _rng.normal(s) * 0.05)(B, S, D)),
            "w_gate": _w((lambda *s: _rng.normal(s) * 0.05)(D, F)),
            "w_up": _w((lambda *s: _rng.normal(s) * 0.05)(D, F)),
            "w_down": _w((lambda *s: _rng.normal(s) * 0.05)(F, D)),
        }
    _B_in = _B_setup()

    return {
        "A_x": _A_in["x"],
        "A_wqkv": _A_in["wqkv"],
        "A_w_phi": _A_in["w_phi"],
        "A_wo": _A_in["wo"],
        "B_x": _B_in["x"],
        "B_w_gate": _B_in["w_gate"],
        "B_w_up": _B_in["w_up"],
        "B_w_down": _B_in["w_down"],
    }

def reference(A_x, A_wqkv, A_w_phi, A_wo, B_x, B_w_gate, B_w_up, B_w_down):
    def _A_ref(x, wqkv, w_phi, wo):
        B, S, D = x.shape
        H = 32; Dh = D // H
        qkv = (lambda x, *d: x.transpose(*d))((x @ wqkv).reshape(B, S, 3, H, Dh), 2, 0, 3, 1, 4)
        q, k, v = qkv[0], qkv[1], qkv[2]
        pq = jnp.einsum("bhsd,hdf->bhsf", q, w_phi)
        pk = jnp.einsum("bhsd,hdf->bhsf", k, w_phi)
        phi_q = jnp.concatenate([_softmax(pq, axis=-1), _softmax(-pq, axis=-1)], axis=-1)
        phi_k = jnp.concatenate([_softmax(pk, axis=-1), _softmax(-pk, axis=-1)], axis=-1)
        kv = jnp.einsum("bhsf,bhsd->bhfd", phi_k, v)
        z  = jnp.einsum("bhsf->bhf", phi_k)
        num = jnp.einsum("bhqf,bhfd->bhqd", phi_q, kv)
        den = jnp.einsum("bhqf,bhf->bhq", phi_q, z)[..., None] + 1e-6
        o = num / den
        return (lambda x, *d: x.transpose(*d))(o, 0, 2, 1, 3).reshape(B, S, D) @ wo

    def _B_ref(x, w_gate, w_up, w_down):
        return (_gelu(x @ w_gate) * (x @ w_up)) @ w_down

    x = A_x
    h = x + _A_ref(_layernorm(x, axis=-1), A_wqkv, A_w_phi, A_wo)
    h2 = h + _B_ref(_layernorm(h, axis=-1), B_w_gate, B_w_up, B_w_down)
    return h2
```

```python
import functools
import jax
import jax.numpy as jnp
from jax import lax
from jax.experimental import pallas as pl
from jax.experimental.pallas import tpu as pltpu

S, D, H, DH, F = 2048, 640, 32, 20, 1536
NG = 16
LOG2E = 1.4426950408889634
NT = (((1,), (1,)), ((), ()))
f32 = jnp.float32
bf16 = jnp.bfloat16


def _ln(x):
    m = jnp.mean(x, axis=-1, keepdims=True)
    xc = x - m
    v = jnp.mean(xc * xc, axis=-1, keepdims=True)
    return xc * lax.rsqrt(v + 1e-5)


def _rcp(x):
    r = pl.reciprocal(x, approx=True)
    return r * (2.0 - x * r)


def _allred(m, op):
    m = op(m, pltpu.roll(m, 2, 0))
    return op(m, pltpu.roll(m, 4, 0))


def _feat1(p):
    ps = [p[8 * v:8 * v + 8] for v in range(5)]
    mx = functools.reduce(jnp.maximum, ps)
    mn = functools.reduce(jnp.minimum, ps)
    mx = _allred(mx, jnp.maximum)
    mn = _allred(mn, jnp.minimum)
    ep = [jnp.exp2(q - mx) for q in ps]
    en = [jnp.exp2(mn - q) for q in ps]
    rp = _rcp(_allred(functools.reduce(jnp.add, ep), jnp.add))
    rn = _rcp(_allred(functools.reduce(jnp.add, en), jnp.add))
    return jnp.concatenate([e * rp for e in ep] + [e * rn for e in en], axis=0).astype(bf16)


def _featn(p):
    w = p.shape[1]
    ng = p.shape[0] // 40
    p4 = p.reshape(ng, 5, 8, w)

    def allred(m, op):
        m = op(m, pltpu.roll(m, 2, 1))
        return op(m, pltpu.roll(m, 4, 1))

    mx = allred(jnp.max(p4, axis=1), jnp.maximum)
    mn = allred(jnp.min(p4, axis=1), jnp.minimum)
    ep = jnp.exp2(p4 - mx[:, None])
    en = jnp.exp2(mn[:, None] - p4)
    rp = _rcp(allred(jnp.sum(ep, axis=1), jnp.add))
    rn = _rcp(allred(jnp.sum(en, axis=1), jnp.add))
    phi = jnp.concatenate([ep * rp[:, None], en * rn[:, None]], axis=1)
    return phi.reshape(ng, 80, w).astype(bf16)


def _gelu_mul(g, u):
    c = 0.7978845608028654
    inner = g * (c + (c * 0.044715) * (g * g))
    t = jnp.tanh(inner)
    hgu = (0.5 * g) * u
    return hgu + hgu * t


u32 = jnp.uint32


def _pk(v):
    return pltpu.bitcast(v, u32)


def _up(v):
    return pltpu.bitcast(v, bf16)


def _nt(a, b):
    return lax.dot_general(a, b, NT, preferred_element_type=f32)


class Pipe:
    def __init__(self, lag):
        self.lag = lag
        self.pending = []
        self.fill = []

    def item(self, mxu, post):
        r = mxu()
        self.pending.append((post, r))
        if len(self.pending) > self.lag:
            p, v = self.pending.pop(0)
            p(v)
        if self.fill:
            self.fill.pop(0)()

    def drain(self, keep=0):
        while len(self.pending) > keep:
            p, v = self.pending.pop(0)
            p(v)

    def flush_fill(self):
        while self.fill:
            self.fill.pop(0)()


def make(fc=512, R=4, T2=512, op=128, lnc=32, lag=1, wob=128, fg=2):
    T1 = 128 * R
    P0 = 256
    P1 = 512
    n1 = (S - P1) // T1
    n2 = S // T2
    HA = T2 // 2
    npc = T2 // op

    def kernel(x_hbm, wqkv_hbm, wphi_hbm, wo_hbm, wg_hbm, wu_hbm, wd_hbm, out_hbm,
               x_v, wq_v, wk_v, wv_v, wphi_v, wo_v, wg_v, wu_v, wd_v, wqT, wkT, wvT, bcat,
               xn0, xn_buf, phiq, phik, vaug, kvm, oa_buf, out_v,
               sem_i, sem_o):
        def cp(src, dst, k):
            return pltpu.make_async_copy(src, dst, sem_i.at[k])

        def xrows(r0, n, k):
            return cp(x_hbm.at[0, pl.ds(r0, n)], x_v.at[pl.ds(r0, n)], k)
        c_phi = cp(wphi_hbm, wphi_v, 0)
        c_x0 = xrows(0, P0, 1)
        c_ka = cp(wqkv_hbm.at[:, pl.ds(D, 256)], wk_v.at[:, pl.ds(0, 256)], 2)
        c_kb = cp(wqkv_hbm.at[:, pl.ds(D + 256, D - 256)], wk_v.at[:, pl.ds(256, D - 256)], 3)
        c_x0b = xrows(P0, P1 - P0, 4)
        c_q = cp(wqkv_hbm.at[:, pl.ds(0, D)], wq_v, 5)
        c_v = cp(wqkv_hbm.at[:, pl.ds(2 * D, D)], wv_v, 6)

        def xcopy(i):
            return xrows(P1 + i * T1, T1, 7 + i)
        c_wo = cp(wo_hbm, wo_v, 7 + n1)
        c_wg = cp(wg_hbm, wg_v, 8 + n1)
        c_wu = cp(wu_hbm, wu_v, 9 + n1)
        c_wd = cp(wd_hbm, wd_v, 10 + n1)
        for c in [c_phi, c_x0, c_ka, c_kb, c_x0b, c_q, c_v] + [xcopy(i) for i in range(n1)] + [c_wo, c_wg, c_wu, c_wd]:
            c.start()

        def ln_chunks(r0, n, dst, d0):
            def mk(c):
                def f():
                    dst[(d0 + c) // 2:(d0 + c + lnc) // 2, :] = _pk(_ln(x_v[pl.ds(r0 + c, lnc), :].astype(f32)).astype(bf16))
                return f
            return [mk(c) for c in range(0, n, lnc)]

        def feat_post(dst, b, c0):
            def f(p):
                for g in range(0, 4, fg):
                    dst[4 * b + g:4 * b + g + fg, :, pl.ds(c0, 128)] = _pk(_featn(p[40 * g:40 * (g + fg), :]))
            return f

        def v_post(b, c0):
            def f(vT):
                v3 = vT.reshape(4, 40, 128)
                va = jnp.concatenate([v3, jnp.ones((4, 8, 128), f32)], axis=1)
                vaug[4 * b:4 * b + 4, :, pl.ds(c0, 128)] = _pk(va.astype(bf16))
            return f

        def proj(pipe, which, b, xref, xr0, c0):
            wT = (wqT, wkT, wvT)[which]
            post = v_post(b, c0) if which == 2 else feat_post((phiq, phik)[which], b, c0)
            pipe.item(lambda: _nt(_up(wT[80 * b:80 * b + 80, :]), _up(xref[xr0 // 2:xr0 // 2 + 64, :])), post)

        pr = lax.broadcasted_iota(jnp.int32, (D, D), 0)
        pc = lax.broadcasted_iota(jnp.int32, (D, D), 1)
        perm = jnp.where((pr & 31) * DH + (pr >> 5) == pc, 1.0, 0.0).astype(bf16)
        r_i = lax.broadcasted_iota(jnp.int32, (160, 32), 0)
        c_i = lax.broadcasted_iota(jnp.int32, (160, 32), 1)
        E = jnp.where(((r_i % 40) >> 1) == c_i, 1.0, 0.0).astype(bf16)
        r2 = lax.broadcasted_iota(jnp.int32, (160, 128), 0)
        c2 = lax.broadcasted_iota(jnp.int32, (160, 128), 1)
        hr = 2 * (r2 // 40) + (r2 & 1)
        msks = [(6 * t + hr) == ((c2 + 128 * t) // DH) for t in range(5)]
        bcat[...] = jnp.zeros(bcat.shape, f32)

        c_phi.wait()
        for d in range(DH):
            bcat[0:DH, 32 * d:32 * d + 32] = wphi_v[d].astype(f32)
        at = jnp.dot(bcat[...].astype(bf16), perm, preferred_element_type=f32).astype(bf16)
        ptf = jnp.dot(E, at, preferred_element_type=f32)
        pts = [jnp.where(msks[t], ptf[:, 128 * t:128 * t + 128], 0.0).astype(bf16) for t in range(5)]

        def sc(v):
            return (v * LOG2E).astype(bf16)

        def fold_items(pipe, w_v, wT, ts, rs):
            for t in ts:
                def post(r, t=t):
                    rs[t] = r
                    if t >= 1:
                        b = t - 1
                        lo, hi = rs[t - 1], rs[t]
                        parts = []
                        if 40 * b < 120:
                            parts.append(lo[40 * b:120])
                        parts.append(lo[120:160] + hi[0:40])
                        if b > 0:
                            parts.append(hi[40:40 + 40 * b])
                        wT[80 * b:80 * b + 80, :] = _pk(sc(jnp.concatenate(parts, axis=0)))
                r = _nt(pts[t], w_v[:, 128 * t:128 * t + 128])
                post(r)
                if pipe.pending:
                    p, v = pipe.pending.pop(0)
                    p(v)
                if pipe.fill:
                    pipe.fill.pop(0)()

        c_x0.wait()
        for f in ln_chunks(0, P0, xn0, 0):
            f()

        pipe = Pipe(lag)
        rk = {}
        c_ka.wait()
        fold_items(pipe, wk_v, wkT, [0, 1], rk)
        pipe.lag = 100
        for j in range(2):
            proj(pipe, 1, 0, xn0, 128 * j, 128 * j)
        c_kb.wait()
        fold_items(pipe, wk_v, wkT, [2, 3, 4], rk)
        pipe.lag = 2
        for b in range(1, 4):
            for j in range(2):
                proj(pipe, 1, b, xn0, 128 * j, 128 * j)
        c_x0b.wait()
        c_q.wait()
        pipe.fill = ln_chunks(P0, P1 - P0, xn0, P0)
        fold_items(pipe, wq_v, wqT, [0, 1, 2, 3, 4], {})
        for j in range(2):
            for b in range(4):
                proj(pipe, 0, b, xn0, 128 * j, 128 * j)
        pipe.flush_fill()
        for j in range(2, 4):
            for b in range(4):
                proj(pipe, 1, b, xn0, 128 * j, 128 * j)
        c_v.wait()
        xcopy(0).wait()

        def tr(t):
            def f():
                wvT[64 * t:64 * t + 64, :] = _pk(wv_v[:, 128 * t:128 * t + 128].T)
            return f
        pipe.fill = [tr(t) for t in range(5)]
        pipe.lag = lag
        for j in range(2, 4):
            for b in range(4):
                proj(pipe, 0, b, xn0, 128 * j, 128 * j)
        pipe.flush_fill()
        pipe.fill = ln_chunks(P1, 128, xn_buf, 0)
        for j in range(4):
            for b in range(4):
                proj(pipe, 2, b, xn0, 128 * j, 128 * j)
        pipe.flush_fill()
        pipe.drain()

        def p1(i, carry):
            @pl.when(i + 1 < n1)
            def _():
                xcopy(i + 1).wait()

            @pl.when(i + 1 == n1)
            def _():
                c_wo.wait(); c_wg.wait(); c_wu.wait(); c_wd.wait()
            pipe = Pipe(lag)
            for j in range(R):
                c0 = pl.multiple_of(P1 + i * T1 + 128 * j, 128)
                rn = pl.multiple_of(jnp.minimum(P1 + i * T1 + 128 * (j + 1), S - 128), 128)
                pipe.fill = ln_chunks(rn, 128, xn_buf, 128 * ((j + 1) % R))
                for which in (1, 0, 2):
                    for b in range(4):
                        proj(pipe, which, b, xn_buf, 128 * j, c0)
                pipe.flush_fill()
            pipe.drain()
            return carry
        lax.fori_loop(0, n1, p1, 0)

        rr = lax.broadcasted_iota(jnp.int32, (48, 80), 0)
        cc = lax.broadcasted_iota(jnp.int32, (48, 80), 1)
        rowhead = jnp.where(rr < 40, (rr >= 20).astype(jnp.int32), (rr >= 44).astype(jnp.int32))
        msk = (cc & 1) == rowhead
        sub = lax.broadcasted_iota(jnp.int32, (8, HA), 0) < 4

        def num_g(kvg, g, c0):
            nd = jnp.dot(kvg, _up(phiq[g, :, pl.ds(c0, HA)]), preferred_element_type=f32)
            r = _rcp(nd[40:48] + 1e-6)
            rrot = pltpu.roll(r, 4, 0)
            ra = jnp.where(sub, r, rrot)
            rb = jnp.where(sub, rrot, r)
            return [nd[0:8] * ra, nd[8:16] * ra, nd[16:24] * r, nd[24:32] * rb, nd[32:40] * rb]

        def num(c0):
            os = []
            for g in range(NG):
                os += num_g(_up(kvm[g]), g, c0)
            return jnp.concatenate(os, axis=0).astype(bf16).T

        os = []
        prev = None
        for g in range(NG):
            kvg = jnp.where(msk, _nt(_up(vaug[g]), _up(phik[g])), 0.0).astype(bf16)
            kvm[g] = _pk(kvg)
            if prev is not None:
                os += num_g(prev, g - 1, 0)
            prev = kvg
        os += num_g(prev, NG - 1, 0)
        oa_buf[...] = _pk(jnp.concatenate(os, axis=0).astype(bf16).T)

        def ocopy(k):
            return pltpu.make_async_copy(out_v.at[pl.ds(k * op, op)], out_hbm.at[0, pl.ds(k * op, op)], sem_o.at[k])

        def att(o, r0):
            hs, hns = [], []
            for w in range(0, HA, wob):
                at_ = jnp.dot(o[w:w + wob], wo_v[...], preferred_element_type=f32)
                for c in range(0, wob, lnc):
                    h = x_v[pl.ds(r0 + w + c, lnc), :].astype(f32) + at_[c:c + lnc]
                    hs.append(h)
                    hns.append(_ln(h).astype(bf16))
            return jnp.concatenate(hs, axis=0), jnp.concatenate(hns, axis=0)

        def gu(hn, c):
            gt = jnp.dot(hn, wg_v[:, c * fc:(c + 1) * fc], preferred_element_type=f32)
            up = jnp.dot(hn, wu_v[:, c * fc:(c + 1) * fc], preferred_element_type=f32)
            return _gelu_mul(gt, up).astype(bf16)

        def down(c, a):
            return jnp.dot(a, wd_v[c * fc:(c + 1) * fc, :], preferred_element_type=f32)

        nc = F // fc

        def p2(i, carry):
            ra_ = pl.multiple_of(i * T2, T2)
            rb_ = pl.multiple_of(i * T2 + HA, HA)
            rn_ = pl.multiple_of(jnp.minimum(i + 1, n2 - 1) * T2, T2)
            ob = num(rb_)
            ha, hna = att(_up(oa_buf[...]), ra_)
            hb, hnb = att(ob, rb_)
            a0 = jnp.concatenate([gu(hna, 0), gu(hnb, 0)], axis=0)
            oa_buf[...] = _pk(num(rn_))
            hn = jnp.concatenate([hna, hnb], axis=0)
            acc = jnp.concatenate([ha, hb], axis=0) + down(0, a0)
            for c in range(1, nc - 1):
                acc = acc + down(c, gu(hn, c))
            al = gu(hn, nc - 1)
            for k in range(npc):
                res = acc[k * op:(k + 1) * op] + down(nc - 1, al[k * op:(k + 1) * op])
                out_v[pl.ds(pl.multiple_of(i * T2 + k * op, op), op), :] = res.astype(bf16)
                ocopy(i * npc + k).start()
            return carry
        lax.fori_loop(0, n2, p2, 0)
        for k in range(n2 * npc):
            ocopy(k).wait()

    @jax.jit
    def fn(A_x, A_wqkv, A_w_phi, A_wo, B_x, B_w_gate, B_w_up, B_w_down):
        anyspec = pl.BlockSpec(memory_space=pl.ANY)
        wphi_t = jnp.transpose(A_w_phi, (1, 2, 0))
        return pl.pallas_call(
            kernel,
            out_shape=jax.ShapeDtypeStruct((1, S, D), bf16),
            in_specs=[anyspec] * 7,
            out_specs=anyspec,
            scratch_shapes=[
                pltpu.VMEM((S, D), bf16),
                pltpu.VMEM((D, D), bf16),
                pltpu.VMEM((D, D), bf16),
                pltpu.VMEM((D, D), bf16),
                pltpu.VMEM((DH, DH, H), bf16),
                pltpu.VMEM((D, D), bf16),
                pltpu.VMEM((D, F), bf16),
                pltpu.VMEM((D, F), bf16),
                pltpu.VMEM((F, D), bf16),
                pltpu.VMEM((D // 2, D), u32),
                pltpu.VMEM((D // 2, D), u32),
                pltpu.VMEM((D // 2, D), u32),
                pltpu.VMEM((32, D), f32),
                pltpu.VMEM((P1 // 2, D), u32),
                pltpu.VMEM((T1 // 2, D), u32),
                pltpu.VMEM((NG, 40, S), u32),
                pltpu.VMEM((NG, 40, S), u32),
                pltpu.VMEM((NG, 24, S), u32),
                pltpu.VMEM((NG, 24, 80), u32),
                pltpu.VMEM((HA // 2, D), u32),
                pltpu.VMEM((S, D), bf16),
                pltpu.SemaphoreType.DMA((11 + n1,)),
                pltpu.SemaphoreType.DMA((n2 * npc,)),
            ],
            compiler_params=pltpu.CompilerParams(vmem_limit_bytes=100 * 1024 * 1024),
            name="hh",
        )(A_x, A_wqkv, wphi_t, A_wo, B_w_gate, B_w_up, B_w_down)
    return fn


_IMPL = make()


@jax.jit
def pallas_sequential_preLN__linear_kernel_hedgehog__geglu_ffn__prompt_kernel(
    A_x: jax.Array,
    A_wqkv: jax.Array,
    A_w_phi: jax.Array,
    A_wo: jax.Array,
    B_x: jax.Array,
    B_w_gate: jax.Array,
    B_w_up: jax.Array,
    B_w_down: jax.Array,
):
    return _IMPL(A_x, A_wqkv, A_w_phi, A_wo, B_x, B_w_gate, B_w_up, B_w_down)
```

```python
import jax
import jax.numpy as jnp
from jax import lax
from jax.experimental import pallas as pl
from jax.experimental.pallas import tpu as pltpu

S, D, H, DH, F = 2048, 640, 32, 20, 1536
NG = 16
LOG2E = 1.4426950408889634
NT = (((1,), (1,)), ((), ()))
f32 = jnp.float32
bf16 = jnp.bfloat16
u32 = jnp.uint32


def _ln(x):
    m = jnp.mean(x, axis=-1, keepdims=True)
    xc = x - m
    v = jnp.mean(xc * xc, axis=-1, keepdims=True)
    return xc * lax.rsqrt(v + 1e-5)


def _rcp(x):
    r = pl.reciprocal(x, approx=True)
    return r * (2.0 - x * r)


def _featn(p):
    w = p.shape[1]
    ng = p.shape[0] // 40
    p4 = p.reshape(ng, 5, 8, w)

    def allred(m, op):
        m = op(m, pltpu.roll(m, 2, 1))
        return op(m, pltpu.roll(m, 4, 1))

    mx = allred(jnp.max(p4, axis=1), jnp.maximum)
    mn = allred(jnp.min(p4, axis=1), jnp.minimum)
    ep = jnp.exp2(p4 - mx[:, None])
    en = jnp.exp2(mn[:, None] - p4)
    rp = _rcp(allred(jnp.sum(ep, axis=1), jnp.add))
    rn = _rcp(allred(jnp.sum(en, axis=1), jnp.add))
    phi = jnp.concatenate([ep * rp[:, None], en * rn[:, None]], axis=1)
    return phi.reshape(ng, 80, w).astype(bf16)


def _gelu_mul(g, u):
    c = 0.7978845608028654
    inner = g * (c + (c * 0.044715) * (g * g))
    t = jnp.tanh(inner)
    hgu = (0.5 * g) * u
    return hgu + hgu * t


def _pk(v):
    return pltpu.bitcast(v, u32)


def _up(v):
    return pltpu.bitcast(v, bf16)


def _nt(a, b):
    return lax.dot_general(a, b, NT, preferred_element_type=f32)


PIECES = {0: (128, 128, 128, 128), 1: (128, 128, 128, 64, 64), 2: (128, 128, 128, 64, 32, 32), 3: (256, 128, 64, 64),
          4: (192, 128, 96, 64, 32), 5: (128, 128, 128, 64, 48, 16), 6: (256, 128, 64, 32, 32)}


def make(fc=512, NP=6, R=5, T2=512, pcs=2, lnc=64, wob=64, fg=2, defer=2, scopes=0, nw=256, ngl=8, ngs=4, kdef=3, nb=0, ns=0, si=1):
    T1 = 128 * R
    P1 = 128 * NP
    n1 = (S - P1) // T1
    assert P1 + n1 * T1 == S
    n2 = S // T2
    pieces = PIECES[pcs]
    assert sum(pieces) == T2
    npc = len(pieces)
    poff = [sum(pieces[:k]) for k in range(npc)]

    def kernel(*refs):
        @pl.when(pl.program_id(0) == 0)
        def _():
            body(*refs)

    def body(x_hbm, wqkv_hbm, wphi_hbm, wo_hbm, wg_hbm, wu_hbm, wd_hbm, out_hbm,
             x_v, wq_v, wk_v, wv_v, wphi_v, wo_v, wg_v, wu_v, wd_v, wqT, wkT, wvT, bcat,
             xn0, xn_buf, phiq, phik, vaug, kvm, out_v, sem):
        _st = []

        def mark(name=None):
            if not scopes:
                return
            if _st:
                _st.pop().__exit__(None, None, None)
            if name:
                c = jax.named_scope(name)
                c.__enter__()
                _st.append(c)

        def waits(name, cs, starts=()):
            mark(name + "_wait")
            for c in cs:
                c.wait()
            mark(name)
            for c in starts:
                c.start()

        mark("s0")

        def cp(src, dst, k):
            return pltpu.make_async_copy(src, dst, sem.at[k])

        def xrows(r0, r1, k):
            return cp(x_hbm.at[0, pl.ds(r0, r1 - r0)], x_v.at[pl.ds(r0, r1 - r0)], k)

        def wk_cols(c0, n, k):
            return cp(wqkv_hbm.at[:, pl.ds(D + c0, n)], wk_v.at[:, pl.ds(c0, n)], k)
        g_phi = [cp(wphi_hbm, wphi_v, 0)]
        g_x0 = [xrows(0, 256, 1)]
        g_ka = [wk_cols(0, 256, 2)]
        g_kb = [wk_cols(256, 256, 3)]
        g_kc = [wk_cols(512, 128, 0), xrows(256, P1, 0)]
        g_qv = [cp(wqkv_hbm.at[:, pl.ds(0, D)], wq_v, 1), cp(wqkv_hbm.at[:, pl.ds(2 * D, D)], wv_v, 1),
                xrows(P1, P1 + 128, 1)]
        g_xr = [xrows(P1 + 128, S, 2)]
        g_w = [cp(wo_hbm, wo_v, 3), cp(wg_hbm, wg_v, 3), cp(wu_hbm, wu_v, 3), cp(wd_hbm, wd_v, 3)]
        for c in g_phi + g_x0 + g_ka + g_kb:
            c.start()

        def ln_rows(r0, n, dst, d0):
            for c in range(0, n, lnc):
                dst[(d0 + c) // 2:(d0 + c + lnc) // 2, :] = _pk(_ln(x_v[pl.ds(r0 + c, lnc), :].astype(f32)).astype(bf16))

        pending = []

        def drain(keep=0):
            while len(pending) > keep:
                pending.pop(0)()

        def proj(which, ga, ng, xref, xr0, c0):
            wT = (wqT, wkT, wvT)[which]
            p = _nt(_up(wT[20 * ga:20 * (ga + ng), :]), _up(xref[xr0 // 2:xr0 // 2 + 64, :]))

            def post():
                if which == 2:
                    v3 = p.reshape(ng, 40, 128)
                    va = jnp.concatenate([v3, jnp.ones((ng, 8, 128), f32)], axis=1)
                    vaug[ga:ga + ng, :, pl.ds(c0, 128)] = _pk(va.astype(bf16))
                else:
                    dst = (phiq, phik)[which]
                    for g in range(0, ng, fg):
                        dst[ga + g:ga + g + fg, :, pl.ds(c0, 128)] = _pk(_featn(p[40 * g:40 * (g + fg), :]))
            pending.append(post)

        def pj(which, b, j, ng=4):
            proj(which, 4 * b, ng, xn0, 128 * j, 128 * j)

        pr = lax.broadcasted_iota(jnp.int32, (D, D), 0)
        pc = lax.broadcasted_iota(jnp.int32, (D, D), 1)
        perm = jnp.where((pr & 31) * DH + (pr >> 5) == pc, 1.0, 0.0).astype(bf16)
        r_i = lax.broadcasted_iota(jnp.int32, (160, 32), 0)
        c_i = lax.broadcasted_iota(jnp.int32, (160, 32), 1)
        E = jnp.where(((r_i % 40) >> 1) == c_i, 1.0, 0.0).astype(bf16)
        r2 = lax.broadcasted_iota(jnp.int32, (160, 128), 0)
        c2 = lax.broadcasted_iota(jnp.int32, (160, 128), 1)
        hr = 2 * (r2 // 40) + (r2 & 1)
        msks = [(6 * t + hr) == ((c2 + 128 * t) // DH) for t in range(5)]
        bcat[...] = jnp.zeros(bcat.shape, f32)

        waits("s1", g_phi, g_kc)
        for d in range(DH):
            bcat[0:DH, 32 * d:32 * d + 32] = wphi_v[d].astype(f32)
        at = jnp.dot(bcat[...].astype(bf16), perm, preferred_element_type=f32).astype(bf16)
        ptf = jnp.dot(E, at, preferred_element_type=f32)
        pts = [jnp.where(msks[t], ptf[:, 128 * t:128 * t + 128], 0.0).astype(bf16) for t in range(5)]

        def fold(w_v, wT, t, rs):
            rs[t] = _nt(pts[t], w_v[:, 128 * t:128 * t + 128])
            if t >= 1:
                b = t - 1
                lo, hi = rs[t - 1], rs[t]
                parts = []
                if 40 * b < 120:
                    parts.append(lo[40 * b:120])
                parts.append(lo[120:160] + hi[0:40])
                if b > 0:
                    parts.append(hi[40:40 + 40 * b])
                wT[80 * b:80 * b + 80, :] = _pk((jnp.concatenate(parts, axis=0) * LOG2E).astype(bf16))

        waits("s2", g_x0, g_qv)
        ln_rows(0, 256, xn0, 0)

        rk, rq = {}, {}
        waits("s3", g_ka, g_xr)
        fold(wk_v, wkT, 0, rk)
        fold(wk_v, wkT, 1, rk)
        pj(1, 0, 0)
        pj(1, 0, 1)
        waits("s4", g_kb, g_w)
        fold(wk_v, wkT, 2, rk)
        fold(wk_v, wkT, 3, rk)
        for b, j in [(1, 0), (1, 1), (2, 0), (2, 1)]:
            pj(1, b, j)
        drain(defer)
        waits("s5", g_kc)
        fold(wk_v, wkT, 4, rk)
        ln_rows(256, P1 - 256, xn0, 256)
        ks = [(3, 0), (3, 1)] + [(b, j) for j in range(2, NP) for b in range(4)]
        for b, j in ks[:len(ks) - kdef]:
            pj(1, b, j)
        drain(defer)
        waits("s6", g_qv)
        for t in range(5):
            fold(wq_v, wqT, t, rq)
        for b, j in ks[len(ks) - kdef:]:
            pj(1, b, j)
        for t in range(5):
            wvT[64 * t:64 * t + 64, :] = _pk(wv_v[:, 128 * t:128 * t + 128].T)
        ln_rows(P1, 128, xn_buf, 0)
        for which in (0, 2):
            for j in range(NP):
                for b in range(0, 4, ngs // 4):
                    pj(which, b, j, ngs)
        drain()

        def p1(i, carry):
            for j in range(R):
                c0 = pl.multiple_of(P1 + i * T1 + 128 * j, 128)
                rn = pl.multiple_of(jnp.minimum(P1 + i * T1 + 128 * (j + 1), S - 128), 128)
                ln_rows(rn, 128, xn_buf, 128 * ((j + 1) % R))
                for which in (1, 0, 2):
                    for g in range(0, NG, ngl):
                        proj(which, g, ngl, xn_buf, 128 * j, c0)
                        drain()
            return carry
        waits("s8_loop1", g_xr)
        lax.fori_loop(0, n1, p1, 0)
        mark("s9_kv")

        rr = lax.broadcasted_iota(jnp.int32, (48, 80), 0)
        cc = lax.broadcasted_iota(jnp.int32, (48, 80), 1)
        rowhead = jnp.where(rr < 40, (rr >= 20).astype(jnp.int32), (rr >= 44).astype(jnp.int32))
        msk = (cc & 1) == rowhead
        for g in range(NG):
            kvm[g] = _pk(jnp.where(msk, _nt(_up(vaug[g]), _up(phik[g])), 0.0).astype(bf16))

        def num(c0, n):
            sub = lax.broadcasted_iota(jnp.int32, (8, n), 0) < 4
            os = []
            for g in range(NG):
                nd = jnp.dot(_up(kvm[g]), _up(phiq[g, :, pl.ds(c0, n)]), preferred_element_type=f32)
                r = _rcp(nd[40:48] + 1e-6)
                rrot = pltpu.roll(r, 4, 0)
                ra = jnp.where(sub, r, rrot)
                rb = jnp.where(sub, rrot, r)
                os += [nd[0:8] * ra, nd[8:16] * ra, nd[16:24] * r, nd[24:32] * rb, nd[32:40] * rb]
            return jnp.concatenate(os, axis=0).astype(bf16).T

        def ocopy(i, k):
            r0 = i * T2 + poff[k]
            return pltpu.make_async_copy(out_v.at[pl.ds(r0, pieces[k])], out_hbm.at[0, pl.ds(r0, pieces[k])], sem.at[0])

        def att(o, r0):
            n = o.shape[0]
            at_ = jnp.dot(o, wo_v[...], preferred_element_type=f32)
            hs, hns = [], []
            for c in range(0, n, lnc):
                h = x_v[pl.ds(r0 + c, lnc), :].astype(f32) + at_[c:c + lnc]
                hs.append(h)
                hns.append(_ln(h).astype(bf16))
            return hs, hns

        def gu(hn, c):
            gt = jnp.dot(hn, wg_v[:, c * fc:(c + 1) * fc], preferred_element_type=f32)
            up = jnp.dot(hn, wu_v[:, c * fc:(c + 1) * fc], preferred_element_type=f32)
            return _gelu_mul(gt, up).astype(bf16)

        def down(c, a):
            return jnp.dot(a, wd_v[c * fc:(c + 1) * fc, :], preferred_element_type=f32)

        nc = F // fc

        def p2(i, carry):
            nbk = T2 // wob
            rs = [pl.multiple_of(i * T2 + w * wob, wob) for w in range(nbk)]
            o = jnp.concatenate([num(pl.multiple_of(i * T2 + w, nw), nw) for w in range(0, T2, nw)], axis=0)
            hs, hns = [], []
            for w in range(nbk):
                a_, b_ = att(o[w * wob:(w + 1) * wob], rs[w])
                hs += a_
                hns += b_
            hh = len(hns) // 2
            hna = jnp.concatenate(hns[:hh], axis=0)
            hnb = jnp.concatenate(hns[hh:], axis=0)
            a0 = jnp.concatenate([gu(hna, 0), gu(hnb, 0)], axis=0)
            hn = jnp.concatenate(hns, axis=0)
            acc = jnp.concatenate(hs, axis=0) + down(0, a0)
            for c in range(1, nc - 1):
                acc = acc + down(c, gu(hn, c))
            al = gu(hn, nc - 1)
            for k in range(npc):
                lo, hi = poff[k], poff[k] + pieces[k]
                res = acc[lo:hi] + down(nc - 1, al[lo:hi])
                out_v[pl.ds(pl.multiple_of(i * T2 + lo, 16), pieces[k]), :] = res.astype(bf16)
                ocopy(i, k).start()
            return carry
        waits("sa_loop2", g_w)
        lax.fori_loop(0, n2, p2, 0)
        mark("sb_tail")
        pltpu.make_async_copy(out_v, out_hbm.at[0], sem.at[0]).wait()
        mark()

    @jax.jit
    def fn(A_x, A_wqkv, A_w_phi, A_wo, B_x, B_w_gate, B_w_up, B_w_down):
        anyspec = pl.BlockSpec(memory_space=pl.ANY)
        wphi_t = jnp.transpose(A_w_phi, (1, 2, 0))
        return pl.pallas_call(
            kernel,
            out_shape=jax.ShapeDtypeStruct((1, S, D), bf16),
            grid=(2,),
            in_specs=[anyspec] * 7,
            out_specs=anyspec,
            scratch_shapes=[
                pltpu.VMEM((S, D), bf16),
                pltpu.VMEM((D, D), bf16),
                pltpu.VMEM((D, D), bf16),
                pltpu.VMEM((D, D), bf16),
                pltpu.VMEM((DH, DH, H), bf16),
                pltpu.VMEM((D, D), bf16),
                pltpu.VMEM((D, F), bf16),
                pltpu.VMEM((D, F), bf16),
                pltpu.VMEM((F, D), bf16),
                pltpu.VMEM((D // 2, D), u32),
                pltpu.VMEM((D // 2, D), u32),
                pltpu.VMEM((D // 2, D), u32),
                pltpu.VMEM((32, D), f32),
                pltpu.VMEM((P1 // 2, D), u32),
                pltpu.VMEM((T1 // 2, D), u32),
                pltpu.VMEM((NG, 40, S), u32),
                pltpu.VMEM((NG, 40, S), u32),
                pltpu.VMEM((NG, 24, S), u32),
                pltpu.VMEM((NG, 24, 80), u32),
                pltpu.VMEM((S, D), bf16),
                pltpu.SemaphoreType.DMA((4,)),
            ],
            compiler_params=pltpu.CompilerParams(vmem_limit_bytes=100 * 1024 * 1024, disable_bounds_checks=bool(nb),
                                                 disable_semaphore_checks=bool(ns), shape_invariant_numerics=bool(si)),
            name="hh",
        )(A_x, A_wqkv, wphi_t, A_wo, B_w_gate, B_w_up, B_w_down)
    return fn


_IMPL = make(nb=1, ns=1)


@jax.jit
def pallas_sequential_preLN__linear_kernel_hedgehog__geglu_ffn__prompt_kernel(
    A_x: jax.Array,
    A_wqkv: jax.Array,
    A_w_phi: jax.Array,
    A_wo: jax.Array,
    B_x: jax.Array,
    B_w_gate: jax.Array,
    B_w_up: jax.Array,
    B_w_down: jax.Array,
):
    return _IMPL(A_x, A_wqkv, A_w_phi, A_wo, B_x, B_w_gate, B_w_up, B_w_down)
```

```python
import jax
import jax.numpy as jnp
from jax import lax
from jax.experimental import pallas as pl
from jax.experimental.pallas import tpu as pltpu

S, D, H, DH, F = 2048, 640, 32, 20, 1536
NG = H // 2
LOG2E = 1.4426950408889634
NT_DIMS = (((1,), (1,)), ((), ()))
f32 = jnp.float32
bf16 = jnp.bfloat16
u32 = jnp.uint32

NP = 6
R = 5
T1 = 128 * R
P1 = 128 * NP
N1 = (S - P1) // T1
T2 = 512
N2 = S // T2
NW = 256
WOB = 64
LNC = 64
FC = 512
PIECES = (128, 128, 128, 64, 32, 32)
POFF = tuple(sum(PIECES[:k]) for k in range(len(PIECES)))
K_OFF, Q_OFF, V_OFF = 0, 304, 608
assert P1 + N1 * T1 == S and sum(PIECES) == T2


def _ln(x):
    m = jnp.mean(x, axis=-1, keepdims=True)
    xc = x - m
    v = jnp.mean(xc * xc, axis=-1, keepdims=True) + 1e-5
    return xc * jnp.exp2(jnp.log(v) * (-0.5 * LOG2E))


def _rcp(x):
    return pl.reciprocal(x, approx=True)


def _allred(m, op):
    m = op(m, pltpu.roll(m, 2, 0))
    return op(m, pltpu.roll(m, 4, 0))


def _tree(op, xs):
    return op(op(op(xs[0], xs[1]), op(xs[2], xs[3])), xs[4])


def _feat5(ps):
    mx = _allred(_tree(jnp.maximum, ps), jnp.maximum)
    mn = _allred(_tree(jnp.minimum, ps), jnp.minimum)
    ep = [jnp.exp2(q - mx) for q in ps]
    en = [jnp.exp2(mn - q) for q in ps]
    rp = _rcp(_allred(_tree(jnp.add, ep), jnp.add))
    rn = _rcp(_allred(_tree(jnp.add, en), jnp.add))
    return jnp.concatenate([e * rp for e in ep] + [e * rn for e in en], axis=0).astype(bf16)


def _gelu_mul(g, u):
    c = 0.7978845608028654
    t = jnp.tanh(g * (c + (c * 0.044715) * (g * g)))
    hgu = (0.5 * g) * u
    return hgu + hgu * t


def _pk(v):
    return pltpu.bitcast(v, u32)


def _up(v):
    return pltpu.bitcast(v, bf16)


def _nt(a, b):
    return lax.dot_general(a, b, NT_DIMS, preferred_element_type=f32)


def _nn(a, b):
    return jnp.dot(a, b, preferred_element_type=f32)


def _pair_is(a, w):
    return (lax.broadcasted_iota(jnp.int32, (8, w), 0) >> 1) == a


def _body(x_hbm, wqkv_hbm, wphi_hbm, wo_hbm, wg_hbm, wu_hbm, wd_hbm, out_hbm,
          x_v, wq_v, wk_v, wv_v, wphi_v, wo_v, wg_v, wu_v, wd_v, wT, bcat,
          xn0, xn_buf, phiq, phik, vaug, kvm, out_v, sem):
    def cp(src, dst, k):
        return pltpu.make_async_copy(src, dst, sem.at[k])

    def xrows(r0, r1, k):
        return cp(x_hbm.at[0, pl.ds(r0, r1 - r0)], x_v.at[pl.ds(r0, r1 - r0)], k)

    def wk_cols(c0, n, k):
        return cp(wqkv_hbm.at[:, pl.ds(D + c0, n)], wk_v.at[:, pl.ds(c0, n)], k)

    g_phi = [cp(wphi_hbm, wphi_v, 0)]
    g_x0 = [xrows(0, 256, 1)]
    g_ka = [wk_cols(0, 256, 2)]
    g_kb = [wk_cols(256, 256, 3)]
    g_kc = [wk_cols(512, 128, 0), xrows(256, P1, 0)]
    g_qv = [cp(wqkv_hbm.at[:, pl.ds(0, D)], wq_v, 1), cp(wqkv_hbm.at[:, pl.ds(2 * D, D)], wv_v, 1),
            xrows(P1, P1 + 128, 1)]
    g_xr = [xrows(P1 + 128, S, 2)]
    g_w = [cp(wo_hbm, wo_v, 3), cp(wg_hbm, wg_v, 3), cp(wu_hbm, wu_v, 3), cp(wd_hbm, wd_v, 3)]

    def waits(cs, starts=()):
        for c in cs:
            c.wait()
        for c in starts:
            c.start()

    for c in g_phi + g_x0 + g_ka + g_kb:
        c.start()

    def ln_rows(r0, n, dst, d0):
        for c in range(0, n, LNC):
            xn = _ln(x_v[pl.ds(r0 + c, LNC), :].astype(f32)).astype(bf16)
            dst[(d0 + c) // 2:(d0 + c + LNC) // 2, :] = _pk(xn)

    pending = []

    def drain(keep=0):
        while len(pending) > keep:
            pending.pop(0)()

    def feat_block(p, dst, b, c0, rfirst=True):
        ro, mo = (0, 24) if rfirst else (128, 0)
        rs = [p[ro + 8 * a:ro + 8 + 8 * a] for a in range(3)]
        for a in range(4):
            if a < 3:
                v4 = jnp.where(_pair_is(a, 128), 0.0, rs[a])
            else:
                v4 = jnp.where(_pair_is(0, 128), rs[0],
                               jnp.where(_pair_is(1, 128), rs[1], jnp.where(_pair_is(2, 128), rs[2], 0.0)))
            ps = [p[mo + 32 * a + 8 * v:mo + 8 + 32 * a + 8 * v] for v in range(4)] + [v4]
            dst[4 * b + a, :, pl.ds(c0, 128)] = _pk(_feat5(ps))

    def xs(xref, xr0):
        return _up(xref[xr0 // 2:xr0 // 2 + 64, :])

    def proj_qk(off, dst, B, xref, xr0, c0):
        p = _nt(_up(wT[off + 152 * B:off + 152 * B + 152, :]), xs(xref, xr0))

        def post():
            feat_block(p[0:152], dst, 2 * B, c0)
            feat_block(p[152:304], dst, 2 * B + 1, c0)
        pending.append(post)

    def proj_k4(wb, b, j, rfirst):
        p = _nt(wb, xs(xn0, 128 * j))
        pending.append(lambda: feat_block(p[0:152], phik, b, 128 * j, rfirst))

    def proj_v(ga, ng, xref, xr0, c0):
        p = _nt(_up(wT[V_OFF + 20 * ga:V_OFF + 20 * (ga + ng), :]), xs(xref, xr0))

        def post():
            va = jnp.concatenate([p.reshape(ng, 40, 128), jnp.ones((ng, 8, 128), f32)], axis=1)
            vaug[ga:ga + ng, :, pl.ds(c0, 128)] = _pk(va.astype(bf16))
        pending.append(post)

    pr = lax.broadcasted_iota(jnp.int32, (D, D), 0)
    pc = lax.broadcasted_iota(jnp.int32, (D, D), 1)
    perm = jnp.where((pr & 31) * DH + (pr >> 5) == pc, 1.0, 0.0).astype(bf16)
    r_i = lax.broadcasted_iota(jnp.int32, (160, 32), 0)
    c_i = lax.broadcasted_iota(jnp.int32, (160, 32), 1)
    gl = r_i // 40
    sl = (r_i - 40 * gl) >> 1
    q_ = sl - 16
    f_ = jnp.where(sl < 16, sl + 1, jnp.where(q_ == gl, 0, jnp.where(q_ < gl, 17 + q_, 16 + q_)))
    e0 = jnp.where(f_ == c_i, 1.0, 0.0)
    es = []
    for t in range(5):
        off = (120 * t) % 160
        es.append((jnp.concatenate([e0[off:], e0[:off]], axis=0) if off else e0).astype(bf16))
    r2 = lax.broadcasted_iota(jnp.int32, (160, 128), 0)
    hr = 2 * (r2 // 40) + (r2 & 1)
    hc = [(lax.broadcasted_iota(jnp.int32, (1, 128), 1) + 128 * t) // DH - 6 * t for t in range(5)]
    bcat[...] = jnp.zeros(bcat.shape, f32)

    waits(g_phi, g_kc)
    for d in range(DH):
        bcat[0:DH, 32 * d:32 * d + 32] = wphi_v[d].astype(f32)
    at = _nn(bcat[...].astype(bf16), perm).astype(bf16)
    pts = [jnp.where(hr == hc[t], _nn(es[t], at[:, 128 * t:128 * t + 128]), 0.0).astype(bf16) for t in range(5)]

    def fold(w_v, off, t, rs, blk):
        rs[t] = _nt(pts[t], w_v[:, 128 * t:128 * t + 128])
        if t == 0:
            return
        b = t - 1
        lo, hi = rs[t - 1], rs[t]
        parts = []
        if b < 3:
            parts.append(lo[40 * b:120])
        parts.append(lo[120:160] + hi[0:40])
        if b > 0:
            parts.append(hi[40:40 + 40 * b])
        w = jnp.concatenate(parts, axis=0)
        mains, v4s = [], []
        for a in range(4):
            v4 = w[40 * a + 32:40 * a + 40]
            base = _allred(jnp.where(_pair_is(a, D), v4, 0.0), jnp.add)
            mains += [(w[40 * a + 8 * v:40 * a + 8 * v + 8] - base) * LOG2E for v in range(4)]
            v4s.append((v4 - base) * LOG2E)
        shared = [jnp.where(_pair_is(a, D), v4s[3], v4s[a]) for a in range(3)]
        blk[b] = (shared, mains)
        if b % 2 == 1:
            B = b // 2
            rows = blk[b - 1][0] + blk[b - 1][1] + blk[b][0] + blk[b][1]
            wT[off + 152 * B:off + 152 * B + 152, :] = _pk(jnp.concatenate(rows, axis=0).astype(bf16))

    def blk16(slabs, rfirst):
        rows = slabs[0] + slabs[1] if rfirst else slabs[1] + slabs[0]
        return jnp.concatenate(rows + [jnp.zeros((8, D), f32)], axis=0).astype(bf16)

    waits(g_x0, g_qv)
    ln_rows(0, 256, xn0, 0)

    rk, rq, bk, bq = {}, {}, {}, {}
    waits(g_ka, g_xr)
    fold(wk_v, K_OFF, 0, rk, bk)
    fold(wk_v, K_OFF, 1, rk, bk)
    w0 = blk16(bk[0], False)
    proj_k4(w0, 0, 0, False)
    proj_k4(w0, 0, 1, False)

    waits(g_kb, g_w)
    fold(wk_v, K_OFF, 2, rk, bk)
    fold(wk_v, K_OFF, 3, rk, bk)
    w1 = blk16(bk[1], False)
    proj_k4(w1, 1, 0, False)
    proj_k4(w1, 1, 1, False)
    w2 = blk16(bk[2], True)
    proj_k4(w2, 2, 0, True)
    drain(1)

    waits(g_kc)
    fold(wk_v, K_OFF, 4, rk, bk)
    proj_k4(w2, 2, 1, True)
    ln_rows(256, P1 - 256, xn0, 256)
    w3 = blk16(bk[3], True)
    proj_k4(w3, 3, 0, True)
    proj_k4(w3, 3, 1, True)
    for j in range(2, NP):
        for B in range(2):
            proj_qk(K_OFF, phik, B, xn0, 128 * j, 128 * j)
    drain(1)

    waits(g_qv)
    for t in range(5):
        fold(wq_v, Q_OFF, t, rq, bq)
    for t in range(5):
        wT[V_OFF + 64 * t:V_OFF + 64 * t + 64, :] = _pk(wv_v[:, 128 * t:128 * t + 128].T)
    ln_rows(P1, 128, xn_buf, 0)
    for j in range(NP):
        for B in range(2):
            proj_qk(Q_OFF, phiq, B, xn0, 128 * j, 128 * j)
    for j in range(NP):
        for g in range(0, NG, 4):
            if j == NP - 1 and g == NG - 4:
                proj_v(g, 2, xn0, 128 * j, 128 * j)
                proj_v(g + 2, 2, xn0, 128 * j, 128 * j)
            else:
                proj_v(g, 4, xn0, 128 * j, 128 * j)
    drain()

    def p1(i, carry):
        for j in range(R):
            c0 = pl.multiple_of(P1 + i * T1 + 128 * j, 128)
            rn = pl.multiple_of(jnp.minimum(P1 + i * T1 + 128 * (j + 1), S - 128), 128)
            ln_rows(rn, 128, xn_buf, 128 * ((j + 1) % R))
            for off, dst in ((K_OFF, phik), (Q_OFF, phiq)):
                for B in range(2):
                    proj_qk(off, dst, B, xn_buf, 128 * j, c0)
                    drain()
            for g in range(0, NG, 4):
                proj_v(g, 4, xn_buf, 128 * j, c0)
                drain()
        return carry

    waits(g_xr)
    lax.fori_loop(0, N1, p1, 0)

    rr = lax.broadcasted_iota(jnp.int32, (48, 80), 0)
    cc = lax.broadcasted_iota(jnp.int32, (48, 80), 1)
    rowhead = jnp.where(rr < 40, (rr >= 20).astype(jnp.int32), (rr >= 44).astype(jnp.int32))
    msk = (cc & 1) == rowhead
    for g in range(NG):
        kvm[g] = _pk(jnp.where(msk, _nt(_up(vaug[g]), _up(phik[g])), 0.0).astype(bf16))

    def attn_o(c0):
        sub = lax.broadcasted_iota(jnp.int32, (8, NW), 0) < 4
        os = []
        for g in range(NG):
            nd = _nn(_up(kvm[g]), _up(phiq[g, :, pl.ds(c0, NW)]))
            r = _rcp(nd[40:48] + 1e-6)
            rrot = pltpu.roll(r, 4, 0)
            ra = jnp.where(sub, r, rrot)
            rb = jnp.where(sub, rrot, r)
            os += [nd[0:8] * ra, nd[8:16] * ra, nd[16:24] * r, nd[24:32] * rb, nd[32:40] * rb]
        return jnp.concatenate(os, axis=0).astype(bf16).T

    def gu(hn, c):
        gt = _nn(hn, wg_v[:, c * FC:(c + 1) * FC])
        up = _nn(hn, wu_v[:, c * FC:(c + 1) * FC])
        return _gelu_mul(gt, up).astype(bf16)

    def down(c, a):
        return _nn(a, wd_v[c * FC:(c + 1) * FC, :])

    nc = F // FC

    def p2(i, carry):
        o = jnp.concatenate([attn_o(pl.multiple_of(i * T2 + w, NW)) for w in range(0, T2, NW)], axis=0)
        hs, hns = [], []
        for w in range(0, T2, WOB):
            r0 = pl.multiple_of(i * T2 + w, WOB)
            h = x_v[pl.ds(r0, WOB), :].astype(f32) + _nn(o[w:w + WOB], wo_v[...])
            hs.append(h)
            hns.append(_ln(h).astype(bf16))
        half = len(hns) // 2
        a0 = jnp.concatenate([gu(jnp.concatenate(hns[:half], axis=0), 0),
                              gu(jnp.concatenate(hns[half:], axis=0), 0)], axis=0)
        hn = jnp.concatenate(hns, axis=0)
        acc = jnp.concatenate(hs, axis=0) + down(0, a0)
        for c in range(1, nc - 1):
            acc = acc + down(c, gu(hn, c))
        al = gu(hn, nc - 1)
        for lo, n in zip(POFF, PIECES):
            res = acc[lo:lo + n] + down(nc - 1, al[lo:lo + n])
            r0 = pl.multiple_of(i * T2 + lo, 16)
            out_v[pl.ds(r0, n), :] = res.astype(bf16)
            cp(out_v.at[pl.ds(r0, n)], out_hbm.at[0, pl.ds(r0, n)], 0).start()
        return carry

    waits(g_w)
    lax.fori_loop(0, N2, p2, 0)
    cp(out_v, out_hbm.at[0], 0).wait()


def _kernel(*refs):
    @pl.when(pl.program_id(0) == 0)
    def _():
        _body(*refs)


@jax.jit
def pallas_sequential_preLN__linear_kernel_hedgehog__geglu_ffn__prompt_kernel(
    A_x: jax.Array,
    A_wqkv: jax.Array,
    A_w_phi: jax.Array,
    A_wo: jax.Array,
    B_x: jax.Array,
    B_w_gate: jax.Array,
    B_w_up: jax.Array,
    B_w_down: jax.Array,
):
    del B_x
    anyspec = pl.BlockSpec(memory_space=pl.ANY)
    wphi_t = jnp.transpose(A_w_phi, (1, 2, 0))
    return pl.pallas_call(
        _kernel,
        out_shape=jax.ShapeDtypeStruct((1, S, D), bf16),
        grid=(2,),
        in_specs=[anyspec] * 7,
        out_specs=anyspec,
        scratch_shapes=[
            pltpu.VMEM((S, D), bf16),
            pltpu.VMEM((D, D), bf16),
            pltpu.VMEM((D, D), bf16),
            pltpu.VMEM((D, D), bf16),
            pltpu.VMEM((DH, DH, H), bf16),
            pltpu.VMEM((D, D), bf16),
            pltpu.VMEM((D, F), bf16),
            pltpu.VMEM((D, F), bf16),
            pltpu.VMEM((F, D), bf16),
            pltpu.VMEM((928, D), u32),
            pltpu.VMEM((32, D), f32),
            pltpu.VMEM((P1 // 2, D), u32),
            pltpu.VMEM((T1 // 2, D), u32),
            pltpu.VMEM((NG, 40, S), u32),
            pltpu.VMEM((NG, 40, S), u32),
            pltpu.VMEM((NG, 24, S), u32),
            pltpu.VMEM((NG, 24, 80), u32),
            pltpu.VMEM((S, D), bf16),
            pltpu.SemaphoreType.DMA((4,)),
        ],
        compiler_params=pltpu.CompilerParams(
            dimension_semantics=("arbitrary",),
            vmem_limit_bytes=100 * 1024 * 1024,
            disable_bounds_checks=True,
            disable_semaphore_checks=True,
        ),
        name="hh",
    )(A_x, A_wqkv, wphi_t, A_wo, B_w_gate, B_w_up, B_w_down)
```

```python
import jax
import jax.numpy as jnp
from jax import lax
from jax.experimental import pallas as pl
from jax.experimental.pallas import tpu as pltpu

S, D, H, DH, F = 2048, 640, 32, 20, 1536
NG = H // 2
LOG2E = 1.4426950408889634
NT_DIMS = (((1,), (1,)), ((), ()))
f32 = jnp.float32
bf16 = jnp.bfloat16
u32 = jnp.uint32

NP = 5
R = 5
T1 = 128 * R
P1 = 128 * NP
N1 = (S - P1 - 128) // T1
T2 = 512
N2 = S // T2
NW = 256
WOB = 64
LNC = 64
FC = 512
PIECES = (128, 128, 128, 64, 32, 32)
POFF = tuple(sum(PIECES[:k]) for k in range(len(PIECES)))
K_OFF, Q_OFF, V_OFF = 0, 304, 608
assert P1 + N1 * T1 + 128 == S and sum(PIECES) == T2


def _ln(x):
    m = jnp.mean(x, axis=-1, keepdims=True)
    xc = x - m
    v = jnp.mean(xc * xc, axis=-1, keepdims=True) + 1e-5
    return xc * jnp.exp2(jnp.log(v) * (-0.5 * LOG2E))


def _rcp(x):
    return pl.reciprocal(x, approx=True)


def _allred(m, op):
    m = op(m, pltpu.roll(m, 2, 0))
    return op(m, pltpu.roll(m, 4, 0))


def _tree(op, xs):
    return op(op(op(xs[0], xs[1]), op(xs[2], xs[3])), xs[4])


def _feat5(ps):
    mx = _allred(_tree(jnp.maximum, ps), jnp.maximum)
    mn = _allred(_tree(jnp.minimum, ps), jnp.minimum)
    ep = [jnp.exp2(q - mx) for q in ps]
    en = [jnp.exp2(mn - q) for q in ps]
    rp = _rcp(_allred(_tree(jnp.add, ep), jnp.add))
    rn = _rcp(_allred(_tree(jnp.add, en), jnp.add))
    return jnp.concatenate([e * rp for e in ep] + [e * rn for e in en], axis=0).astype(bf16)


def _gelu_mul(g, u):
    c = 0.7978845608028654
    t = jnp.tanh(g * (c + (c * 0.044715) * (g * g)))
    hgu = (0.5 * g) * u
    return hgu + hgu * t


def _pk(v):
    return pltpu.bitcast(v, u32)


def _up(v):
    return pltpu.bitcast(v, bf16)


def _nt(a, b):
    return lax.dot_general(a, b, NT_DIMS, preferred_element_type=f32)


def _nn(a, b):
    return jnp.dot(a, b, preferred_element_type=f32)


def _pair_is(a, w):
    return (lax.broadcasted_iota(jnp.int32, (8, w), 0) >> 1) == a


def _body(x_hbm, wqkv_hbm, wphi_hbm, wo_hbm, wg_hbm, wu_hbm, wd_hbm, out_hbm,
          x_v, wq_v, wk_v, wv_v, wphi_v, wo_v, wg_v, wu_v, wd_v, wT, bcat,
          xn0, xn_buf, phiq, phik, vaug, kvm, out_v, sem):
    def cp(src, dst, k):
        return pltpu.make_async_copy(src, dst, sem.at[k])

    def xrows(r0, r1, k):
        return cp(x_hbm.at[0, pl.ds(r0, r1 - r0)], x_v.at[pl.ds(r0, r1 - r0)], k)

    def wk_cols(c0, n, k):
        return cp(wqkv_hbm.at[:, pl.ds(D + c0, n)], wk_v.at[:, pl.ds(c0, n)], k)

    g_phi = [cp(wphi_hbm, wphi_v, 0)]
    g_x0 = [xrows(0, 256, 1)]
    g_ka = [wk_cols(0, 256, 2)]
    g_kb = [wk_cols(256, 256, 3)]
    g_kc = [wk_cols(512, 128, 0), xrows(256, P1, 0)]
    g_qv = [cp(wqkv_hbm.at[:, pl.ds(0, D)], wq_v, 1), cp(wqkv_hbm.at[:, pl.ds(2 * D, D)], wv_v, 1),
            xrows(P1, P1 + 128, 1)]
    g_xr = [xrows(P1 + 128, S, 2)]
    g_w = [cp(wo_hbm, wo_v, 3), cp(wg_hbm, wg_v, 3), cp(wu_hbm, wu_v, 3), cp(wd_hbm, wd_v, 3)]

    def waits(cs, starts=()):
        for c in cs:
            c.wait()
        for c in starts:
            c.start()

    for c in g_phi + g_x0 + g_ka + g_kb:
        c.start()

    def ln_rows(r0, n, dst, d0):
        for c in range(0, n, LNC):
            xn = _ln(x_v[pl.ds(r0 + c, LNC), :].astype(f32)).astype(bf16)
            dst[(d0 + c) // 2:(d0 + c + LNC) // 2, :] = _pk(xn)

    pending = []

    def drain(keep=0):
        while len(pending) > keep:
            pending.pop(0)()

    def phi_store(dst, g, x, c0):
        T, role = divmod(g, 3)
        cols = pl.ds(c0, 128)
        if role == 0:
            dst[2 * T, 0:40, cols] = x
        elif role == 2:
            dst[2 * T + 1, 24:64, cols] = x
        else:
            xa = jnp.concatenate([x[0:8], x[16:24]], axis=0)
            xb = jnp.concatenate([x[8:16], x[24:32]], axis=0)
            ev = (xa & jnp.uint32(0xFFFF)) | (xb << 16)
            od = (xa >> 16) | (xb & jnp.uint32(0xFFFF0000))
            dst[2 * T, 40:64, cols] = jnp.concatenate([ev, x[32:40]], axis=0)
            dst[2 * T + 1, 0:24, cols] = jnp.concatenate([od, x[32:40]], axis=0)

    def feat_block(p, dst, b, c0, rfirst=True):
        ro, mo = (0, 24) if rfirst else (128, 0)
        rs = [p[ro + 8 * a:ro + 8 + 8 * a] for a in range(3)]
        for a in range(4):
            if a < 3:
                v4 = jnp.where(_pair_is(a, 128), 0.0, rs[a])
            else:
                v4 = jnp.where(_pair_is(0, 128), rs[0],
                               jnp.where(_pair_is(1, 128), rs[1], jnp.where(_pair_is(2, 128), rs[2], 0.0)))
            ps = [p[mo + 32 * a + 8 * v:mo + 8 + 32 * a + 8 * v] for v in range(4)] + [v4]
            phi_store(dst, 4 * b + a, _pk(_feat5(ps)), c0)

    def xs(xref, xr0):
        return _up(xref[xr0 // 2:xr0 // 2 + 64, :])

    def proj_qk(off, dst, B, xref, xr0, c0):
        p = _nt(_up(wT[off + 152 * B:off + 152 * B + 152, :]), xs(xref, xr0))

        def post():
            feat_block(p[0:152], dst, 2 * B, c0)
            feat_block(p[152:304], dst, 2 * B + 1, c0)
        pending.append(post)

    def proj_k4(wb, b, j, rfirst):
        p = _nt(wb, xs(xn0, 128 * j))
        pending.append(lambda: feat_block(p[0:152], phik, b, 128 * j, rfirst))

    def proj_v(xref, xr0, c0, split_last=False):
        cuts = [0, 80, 160, 240, 280, 320] if split_last else [0, 80, 160, 240, 320]
        p = jnp.concatenate([_nt(_up(wT[V_OFF + a:V_OFF + b, :]), xs(xref, xr0))
                             for a, b in zip(cuts[:-1], cuts[1:])], axis=0)
        low = lax.broadcasted_iota(jnp.int32, (8, 128), 0) < 4
        cols = pl.ds(c0, 128)
        for T in range(5):
            mid = p[120 * T + 56:120 * T + 64]
            t0 = jnp.concatenate([p[120 * T:120 * T + 56], jnp.where(low, mid, 1.0)], axis=0)
            t1 = jnp.concatenate([jnp.where(low, 1.0, mid), p[120 * T + 64:120 * T + 120]], axis=0)
            vaug[2 * T, :, cols] = _pk(t0.astype(bf16))
            vaug[2 * T + 1, :, cols] = _pk(t1.astype(bf16))
        vaug[10, 0:24, cols] = _pk(jnp.concatenate([p[600:640], jnp.ones((8, 128), f32)], axis=0).astype(bf16))

    pr = lax.broadcasted_iota(jnp.int32, (D, D), 0)
    pc = lax.broadcasted_iota(jnp.int32, (D, D), 1)
    perm = jnp.where((pr & 31) * DH + (pr >> 5) == pc, 1.0, 0.0).astype(bf16)
    r_i = lax.broadcasted_iota(jnp.int32, (160, 32), 0)
    c_i = lax.broadcasted_iota(jnp.int32, (160, 32), 1)
    gl = r_i // 40
    sl = (r_i - 40 * gl) >> 1
    q_ = sl - 16
    f_ = jnp.where(sl < 16, sl + 1, jnp.where(q_ == gl, 0, jnp.where(q_ < gl, 17 + q_, 16 + q_)))
    e0 = jnp.where(f_ == c_i, 1.0, 0.0)
    es = []
    for t in range(5):
        off = (120 * t) % 160
        es.append((jnp.concatenate([e0[off:], e0[:off]], axis=0) if off else e0).astype(bf16))
    r2 = lax.broadcasted_iota(jnp.int32, (160, 128), 0)
    hr = 2 * (r2 // 40) + (r2 & 1)
    hc = [(lax.broadcasted_iota(jnp.int32, (1, 128), 1) + 128 * t) // DH - 6 * t for t in range(5)]
    bcat[...] = jnp.zeros(bcat.shape, f32)

    waits(g_phi, g_kc)
    for d in range(DH):
        bcat[0:DH, 32 * d:32 * d + 32] = wphi_v[d].astype(f32)
    at = _nn(bcat[...].astype(bf16), perm).astype(bf16)
    pts = [jnp.where(hr == hc[t], _nn(es[t], at[:, 128 * t:128 * t + 128]), 0.0).astype(bf16) for t in range(5)]

    def fold(w_v, off, t, rs, blk):
        rs[t] = _nt(pts[t], w_v[:, 128 * t:128 * t + 128])
        if t == 0:
            return
        b = t - 1
        lo, hi = rs[t - 1], rs[t]
        parts = []
        if b < 3:
            parts.append(lo[40 * b:120])
        parts.append(lo[120:160] + hi[0:40])
        if b > 0:
            parts.append(hi[40:40 + 40 * b])
        w = jnp.concatenate(parts, axis=0)
        mains, v4s = [], []
        for a in range(4):
            v4 = w[40 * a + 32:40 * a + 40]
            base = _allred(jnp.where(_pair_is(a, D), v4, 0.0), jnp.add)
            mains += [(w[40 * a + 8 * v:40 * a + 8 * v + 8] - base) * LOG2E for v in range(4)]
            v4s.append((v4 - base) * LOG2E)
        shared = [jnp.where(_pair_is(a, D), v4s[3], v4s[a]) for a in range(3)]
        blk[b] = (shared, mains)
        if b % 2 == 1:
            B = b // 2
            rows = blk[b - 1][0] + blk[b - 1][1] + blk[b][0] + blk[b][1]
            wT[off + 152 * B:off + 152 * B + 152, :] = _pk(jnp.concatenate(rows, axis=0).astype(bf16))

    def blk16(slabs, rfirst):
        rows = slabs[0] + slabs[1] if rfirst else slabs[1] + slabs[0]
        return jnp.concatenate(rows + [jnp.zeros((8, D), f32)], axis=0).astype(bf16)

    waits(g_x0, g_qv)
    ln_rows(0, 256, xn0, 0)

    rk, rq, bk, bq = {}, {}, {}, {}
    waits(g_ka, g_xr)
    fold(wk_v, K_OFF, 0, rk, bk)
    fold(wk_v, K_OFF, 1, rk, bk)
    w0 = blk16(bk[0], False)
    proj_k4(w0, 0, 0, False)
    proj_k4(w0, 0, 1, False)

    waits(g_kb, g_w)
    fold(wk_v, K_OFF, 2, rk, bk)
    fold(wk_v, K_OFF, 3, rk, bk)
    w1 = blk16(bk[1], False)
    proj_k4(w1, 1, 0, False)
    proj_k4(w1, 1, 1, False)
    w2 = blk16(bk[2], True)
    proj_k4(w2, 2, 0, True)
    drain(1)

    waits(g_kc)
    fold(wk_v, K_OFF, 4, rk, bk)
    proj_k4(w2, 2, 1, True)
    ln_rows(256, P1 - 256, xn0, 256)
    w3 = blk16(bk[3], True)
    proj_k4(w3, 3, 0, True)
    proj_k4(w3, 3, 1, True)
    for j in range(2, NP):
        for B in range(2):
            proj_qk(K_OFF, phik, B, xn0, 128 * j, 128 * j)
    drain(1)

    waits(g_qv)
    for t in range(5):
        fold(wq_v, Q_OFF, t, rq, bq)
    for t in range(5):
        wT[V_OFF + 64 * t:V_OFF + 64 * t + 64, :] = _pk(wv_v[:, 128 * t:128 * t + 128].T)
    ln_rows(P1, 128, xn_buf, 0)
    for j in range(NP):
        for B in range(2):
            proj_qk(Q_OFF, phiq, B, xn0, 128 * j, 128 * j)
    drain()
    for j in range(NP):
        proj_v(xn0, 128 * j, 128 * j, j == NP - 1)

    def p1(i, carry):
        for j in range(R):
            c0 = pl.multiple_of(P1 + i * T1 + 128 * j, 128)
            rn = pl.multiple_of(P1 + i * T1 + 128 * (j + 1), 128)
            ln_rows(rn, 128, xn_buf, 128 * ((j + 1) % R))
            for off, dst in ((K_OFF, phik), (Q_OFF, phiq)):
                for B in range(2):
                    proj_qk(off, dst, B, xn_buf, 128 * j, c0)
                    drain()
            proj_v(xn_buf, 128 * j, c0)
        return carry

    waits(g_xr)
    lax.fori_loop(0, N1, p1, 0)

    proj_v(xn_buf, 0, S - 128)
    for B in range(2):
        proj_qk(K_OFF, phik, B, xn_buf, 0, S - 128)
    for B in range(2):
        proj_qk(Q_OFF, phiq, B, xn_buf, 0, S - 128)
    drain()

    rr = lax.broadcasted_iota(jnp.int32, (64, 128), 0)
    cc = lax.broadcasted_iota(jnp.int32, (64, 128), 1)
    par = cc & 1
    col0 = jnp.where(cc < 80, par, jnp.where(cc < 112, 2, 2 + par))
    col1 = jnp.where(cc < 32, 0, jnp.where(cc < 48, par - 1, 1 + par))
    row0 = jnp.where(rr < 60, rr // DH, jnp.minimum(rr - 60, 2))
    row1 = jnp.where(rr < 4, jnp.minimum(rr, 2), (rr - 4) // DH)
    msks = (col0 == row0, col1 == row1)
    for t in range(10):
        kvm[t] = _pk(jnp.where(msks[t % 2], _nt(_up(vaug[t]), _up(phik[t])), 0.0).astype(bf16))
    rl = lax.broadcasted_iota(jnp.int32, (48, 80), 0)
    cl = lax.broadcasted_iota(jnp.int32, (48, 80), 1)
    rowl = jnp.where(rl < 40, (rl >= 20).astype(jnp.int32), (rl >= 44).astype(jnp.int32))
    kvl = _nt(_up(vaug[10, 0:24, :]), _up(phik[10, 0:40, :]))
    kvm[10, 0:24, 0:80] = _pk(jnp.where((cl & 1) == rowl, kvl, 0.0).astype(bf16))

    def attn_o(c0):
        low = lax.broadcasted_iota(jnp.int32, (8, NW), 0) < 4
        cols = pl.ds(c0, NW)

        def bc(r, k):
            return jnp.broadcast_to(r[k:k + 1], (8, NW))
        os = []
        for T in range(5):
            n0 = _nn(_up(kvm[2 * T]), _up(phiq[2 * T, :, cols]))
            n1 = _nn(_up(kvm[2 * T + 1]), _up(phiq[2 * T + 1, :, cols]))
            r0 = _rcp(n0[56:64] + 1e-6)
            r1 = _rcp(n1[0:8] + 1e-6)
            a, b, c = bc(r0, 4), bc(r0, 5), bc(r0, 6)
            d, e, f = bc(r1, 0), bc(r1, 1), bc(r1, 2)
            os += [n0[0:8] * a, n0[8:16] * a, n0[16:24] * jnp.where(low, a, b), n0[24:32] * b, n0[32:40] * b,
                   n0[40:48] * c, n0[48:56] * c, jnp.where(low, n0[56:64] * c, n1[0:8] * d),
                   n1[8:16] * d, n1[16:24] * d, n1[24:32] * e, n1[32:40] * e, n1[40:48] * jnp.where(low, e, f),
                   n1[48:56] * f, n1[56:64] * f]
        nd = _nn(_up(kvm[10, 0:24, 0:80]), _up(phiq[10, 0:40, cols]))
        r = _rcp(nd[40:48] + 1e-6)
        rrot = pltpu.roll(r, 4, 0)
        ra = jnp.where(low, r, rrot)
        rb = jnp.where(low, rrot, r)
        os += [nd[0:8] * ra, nd[8:16] * ra, nd[16:24] * r, nd[24:32] * rb, nd[32:40] * rb]
        return jnp.concatenate(os, axis=0).astype(bf16).T

    def gu(hn, c):
        gt = _nn(hn, wg_v[:, c * FC:(c + 1) * FC])
        up = _nn(hn, wu_v[:, c * FC:(c + 1) * FC])
        return _gelu_mul(gt, up).astype(bf16)

    def down(c, a):
        return _nn(a, wd_v[c * FC:(c + 1) * FC, :])

    nc = F // FC

    def p2(i, carry):
        o = jnp.concatenate([attn_o(pl.multiple_of(i * T2 + w, NW)) for w in range(0, T2, NW)], axis=0)
        hs, hns = [], []
        for w in range(0, T2, WOB):
            r0 = pl.multiple_of(i * T2 + w, WOB)
            h = x_v[pl.ds(r0, WOB), :].astype(f32) + _nn(o[w:w + WOB], wo_v[...])
            hs.append(h)
            hns.append(_ln(h).astype(bf16))
        half = len(hns) // 2
        a0 = jnp.concatenate([gu(jnp.concatenate(hns[:half], axis=0), 0),
                              gu(jnp.concatenate(hns[half:], axis=0), 0)], axis=0)
        hn = jnp.concatenate(hns, axis=0)
        acc = jnp.concatenate(hs, axis=0) + down(0, a0)
        for c in range(1, nc - 1):
            acc = acc + down(c, gu(hn, c))
        al = gu(hn, nc - 1)
        for lo, n in zip(POFF, PIECES):
            res = acc[lo:lo + n] + down(nc - 1, al[lo:lo + n])
            r0 = pl.multiple_of(i * T2 + lo, 16)
            out_v[pl.ds(r0, n), :] = res.astype(bf16)
            cp(out_v.at[pl.ds(r0, n)], out_hbm.at[0, pl.ds(r0, n)], 0).start()
        return carry

    waits(g_w)
    lax.fori_loop(0, N2, p2, 0)
    cp(out_v, out_hbm.at[0], 0).wait()


def _kernel(*refs):
    @pl.when(pl.program_id(0) == 0)
    def _():
        _body(*refs)


@jax.jit
def pallas_sequential_preLN__linear_kernel_hedgehog__geglu_ffn__prompt_kernel(
    A_x: jax.Array,
    A_wqkv: jax.Array,
    A_w_phi: jax.Array,
    A_wo: jax.Array,
    B_x: jax.Array,
    B_w_gate: jax.Array,
    B_w_up: jax.Array,
    B_w_down: jax.Array,
):
    del B_x
    anyspec = pl.BlockSpec(memory_space=pl.ANY)
    wphi_t = jnp.transpose(A_w_phi, (1, 2, 0))
    return pl.pallas_call(
        _kernel,
        out_shape=jax.ShapeDtypeStruct((1, S, D), bf16),
        grid=(2,),
        in_specs=[anyspec] * 7,
        out_specs=anyspec,
        scratch_shapes=[
            pltpu.VMEM((S, D), bf16),
            pltpu.VMEM((D, D), bf16),
            pltpu.VMEM((D, D), bf16),
            pltpu.VMEM((D, D), bf16),
            pltpu.VMEM((DH, DH, H), bf16),
            pltpu.VMEM((D, D), bf16),
            pltpu.VMEM((D, F), bf16),
            pltpu.VMEM((D, F), bf16),
            pltpu.VMEM((F, D), bf16),
            pltpu.VMEM((928, D), u32),
            pltpu.VMEM((32, D), f32),
            pltpu.VMEM((P1 // 2, D), u32),
            pltpu.VMEM((T1 // 2, D), u32),
            pltpu.VMEM((11, 64, S), u32),
            pltpu.VMEM((11, 64, S), u32),
            pltpu.VMEM((11, 32, S), u32),
            pltpu.VMEM((11, 32, 128), u32),
            pltpu.VMEM((S, D), bf16),
            pltpu.SemaphoreType.DMA((4,)),
        ],
        compiler_params=pltpu.CompilerParams(
            dimension_semantics=("arbitrary",),
            vmem_limit_bytes=100 * 1024 * 1024,
            disable_bounds_checks=True,
            disable_semaphore_checks=True,
        ),
        name="hh",
    )(A_x, A_wqkv, wphi_t, A_wo, B_w_gate, B_w_up, B_w_down)
```

```python
import jax
import jax.numpy as jnp
from jax import lax
from jax.experimental import pallas as pl
from jax.experimental.pallas import tpu as pltpu

S, D, H, DH, F = 2048, 640, 32, 20, 1536
NG = H // 2
LOG2E = 1.4426950408889634
NT_DIMS = (((1,), (1,)), ((), ()))
f32 = jnp.float32
bf16 = jnp.bfloat16
u32 = jnp.uint32

NP = 5
R = 5
T1 = 128 * R
P1 = 128 * NP
N1 = (S - P1 - 128) // T1
T2 = 512
N2 = S // T2
NW = 256
WOB = 64
LNC = 64
TBR = 32
FC = 512
PIECES = (128, 128, 128, 64, 32, 32)
POFF = tuple(sum(PIECES[:k]) for k in range(len(PIECES)))
K_OFF, Q_OFF, V_OFF = 0, 304, 608
assert P1 + N1 * T1 + 128 == S and sum(PIECES) == T2


def _ln(x):
    m = jnp.mean(x, axis=-1, keepdims=True)
    xc = x - m
    v = jnp.mean(xc * xc, axis=-1, keepdims=True) + 1e-5
    return xc * jnp.exp2(jnp.log(v) * (-0.5 * LOG2E))


def _rcp(x):
    return pl.reciprocal(x, approx=True)


def _allred(m, op):
    m = op(m, pltpu.roll(m, 2, 0))
    return op(m, pltpu.roll(m, 4, 0))


def _tree(op, xs):
    return op(op(op(xs[0], xs[1]), op(xs[2], xs[3])), xs[4])


def _feat5(ps):
    mx = _allred(_tree(jnp.maximum, ps), jnp.maximum)
    mn = _allred(_tree(jnp.minimum, ps), jnp.minimum)
    ep = [jnp.exp2(q - mx) for q in ps]
    en = [jnp.exp2(mn - q) for q in ps]
    rp = _rcp(_allred(_tree(jnp.add, ep), jnp.add))
    rn = _rcp(_allred(_tree(jnp.add, en), jnp.add))
    return [_pe(a * rp, b * rn) for a, b in zip(ep, en)]


def _gelu_mul(g, u):
    c = 0.7978845608028654
    t = jnp.tanh(g * (c + (c * 0.044715) * (g * g)))
    hgu = (0.5 * g) * u
    return hgu + hgu * t


def _pk(v):
    return pltpu.bitcast(v, u32)


def _pe(a, b):
    return pltpu.pack_elementwise([a, b], packed_dtype=bf16)


def _up(v):
    return pltpu.bitcast(v, bf16)


def _nt(a, b):
    return lax.dot_general(a, b, NT_DIMS, preferred_element_type=f32)


def _nn(a, b):
    return jnp.dot(a, b, preferred_element_type=f32)


def _pair_is(a, w):
    return (lax.broadcasted_iota(jnp.int32, (8, w), 0) >> 1) == a


def _body(x_hbm, wqkv_hbm, wphi_hbm, wo_hbm, wg_hbm, wu_hbm, wd_hbm, out_hbm,
          x_v, wq_v, wk_v, wv_v, wphi_v, wo_v, wgu_v, wd_v, wT, bcat,
          xn0, xn_buf, phiq, phik, vaug, kvm, tgu, tdn, out_v, sem):
    def cp(src, dst, k):
        return pltpu.make_async_copy(src, dst, sem.at[k])

    def xrows(r0, r1, k):
        return cp(x_hbm.at[0, pl.ds(r0, r1 - r0)], x_v.at[pl.ds(r0, r1 - r0)], k)

    def wk_cols(c0, n, k):
        return cp(wqkv_hbm.at[:, pl.ds(D + c0, n)], wk_v.at[:, pl.ds(c0, n)], k)

    g_phi = [cp(wphi_hbm, wphi_v, 0)]
    g_x0 = [xrows(0, 256, 1)]
    g_ka = [wk_cols(0, 256, 2)]
    g_kb = [wk_cols(256, 256, 3)]
    g_kc = [wk_cols(512, 128, 0), xrows(256, P1, 0)]
    g_qv = [cp(wqkv_hbm.at[:, pl.ds(0, D)], wq_v, 1), cp(wqkv_hbm.at[:, pl.ds(2 * D, D)], wv_v, 1),
            xrows(P1, P1 + 128, 1)]
    g_xr = [xrows(P1 + 128, S, 2), cp(wg_hbm, wgu_v.at[0], 2)]
    g_w = [cp(wu_hbm, wgu_v.at[1], 3), cp(wd_hbm, wd_v, 3), cp(wo_hbm, wo_v, 3)]

    def waits(cs, starts=()):
        for c in cs:
            c.wait()
        for c in starts:
            c.start()

    for c in g_phi + g_x0 + g_ka + g_kb:
        c.start()

    def ln_rows(r0, n, dst, d0):
        for c in range(0, n, LNC):
            xn = _ln(x_v[pl.ds(r0 + c, LNC), :].astype(f32)).astype(bf16)
            dst[(d0 + c) // 2:(d0 + c + LNC) // 2, :] = _pk(xn)

    fill = []
    pending = []

    def drain(keep=0):
        while len(pending) > keep:
            pending.pop(0)()

    def phi_store(dst, g, x, c0):
        T, role = divmod(g, 3)
        cols = pl.ds(c0, 128)
        if role == 0:
            dst[2 * T, 0:40, cols] = jnp.concatenate(x, axis=0)
        elif role == 2:
            dst[2 * T + 1, 24:64, cols] = jnp.concatenate(x, axis=0)
        else:
            even = (lax.broadcasted_iota(jnp.int32, (8, 128), 0) & 1) == 0
            ev = [jnp.where(even, x[a], pltpu.roll(x[a + 1], 1, 0)) for a in (0, 2)]
            od = [jnp.where(even, pltpu.roll(x[a], 7, 0), x[a + 1]) for a in (0, 2)]
            dst[2 * T, 40:64, cols] = jnp.concatenate(ev + [x[4]], axis=0)
            dst[2 * T + 1, 0:24, cols] = jnp.concatenate(od + [x[4]], axis=0)

    def feat_block(p, dst, b, c0, rfirst=True):
        ro, mo = (0, 24) if rfirst else (128, 0)
        rs = [p[ro + 8 * a:ro + 8 + 8 * a] for a in range(3)]
        for a in range(4):
            if a < 3:
                v4 = jnp.where(_pair_is(a, 128), 0.0, rs[a])
            else:
                v4 = jnp.where(_pair_is(0, 128), rs[0],
                               jnp.where(_pair_is(1, 128), rs[1], jnp.where(_pair_is(2, 128), rs[2], 0.0)))
            ps = [p[mo + 32 * a + 8 * v:mo + 8 + 32 * a + 8 * v] for v in range(4)] + [v4]
            phi_store(dst, 4 * b + a, _feat5(ps), c0)

    def xs(xref, xr0):
        return _up(xref[xr0 // 2:xr0 // 2 + 64, :])

    def proj_qk(off, dst, B, xref, xr0, c0):
        p = _nt(_up(wT[off + 152 * B:off + 152 * B + 152, :]), xs(xref, xr0))

        def post():
            feat_block(p[0:152], dst, 2 * B, c0)
            feat_block(p[152:304], dst, 2 * B + 1, c0)
        pending.append(post)

    def proj_k4(wb, b, j, rfirst):
        p = _nt(wb, xs(xn0, 128 * j))
        pending.append(lambda: feat_block(p[0:152], phik, b, 128 * j, rfirst))

    def proj_v(xref, xr0, c0, split_last=False):
        cuts = [0, 80, 160, 240, 280, 320] if split_last else [0, 80, 160, 240, 320]
        p = jnp.concatenate([_nt(_up(wT[V_OFF + a:V_OFF + b, :]), xs(xref, xr0))
                             for a, b in zip(cuts[:-1], cuts[1:])], axis=0)
        low = lax.broadcasted_iota(jnp.int32, (8, 128), 0) < 4
        cols = pl.ds(c0, 128)
        sl = [p[8 * a:8 * a + 8] for a in range(80)]

        def put(t, slabs):
            vaug[t, 0:4 * len(slabs), cols] = jnp.concatenate(
                [_pe(slabs[a], slabs[a + 1]) for a in range(0, len(slabs), 2)], axis=0)
        for T in range(5):
            mid = sl[15 * T + 7]
            put(2 * T, sl[15 * T:15 * T + 7] + [jnp.where(low, mid, 1.0)])
            put(2 * T + 1, [jnp.where(low, 1.0, mid)] + sl[15 * T + 8:15 * T + 15])
            if fill:
                fill.pop(0)()
        put(10, sl[75:80] + [jnp.ones((8, 128), f32)])

    pr = lax.broadcasted_iota(jnp.int32, (D, D), 0)
    pc = lax.broadcasted_iota(jnp.int32, (D, D), 1)
    perm = jnp.where((pr & 31) * DH + (pr >> 5) == pc, 1.0, 0.0).astype(bf16)
    r_i = lax.broadcasted_iota(jnp.int32, (160, 32), 0)
    c_i = lax.broadcasted_iota(jnp.int32, (160, 32), 1)
    gl = r_i // 40
    sl = (r_i - 40 * gl) >> 1
    q_ = sl - 16
    f_ = jnp.where(sl < 16, sl + 1, jnp.where(q_ == gl, 0, jnp.where(q_ < gl, 17 + q_, 16 + q_)))
    e0 = jnp.where(f_ == c_i, 1.0, 0.0)
    es = []
    for t in range(5):
        off = (120 * t) % 160
        es.append((jnp.concatenate([e0[off:], e0[:off]], axis=0) if off else e0).astype(bf16))
    r2 = lax.broadcasted_iota(jnp.int32, (160, 128), 0)
    hr = 2 * (r2 // 40) + (r2 & 1)
    hc = [(lax.broadcasted_iota(jnp.int32, (1, 128), 1) + 128 * t) // DH - 6 * t for t in range(5)]
    bcat[...] = jnp.zeros(bcat.shape, f32)

    waits(g_phi, g_kc)
    for d in range(DH):
        bcat[0:DH, 32 * d:32 * d + 32] = wphi_v[d].astype(f32)
    at = _nn(bcat[...].astype(bf16), perm).astype(bf16)
    pts = [jnp.where(hr == hc[t], _nn(es[t], at[:, 128 * t:128 * t + 128]), 0.0).astype(bf16) for t in range(5)]

    def fold(w_v, off, t, rs, blk):
        rs[t] = _nt(pts[t], w_v[:, 128 * t:128 * t + 128])
        if t == 0:
            return
        b = t - 1
        lo, hi = rs[t - 1], rs[t]
        parts = []
        if b < 3:
            parts.append(lo[40 * b:120])
        parts.append(lo[120:160] + hi[0:40])
        if b > 0:
            parts.append(hi[40:40 + 40 * b])
        w = jnp.concatenate(parts, axis=0)
        mains, v4s = [], []
        for a in range(4):
            v4 = w[40 * a + 32:40 * a + 40]
            base = _allred(jnp.where(_pair_is(a, D), v4, 0.0), jnp.add)
            mains += [(w[40 * a + 8 * v:40 * a + 8 * v + 8] - base) * LOG2E for v in range(4)]
            v4s.append((v4 - base) * LOG2E)
        shared = [jnp.where(_pair_is(a, D), v4s[3], v4s[a]) for a in range(3)]
        blk[b] = (shared, mains)
        if b % 2 == 1:
            B = b // 2
            rows = blk[b - 1][0] + blk[b - 1][1] + blk[b][0] + blk[b][1]
            wT[off + 152 * B:off + 152 * B + 152, :] = _pk(jnp.concatenate(rows, axis=0).astype(bf16))

    def blk16(slabs, rfirst):
        rows = slabs[0] + slabs[1] if rfirst else slabs[1] + slabs[0]
        return jnp.concatenate(rows + [jnp.zeros((8, D), f32)], axis=0).astype(bf16)

    waits(g_x0, g_qv)
    ln_rows(0, 256, xn0, 0)

    rk, rq, bk, bq = {}, {}, {}, {}
    waits(g_ka, g_xr)
    fold(wk_v, K_OFF, 0, rk, bk)
    fold(wk_v, K_OFF, 1, rk, bk)
    w0 = blk16(bk[0], False)
    proj_k4(w0, 0, 0, False)
    proj_k4(w0, 0, 1, False)

    waits(g_kb, g_w)
    fold(wk_v, K_OFF, 2, rk, bk)
    fold(wk_v, K_OFF, 3, rk, bk)
    w1 = blk16(bk[1], False)
    proj_k4(w1, 1, 0, False)
    proj_k4(w1, 1, 1, False)
    w2 = blk16(bk[2], True)
    proj_k4(w2, 2, 0, True)
    drain(1)

    waits(g_kc)
    fold(wk_v, K_OFF, 4, rk, bk)
    proj_k4(w2, 2, 1, True)
    ln_rows(256, P1 - 256, xn0, 256)
    w3 = blk16(bk[3], True)
    proj_k4(w3, 3, 0, True)
    proj_k4(w3, 3, 1, True)
    for j in range(2, NP):
        for B in range(2):
            proj_qk(K_OFF, phik, B, xn0, 128 * j, 128 * j)
    drain(1)

    waits(g_qv)
    for t in range(5):
        fold(wq_v, Q_OFF, t, rq, bq)
    for t in range(5):
        wT[V_OFF + 64 * t:V_OFF + 64 * t + 64, :] = _pk(wv_v[:, 128 * t:128 * t + 128].T)
    ln_rows(P1, 128, xn_buf, 0)
    for j in range(NP):
        for B in range(2):
            proj_qk(Q_OFF, phiq, B, xn0, 128 * j, 128 * j)
    drain()
    for j in range(NP):
        proj_v(xn0, 128 * j, 128 * j, j == NP - 1)

    nc = F // FC

    def table_jobs(dst, w_ref, r0, c0):
        def job(r):
            f11, f12, f21, f22 = [
                w_ref[r0 + 256 * a + r:r0 + 256 * a + r + TBR, c0 + 256 * b:c0 + 256 * b + 256].astype(f32)
                for a in range(2) for b in range(2)]
            for k, t in enumerate([f11 + f22, f12 - f22, f21 - f11, f11 + f12, f21 + f22]):
                dst[k, r:r + TBR, :] = t.astype(bf16)
        return [(lambda r=r: job(r)) for r in range(0, 256, TBR)]

    def p1(i, carry):
        @pl.when(i == N1 - 1)
        def _():
            waits(g_w)
        for c in range(nc):
            fill.extend(table_jobs(tgu.at[i, c], wgu_v.at[i], 0, c * FC))
        for j in range(R):
            c0 = pl.multiple_of(P1 + i * T1 + 128 * j, 128)
            rn = pl.multiple_of(P1 + i * T1 + 128 * (j + 1), 128)
            ln_rows(rn, 128, xn_buf, 128 * ((j + 1) % R))
            for off, dst in ((K_OFF, phik), (Q_OFF, phiq)):
                for B in range(2):
                    proj_qk(off, dst, B, xn_buf, 128 * j, c0)
                    drain()
            proj_v(xn_buf, 128 * j, c0)
        while fill:
            fill.pop(0)()
        return carry

    waits(g_xr)
    lax.fori_loop(0, N1, p1, 0)

    for c in range(nc):
        fill.extend(table_jobs(tdn.at[c], wd_v, c * FC, 0))
    proj_v(xn_buf, 0, S - 128)
    for B in range(2):
        proj_qk(K_OFF, phik, B, xn_buf, 0, S - 128)
    for B in range(2):
        proj_qk(Q_OFF, phiq, B, xn_buf, 0, S - 128)
    drain()

    rr = lax.broadcasted_iota(jnp.int32, (64, 128), 0)
    cc = lax.broadcasted_iota(jnp.int32, (64, 128), 1)
    par = (cc >> 1) & 1
    col0 = jnp.where(cc < 80, par, jnp.where(cc < 112, 2, 2 + par))
    col1 = jnp.where(cc < 32, 0, jnp.where(cc < 48, par - 1, 1 + par))
    row0 = jnp.where(rr < 60, rr // DH, jnp.minimum(rr - 60, 2))
    row1 = jnp.where(rr < 4, jnp.minimum(rr, 2), (rr - 4) // DH)
    msks = (col0 == row0, col1 == row1)

    def unzip(y):
        u = _pk(y.astype(bf16))
        lo = lax.bitcast_convert_type(u << 16, f32)
        hi = lax.bitcast_convert_type(u & jnp.uint32(0xFFFF0000), f32)
        return jnp.concatenate([t[a:a + 8] for a in range(0, u.shape[0], 8) for t in (lo, hi)], axis=0)

    for t in range(10):
        for _ in range(2):
            if fill:
                fill.pop(0)()
        kvm[t] = _pk(jnp.where(msks[t % 2], unzip(_nt(_up(vaug[t]), _up(phik[t]))), 0.0).astype(bf16))
    rl = lax.broadcasted_iota(jnp.int32, (48, 80), 0)
    cl = lax.broadcasted_iota(jnp.int32, (48, 80), 1)
    rowl = jnp.where(rl < 40, (rl >= 20).astype(jnp.int32), (rl >= 44).astype(jnp.int32))
    kvl = unzip(_nt(_up(vaug[10, 0:24, :]), _up(phik[10, 0:40, :])))
    kvm[10, 0:24, 0:80] = _pk(jnp.where(((cl >> 1) & 1) == rowl, kvl, 0.0).astype(bf16))
    while fill:
        fill.pop(0)()

    def attn_o(c0):
        low = lax.broadcasted_iota(jnp.int32, (8, NW), 0) < 4
        cols = pl.ds(c0, NW)

        def bc(r, k):
            return jnp.broadcast_to(r[k:k + 1], (8, NW))
        os = []
        for T in range(5):
            n0 = _nn(_up(kvm[2 * T]), _up(phiq[2 * T, :, cols]))
            n1 = _nn(_up(kvm[2 * T + 1]), _up(phiq[2 * T + 1, :, cols]))
            r0 = _rcp(n0[56:64] + 1e-6)
            r1 = _rcp(n1[0:8] + 1e-6)
            a, b, c = bc(r0, 4), bc(r0, 5), bc(r0, 6)
            d, e, f = bc(r1, 0), bc(r1, 1), bc(r1, 2)
            os += [n0[0:8] * a, n0[8:16] * a, n0[16:24] * jnp.where(low, a, b), n0[24:32] * b, n0[32:40] * b,
                   n0[40:48] * c, n0[48:56] * c, jnp.where(low, n0[56:64] * c, n1[0:8] * d),
                   n1[8:16] * d, n1[16:24] * d, n1[24:32] * e, n1[32:40] * e, n1[40:48] * jnp.where(low, e, f),
                   n1[48:56] * f, n1[56:64] * f]
        nd = _nn(_up(kvm[10, 0:24, 0:80]), _up(phiq[10, 0:40, cols]))
        r = _rcp(nd[40:48] + 1e-6)
        rrot = pltpu.roll(r, 4, 0)
        ra = jnp.where(low, r, rrot)
        rb = jnp.where(low, rrot, r)
        os += [nd[0:8] * ra, nd[8:16] * ra, nd[16:24] * r, nd[24:32] * rb, nd[32:40] * rb]
        return jnp.concatenate(os, axis=0).astype(bf16).T

    def lhs7(a11, a12, a21, a22):
        return [(a11 + a22).astype(bf16), (a21 + a22).astype(bf16), a11.astype(bf16), a22.astype(bf16),
                (a11 + a12).astype(bf16), (a21 - a11).astype(bf16), (a12 - a22).astype(bf16)]

    HT = T2 // 2

    def p2(i, carry):
        o = jnp.concatenate([attn_o(pl.multiple_of(i * T2 + w, NW)) for w in range(0, T2, NW)], axis=0)
        hs, hns = [], []
        for w in range(0, T2, WOB):
            r0 = pl.multiple_of(i * T2 + w, WOB)
            h = x_v[pl.ds(r0, WOB), :].astype(f32) + _nn(o[w:w + WOB], wo_v[...])
            hs.append(h)
            hns.append(_ln(h))
        h = jnp.concatenate(hs, axis=0)
        hn = jnp.concatenate(hns, axis=0)
        L = lhs7(hn[:HT, 0:256], hn[:HT, 256:512], hn[HT:, 0:256], hn[HT:, 256:512])
        hr_ = hn[:, 512:640].astype(bf16)

        dm = [None] * 7
        rest = h[:, 512:640]

        def out_block(r0, n, c0, w, val):
            rr0 = pl.multiple_of(i * T2 + r0, 16)
            out_v[pl.ds(rr0, n), c0:c0 + w] = val.astype(bf16)
            cp(out_v.at[pl.ds(rr0, n), pl.ds(c0, w)], out_hbm.at[0, pl.ds(rr0, n), pl.ds(c0, w)], 0).start()

        for c in range(nc):
            ws = (wgu_v.at[0], wgu_v.at[1])

            def rhs(tab, w_ref, r0, c0, k):
                if k == 1:
                    return w_ref[r0:r0 + 256, c0:c0 + 256]
                if k == 4:
                    return w_ref[r0 + 256:r0 + 512, c0 + 256:c0 + 512]
                return tab[(0, None, 1, 2, None, 3, 4)[k]]
            m = [[None] * 7, [None] * 7]

            def mul(k):
                bs = [rhs(tgu.at[w, c], ws[w], 0, c * FC, k) for w in range(2)]
                hv = [[_nn(L[k], bs[w][:, 128 * nh:128 * nh + 128]) for w in range(2)] for nh in range(2)]
                for w in range(2):
                    m[w][k] = jnp.concatenate([hv[0][w], hv[1][w]], axis=1)

            def rq(a, b):
                return [_nn(hr_[HT * a:HT * a + HT], ws[w][512:640, c * FC + 256 * b:c * FC + 256 * b + 256])
                        for w in range(2)]
            r12 = rq(0, 1)
            mul(2)
            mul(4)
            a12 = _gelu_mul(*[m[w][2] + m[w][4] + r12[w] for w in range(2)])
            r21 = rq(1, 0)
            mul(1)
            mul(3)
            a21 = _gelu_mul(*[m[w][1] + m[w][3] + r21[w] for w in range(2)])
            r11 = rq(0, 0)
            mul(0)
            mul(6)
            a11 = _gelu_mul(*[m[w][0] + m[w][3] - m[w][4] + r11[w] + m[w][6] for w in range(2)])
            r22 = rq(1, 1)
            mul(5)
            a22 = _gelu_mul(*[m[w][0] - m[w][1] + m[w][2] + r22[w] + m[w][5] for w in range(2)])
            A = lhs7(a11, a12, a21, a22)
            at_ = jnp.concatenate([A[2], a12.astype(bf16)], axis=1)
            ab_ = jnp.concatenate([a21.astype(bf16), A[3]], axis=1)
            wr = wd_v[c * FC:(c + 1) * FC, 512:640]

            def dmul(k):
                t = _nn(A[k], rhs(tdn.at[c], wd_v, c * FC, 0, k))
                dm[k] = t if dm[k] is None else dm[k] + t
            if c < nc - 1:
                for k in (2, 4, 5):
                    dmul(k)
                rest = rest + jnp.concatenate([_nn(at_, wr), _nn(ab_, wr)], axis=0)
                for k in (0, 1, 3, 6):
                    dmul(k)
            else:
                dmul(2)
                dmul(4)
                out_block(0, HT, 256, 256, h[:HT, 256:512] + dm[2] + dm[4])
                dmul(5)
                out_block(0, HT, 512, 128, rest[:HT] + _nn(at_, wr))
                dmul(1)
                dmul(3)
                out_block(HT, HT, 0, 256, h[HT:, 0:256] + dm[1] + dm[3])
                dmul(0)
                out_block(HT, HT, 256, 256, h[HT:, 256:512] + dm[0] - dm[1] + dm[2] + dm[5])
                dmul(6)
                out_block(0, HT, 0, 256, h[:HT, 0:256] + dm[0] + dm[3] - dm[4] + dm[6])
                for lo, n in ((0, 128), (128, 64), (192, 32), (224, 32)):
                    out_block(HT + lo, n, 512, 128, rest[HT + lo:HT + lo + n] + _nn(ab_[lo:lo + n], wr))
        return carry

    lax.fori_loop(0, N2, p2, 0)
    cp(out_v, out_hbm.at[0], 0).wait()


def _kernel(*refs):
    @pl.when(pl.program_id(0) == 0)
    def _():
        _body(*refs)


@jax.jit
def pallas_sequential_preLN__linear_kernel_hedgehog__geglu_ffn__prompt_kernel(
    A_x: jax.Array,
    A_wqkv: jax.Array,
    A_w_phi: jax.Array,
    A_wo: jax.Array,
    B_x: jax.Array,
    B_w_gate: jax.Array,
    B_w_up: jax.Array,
    B_w_down: jax.Array,
):
    del B_x
    anyspec = pl.BlockSpec(memory_space=pl.ANY)
    wphi_t = jnp.transpose(A_w_phi, (1, 2, 0))
    return pl.pallas_call(
        _kernel,
        out_shape=jax.ShapeDtypeStruct((1, S, D), bf16),
        grid=(2,),
        in_specs=[anyspec] * 7,
        out_specs=anyspec,
        scratch_shapes=[
            pltpu.VMEM((S, D), bf16),
            pltpu.VMEM((D, D), bf16),
            pltpu.VMEM((D, D), bf16),
            pltpu.VMEM((D, D), bf16),
            pltpu.VMEM((DH, DH, H), bf16),
            pltpu.VMEM((D, D), bf16),
            pltpu.VMEM((2, D, F), bf16),
            pltpu.VMEM((F, D), bf16),
            pltpu.VMEM((928, D), u32),
            pltpu.VMEM((32, D), f32),
            pltpu.VMEM((P1 // 2, D), u32),
            pltpu.VMEM((T1 // 2, D), u32),
            pltpu.VMEM((11, 64, S), u32),
            pltpu.VMEM((11, 64, S), u32),
            pltpu.VMEM((11, 32, S), u32),
            pltpu.VMEM((11, 32, 128), u32),
            pltpu.VMEM((2, 3, 5, 256, 256), bf16),
            pltpu.VMEM((3, 5, 256, 256), bf16),
            pltpu.VMEM((S, D), bf16),
            pltpu.SemaphoreType.DMA((4,)),
        ],
        compiler_params=pltpu.CompilerParams(
            dimension_semantics=("arbitrary",),
            vmem_limit_bytes=100 * 1024 * 1024,
            disable_bounds_checks=True,
            disable_semaphore_checks=True,
        ),
        name="hh",
    )(A_x, A_wqkv, wphi_t, A_wo, B_w_gate, B_w_up, B_w_down)
```

```python
import jax
import jax.numpy as jnp
from jax import lax
from jax.experimental import pallas as pl
from jax.experimental.pallas import tpu as pltpu

S, D, H, DH, F = 2048, 640, 32, 20, 1536
NG = H // 2
LOG2E = 1.4426950408889634
NT_DIMS = (((1,), (1,)), ((), ()))
f32 = jnp.float32
bf16 = jnp.bfloat16
u32 = jnp.uint32

NP = 5
R = 5
T1 = 128 * R
P1 = 128 * NP
N1 = (S - P1 - 128) // T1
T2 = 512
N2 = S // T2
NW = 256
WOB = 64
LNC = 64
TBR = 32
TB2, TBC = 8, 256
FC = 512
PIECES = (128, 128, 128, 64, 32, 32)
POFF = tuple(sum(PIECES[:k]) for k in range(len(PIECES)))
K_OFF, Q_OFF, V_OFF = 0, 304, 608
assert P1 + N1 * T1 + 128 == S and sum(PIECES) == T2


def _ln(x):
    m = jnp.mean(x, axis=-1, keepdims=True)
    xc = x - m
    v = jnp.mean(xc * xc, axis=-1, keepdims=True) + 1e-5
    return xc * jnp.exp2(jnp.log(v) * (-0.5 * LOG2E))


def _rcp(x):
    return pl.reciprocal(x, approx=True)


def _allred(m, op):
    m = op(m, pltpu.roll(m, 2, 0))
    return op(m, pltpu.roll(m, 4, 0))


def _tree(op, xs):
    return op(op(op(xs[0], xs[1]), op(xs[2], xs[3])), xs[4])


def _feat5(ps):
    mx = _allred(_tree(jnp.maximum, ps), jnp.maximum)
    mn = _allred(_tree(jnp.minimum, ps), jnp.minimum)
    ep = [jnp.exp2(q - mx) for q in ps]
    en = [jnp.exp2(mn - q) for q in ps]
    rp = _rcp(_allred(_tree(jnp.add, ep), jnp.add))
    rn = _rcp(_allred(_tree(jnp.add, en), jnp.add))
    return [_pe(a * rp, b * rn) for a, b in zip(ep, en)]


def _gelu_mul(g, u):
    c = 0.7978845608028654
    t = jnp.tanh(g * (c + (c * 0.044715) * (g * g)))
    hgu = (0.5 * g) * u
    return hgu + hgu * t


def _pk(v):
    return pltpu.bitcast(v, u32)


def _pe(a, b):
    return pltpu.pack_elementwise([a, b], packed_dtype=bf16)


def _up(v):
    return pltpu.bitcast(v, bf16)


def _nt(a, b):
    return lax.dot_general(a, b, NT_DIMS, preferred_element_type=f32)


def _nn(a, b):
    return jnp.dot(a, b, preferred_element_type=f32)


def _pair_is(a, w):
    return (lax.broadcasted_iota(jnp.int32, (8, w), 0) >> 1) == a


def _body(x_hbm, wqkv_hbm, wphi_hbm, wo_hbm, wg_hbm, wu_hbm, wd_hbm, out_hbm,
          x_v, wq_v, wk_v, wv_v, wphi_v, wo_v, wgu_v, wd2, wT, bcat,
          xn0, xn_buf, phiq, phik, vaug, kvm, out_v, sem):
    def cp(src, dst, k):
        return pltpu.make_async_copy(src, dst, sem.at[k])

    def xrows(r0, r1, k):
        return cp(x_hbm.at[0, pl.ds(r0, r1 - r0)], x_v.at[pl.ds(r0, r1 - r0)], k)

    def wk_cols(c0, n, k):
        return cp(wqkv_hbm.at[:, pl.ds(D + c0, n)], wk_v.at[:, pl.ds(c0, n)], k)

    g_phi = [cp(wphi_hbm, wphi_v, 0)]
    g_x0 = [xrows(0, 256, 1)]
    g_ka = [wk_cols(0, 256, 2)]
    g_kb = [wk_cols(256, 256, 3)]
    g_kc = [wk_cols(512, 128, 0), xrows(256, P1, 0)]
    g_qv = [cp(wqkv_hbm.at[:, pl.ds(0, D)], wq_v, 1), cp(wqkv_hbm.at[:, pl.ds(2 * D, D)], wv_v, 1),
            xrows(P1, P1 + 128, 1)]
    g_xr = [xrows(P1 + 128, S, 2), cp(wg_hbm, wgu_v.at[0, pl.ds(0, D)], 2)]
    g_w = [cp(wu_hbm, wgu_v.at[1, pl.ds(0, D)], 3), cp(wd_hbm, wd2.at[0, pl.ds(0, F)], 3), cp(wo_hbm, wo_v, 3)]

    def waits(cs, starts=()):
        for c in cs:
            c.wait()
        for c in starts:
            c.start()

    for c in g_phi + g_x0 + g_ka + g_kb:
        c.start()

    def ln_rows(r0, n, dst, d0):
        for c in range(0, n, LNC):
            xn = _ln(x_v[pl.ds(r0 + c, LNC), :].astype(f32)).astype(bf16)
            dst[(d0 + c) // 2:(d0 + c + LNC) // 2, :] = _pk(xn)

    fill = []
    pending = []

    def drain(keep=0):
        while len(pending) > keep:
            pending.pop(0)()

    def phi_store(dst, g, x, c0):
        T, role = divmod(g, 3)
        cols = pl.ds(c0, 128)
        if role == 0:
            dst[2 * T, 0:40, cols] = jnp.concatenate(x, axis=0)
        elif role == 2:
            dst[2 * T + 1, 24:64, cols] = jnp.concatenate(x, axis=0)
        else:
            even = (lax.broadcasted_iota(jnp.int32, (8, 128), 0) & 1) == 0
            ev = [jnp.where(even, x[a], pltpu.roll(x[a + 1], 1, 0)) for a in (0, 2)]
            od = [jnp.where(even, pltpu.roll(x[a], 7, 0), x[a + 1]) for a in (0, 2)]
            dst[2 * T, 40:64, cols] = jnp.concatenate(ev + [x[4]], axis=0)
            dst[2 * T + 1, 0:24, cols] = jnp.concatenate(od + [x[4]], axis=0)

    def feat_block(p, dst, b, c0, rfirst=True):
        ro, mo = (0, 24) if rfirst else (128, 0)
        rs = [p[ro + 8 * a:ro + 8 + 8 * a] for a in range(3)]
        for a in range(4):
            if a < 3:
                v4 = jnp.where(_pair_is(a, 128), 0.0, rs[a])
            else:
                v4 = jnp.where(_pair_is(0, 128), rs[0],
                               jnp.where(_pair_is(1, 128), rs[1], jnp.where(_pair_is(2, 128), rs[2], 0.0)))
            ps = [p[mo + 32 * a + 8 * v:mo + 8 + 32 * a + 8 * v] for v in range(4)] + [v4]
            phi_store(dst, 4 * b + a, _feat5(ps), c0)

    def xs(xref, xr0):
        return _up(xref[xr0 // 2:xr0 // 2 + 64, :])

    def proj_qk(off, dst, B, xref, xr0, c0):
        p = _nt(_up(wT[off + 152 * B:off + 152 * B + 152, :]), xs(xref, xr0))

        def post():
            feat_block(p[0:152], dst, 2 * B, c0)
            feat_block(p[152:304], dst, 2 * B + 1, c0)
        pending.append(post)

    def proj_k4(wb, b, j, rfirst):
        p = _nt(wb, xs(xn0, 128 * j))
        pending.append(lambda: feat_block(p[0:152], phik, b, 128 * j, rfirst))

    def proj_v(xref, xr0, c0, split_last=False):
        cuts = [0, 80, 160, 240, 280, 320] if split_last else [0, 80, 160, 240, 320]
        p = jnp.concatenate([_nt(_up(wT[V_OFF + a:V_OFF + b, :]), xs(xref, xr0))
                             for a, b in zip(cuts[:-1], cuts[1:])], axis=0)
        low = lax.broadcasted_iota(jnp.int32, (8, 128), 0) < 4
        cols = pl.ds(c0, 128)
        sl = [p[8 * a:8 * a + 8] for a in range(80)]

        def put(t, slabs):
            vaug[t, 0:4 * len(slabs), cols] = jnp.concatenate(
                [_pe(slabs[a], slabs[a + 1]) for a in range(0, len(slabs), 2)], axis=0)
        for T in range(5):
            mid = sl[15 * T + 7]
            put(2 * T, sl[15 * T:15 * T + 7] + [jnp.where(low, mid, 1.0)])
            put(2 * T + 1, [jnp.where(low, 1.0, mid)] + sl[15 * T + 8:15 * T + 15])
            if fill:
                fill.pop(0)()
        put(10, sl[75:80] + [jnp.ones((8, 128), f32)])

    pr = lax.broadcasted_iota(jnp.int32, (D, D), 0)
    pc = lax.broadcasted_iota(jnp.int32, (D, D), 1)
    perm = jnp.where((pr & 31) * DH + (pr >> 5) == pc, 1.0, 0.0).astype(bf16)
    r_i = lax.broadcasted_iota(jnp.int32, (160, 32), 0)
    c_i = lax.broadcasted_iota(jnp.int32, (160, 32), 1)
    gl = r_i // 40
    sl = (r_i - 40 * gl) >> 1
    q_ = sl - 16
    f_ = jnp.where(sl < 16, sl + 1, jnp.where(q_ == gl, 0, jnp.where(q_ < gl, 17 + q_, 16 + q_)))
    e0 = jnp.where(f_ == c_i, 1.0, 0.0)
    es = []
    for t in range(5):
        off = (120 * t) % 160
        es.append((jnp.concatenate([e0[off:], e0[:off]], axis=0) if off else e0).astype(bf16))
    r2 = lax.broadcasted_iota(jnp.int32, (160, 128), 0)
    hr = 2 * (r2 // 40) + (r2 & 1)
    hc = [(lax.broadcasted_iota(jnp.int32, (1, 128), 1) + 128 * t) // DH - 6 * t for t in range(5)]
    bcat[...] = jnp.zeros(bcat.shape, f32)

    waits(g_phi, g_kc)
    for d in range(DH):
        bcat[0:DH, 32 * d:32 * d + 32] = wphi_v[d].astype(f32)
    at = _nn(bcat[...].astype(bf16), perm).astype(bf16)
    pts = [jnp.where(hr == hc[t], _nn(es[t], at[:, 128 * t:128 * t + 128]), 0.0).astype(bf16) for t in range(5)]

    def fold(w_v, off, t, rs, blk):
        rs[t] = _nt(pts[t], w_v[:, 128 * t:128 * t + 128])
        if t == 0:
            return
        b = t - 1
        lo, hi = rs[t - 1], rs[t]
        parts = []
        if b < 3:
            parts.append(lo[40 * b:120])
        parts.append(lo[120:160] + hi[0:40])
        if b > 0:
            parts.append(hi[40:40 + 40 * b])
        w = jnp.concatenate(parts, axis=0)
        mains, v4s = [], []
        for a in range(4):
            v4 = w[40 * a + 32:40 * a + 40]
            base = _allred(jnp.where(_pair_is(a, D), v4, 0.0), jnp.add)
            mains += [(w[40 * a + 8 * v:40 * a + 8 * v + 8] - base) * LOG2E for v in range(4)]
            v4s.append((v4 - base) * LOG2E)
        shared = [jnp.where(_pair_is(a, D), v4s[3], v4s[a]) for a in range(3)]
        blk[b] = (shared, mains)
        if b % 2 == 1:
            B = b // 2
            rows = blk[b - 1][0] + blk[b - 1][1] + blk[b][0] + blk[b][1]
            wT[off + 152 * B:off + 152 * B + 152, :] = _pk(jnp.concatenate(rows, axis=0).astype(bf16))

    def blk16(slabs, rfirst):
        rows = slabs[0] + slabs[1] if rfirst else slabs[1] + slabs[0]
        return jnp.concatenate(rows + [jnp.zeros((8, D), f32)], axis=0).astype(bf16)

    waits(g_x0, g_qv)
    ln_rows(0, 256, xn0, 0)

    rk, rq, bk, bq = {}, {}, {}, {}
    waits(g_ka, g_xr)
    fold(wk_v, K_OFF, 0, rk, bk)
    fold(wk_v, K_OFF, 1, rk, bk)
    w0 = blk16(bk[0], False)
    proj_k4(w0, 0, 0, False)
    proj_k4(w0, 0, 1, False)

    waits(g_kb, g_w)
    fold(wk_v, K_OFF, 2, rk, bk)
    fold(wk_v, K_OFF, 3, rk, bk)
    w1 = blk16(bk[1], False)
    proj_k4(w1, 1, 0, False)
    proj_k4(w1, 1, 1, False)
    w2 = blk16(bk[2], True)
    proj_k4(w2, 2, 0, True)
    drain(1)

    waits(g_kc)
    fold(wk_v, K_OFF, 4, rk, bk)
    proj_k4(w2, 2, 1, True)
    ln_rows(256, P1 - 256, xn0, 256)
    w3 = blk16(bk[3], True)
    proj_k4(w3, 3, 0, True)
    proj_k4(w3, 3, 1, True)
    for j in range(2, NP):
        for B in range(2):
            proj_qk(K_OFF, phik, B, xn0, 128 * j, 128 * j)
    drain(1)

    waits(g_qv)
    for t in range(5):
        fold(wq_v, Q_OFF, t, rq, bq)
    for t in range(5):
        wT[V_OFF + 64 * t:V_OFF + 64 * t + 64, :] = _pk(wv_v[:, 128 * t:128 * t + 128].T)
    ln_rows(P1, 128, xn_buf, 0)
    for j in range(NP):
        for B in range(2):
            proj_qk(Q_OFF, phiq, B, xn0, 128 * j, 128 * j)
    drain()
    for j in range(NP):
        proj_v(xn0, 128 * j, 128 * j, j == NP - 1)

    nc = F // FC

    def tables(ref, src, dst, r0, c0, place):
        for r in range(0, 256, TB2):
            for l in range(0, 256, TBC):
                f11, f12, f21, f22 = [
                    ref[src, r0 + 256 * a + r:r0 + 256 * a + r + TB2, c0 + 256 * b + l:c0 + 256 * b + l + TBC].astype(f32)
                    for a in range(2) for b in range(2)]
                for k, t in enumerate([f11 + f22, f12 - f22, f21 - f11, f11 + f12, f21 + f22]):
                    r1, c1 = place(k)
                    ref[dst, r1 + r:r1 + r + TB2, c1 + l:c1 + l + TBC] = t.astype(bf16)

    def rhs7(b11, b12, b21, b22):
        return [b11 + b22, b11, b12 - b22, b21 - b11, b22, b11 + b12, b21 + b22]

    RH = ((0, 3), (0,), (1, 3), (2, 0), (3,), (0, 1), (2, 3))
    SG = (1, 0, -1, -1, 0, 1, 1)

    def tables2(ref, src, dst, c0):
        for r in range(0, 128, 8):
            for k1 in range(7):
                def ld(q, a):
                    r0 = 256 * (q // 2) + 128 * a + r
                    return ref[src, r0:r0 + 8, c0 + 256 * (q % 2):c0 + 256 * (q % 2) + 256].astype(f32)
                rows = []
                for a in range(2):
                    t = ld(RH[k1][0], a)
                    if SG[k1] > 0:
                        t = t + ld(RH[k1][1], a)
                    elif SG[k1] < 0:
                        t = t - ld(RH[k1][1], a)
                    rows.append(t)
                ts = rhs7(rows[0][:, 0:128], rows[0][:, 128:256], rows[1][:, 0:128], rows[1][:, 128:256])
                ref[dst, 256 * k1 + r:256 * k1 + r + 8, c0:c0 + 512] = jnp.concatenate(ts[0:4], axis=1).astype(bf16)
                ref[dst, 256 * k1 + 128 + r:256 * k1 + 128 + r + 8, c0:c0 + 384] = jnp.concatenate(ts[4:7], axis=1).astype(bf16)

    def gu_place(c):
        return lambda k: (256 * (k // 2), c * FC + 256 * (k % 2))

    def dn_place(c):
        return lambda k: (256 * ((5 * c + k) // 2), 256 * ((5 * c + k) % 2))

    def p1(i, carry):
        @pl.when(i == N1 - 1)
        def _():
            waits(g_w)
        for c in range(nc):
            tables2(wgu_v, i, jnp.minimum(i, 1) + 2, c * FC)
        for j in range(R):
            c0 = pl.multiple_of(P1 + i * T1 + 128 * j, 128)
            rn = pl.multiple_of(P1 + i * T1 + 128 * (j + 1), 128)
            ln_rows(rn, 128, xn_buf, 128 * ((j + 1) % R))
            for off, dst in ((K_OFF, phik), (Q_OFF, phiq)):
                for B in range(2):
                    proj_qk(off, dst, B, xn_buf, 128 * j, c0)
                    drain()
            proj_v(xn_buf, 128 * j, c0)
        while fill:
            fill.pop(0)()
        return carry

    waits(g_xr)
    lax.fori_loop(0, N1, p1, 0)

    pid = pl.program_id(0)
    for c in range(nc):
        tables(wd2, pid, 1, c * FC, 0, dn_place(c))
    proj_v(xn_buf, 0, S - 128)
    for B in range(2):
        proj_qk(K_OFF, phik, B, xn_buf, 0, S - 128)
    for B in range(2):
        proj_qk(Q_OFF, phiq, B, xn_buf, 0, S - 128)
    drain()

    rr = lax.broadcasted_iota(jnp.int32, (64, 128), 0)
    cc = lax.broadcasted_iota(jnp.int32, (64, 128), 1)
    par = (cc >> 1) & 1
    col0 = jnp.where(cc < 80, par, jnp.where(cc < 112, 2, 2 + par))
    col1 = jnp.where(cc < 32, 0, jnp.where(cc < 48, par - 1, 1 + par))
    row0 = jnp.where(rr < 60, rr // DH, jnp.minimum(rr - 60, 2))
    row1 = jnp.where(rr < 4, jnp.minimum(rr, 2), (rr - 4) // DH)
    msks = (col0 == row0, col1 == row1)

    def unzip(y):
        u = _pk(y.astype(bf16))
        lo = lax.bitcast_convert_type(u << 16, f32)
        hi = lax.bitcast_convert_type(u & jnp.uint32(0xFFFF0000), f32)
        return jnp.concatenate([t[a:a + 8] for a in range(0, u.shape[0], 8) for t in (lo, hi)], axis=0)

    for t in range(10):
        for _ in range(2):
            if fill:
                fill.pop(0)()
        kvm[t] = _pk(jnp.where(msks[t % 2], unzip(_nt(_up(vaug[t]), _up(phik[t]))), 0.0).astype(bf16))
    rl = lax.broadcasted_iota(jnp.int32, (48, 80), 0)
    cl = lax.broadcasted_iota(jnp.int32, (48, 80), 1)
    rowl = jnp.where(rl < 40, (rl >= 20).astype(jnp.int32), (rl >= 44).astype(jnp.int32))
    kvl = unzip(_nt(_up(vaug[10, 0:24, :]), _up(phik[10, 0:40, :])))
    kvm[10, 0:24, 0:80] = _pk(jnp.where(((cl >> 1) & 1) == rowl, kvl, 0.0).astype(bf16))
    while fill:
        fill.pop(0)()

    def attn_o(c0):
        low = lax.broadcasted_iota(jnp.int32, (8, NW), 0) < 4
        cols = pl.ds(c0, NW)

        def bc(r, k):
            return jnp.broadcast_to(r[k:k + 1], (8, NW))
        os = []
        for T in range(5):
            n0 = _nn(_up(kvm[2 * T]), _up(phiq[2 * T, :, cols]))
            n1 = _nn(_up(kvm[2 * T + 1]), _up(phiq[2 * T + 1, :, cols]))
            r0 = _rcp(n0[56:64] + 1e-6)
            r1 = _rcp(n1[0:8] + 1e-6)
            a, b, c = bc(r0, 4), bc(r0, 5), bc(r0, 6)
            d, e, f = bc(r1, 0), bc(r1, 1), bc(r1, 2)
            os += [n0[0:8] * a, n0[8:16] * a, n0[16:24] * jnp.where(low, a, b), n0[24:32] * b, n0[32:40] * b,
                   n0[40:48] * c, n0[48:56] * c, jnp.where(low, n0[56:64] * c, n1[0:8] * d),
                   n1[8:16] * d, n1[16:24] * d, n1[24:32] * e, n1[32:40] * e, n1[40:48] * jnp.where(low, e, f),
                   n1[48:56] * f, n1[56:64] * f]
        nd = _nn(_up(kvm[10, 0:24, 0:80]), _up(phiq[10, 0:40, cols]))
        r = _rcp(nd[40:48] + 1e-6)
        rrot = pltpu.roll(r, 4, 0)
        ra = jnp.where(low, r, rrot)
        rb = jnp.where(low, rrot, r)
        os += [nd[0:8] * ra, nd[8:16] * ra, nd[16:24] * r, nd[24:32] * rb, nd[32:40] * rb]
        return jnp.concatenate(os, axis=0).astype(bf16).T

    def lhs7(a11, a12, a21, a22):
        return [(a11 + a22).astype(bf16), (a21 + a22).astype(bf16), a11.astype(bf16), a22.astype(bf16),
                (a11 + a12).astype(bf16), (a21 - a11).astype(bf16), (a12 - a22).astype(bf16)]

    NS = T2 // 64

    def quarter(x, q):
        return jnp.concatenate([x[64 * s_ + 16 * q:64 * s_ + 16 * q + 16] for s_ in range(NS)], axis=0)

    def natural(qs, s0, s1):
        return jnp.concatenate([qs[q][16 * s_:16 * s_ + 16] for s_ in range(s0, s1) for q in range(4)], axis=0)

    def comb(q):
        return [[q[3] - q[4] + q[0] + q[6], q[2] + q[4]], [q[1] + q[3], q[2] - q[1] + q[0] + q[5]]]

    def run(*streams):
        streams = [list(t) for t in streams]
        while any(streams):
            for t in streams:
                if t:
                    t.pop(0)()

    def p2(i, carry):
        o = jnp.concatenate([attn_o(pl.multiple_of(i * T2 + w, NW)) for w in range(0, T2, NW)], axis=0)
        hs, hns = [], []
        for w in range(0, T2, 64):
            r0 = pl.multiple_of(i * T2 + w, 64)
            h = x_v[pl.ds(r0, 64), :].astype(f32) + _nn(o[w:w + 64], wo_v[...])
            hs.append(h)
            hns.append(_ln(h))
        h = jnp.concatenate(hs, axis=0)
        hn = jnp.concatenate(hns, axis=0)
        hq = [quarter(hn[:, 0:512], q) for q in range(4)]
        top = jnp.concatenate(hq[0:2], axis=0)
        bot = jnp.concatenate(hq[2:4], axis=0)
        a11_, a12_, a21_, a22_ = top[:, 0:256], top[:, 256:512], bot[:, 0:256], bot[:, 256:512]
        L1 = [a11_ + a22_, a21_ + a22_, a11_, a22_, a11_ + a12_, a21_ - a11_, a12_ - a22_]
        L = [lhs7(t[:128, :128], t[:128, 128:], t[128:, :128], t[128:, 128:]) for t in L1]
        hr_ = hn[:, 512:640].astype(bf16)

        gp = {}
        rp = {}
        dp = {}
        dr = {rb: h[128 * rb:128 * rb + 128, 512:640] for rb in range(4)}
        act = {}
        dl = {}

        def G(c, k):
            def step(k2):
                r0, c1 = 256 * k + 128 * (k2 // 4), c * FC + 128 * (k2 % 4)
                for w in range(2):
                    gp[c, w, k, k2] = _nn(L[k][k2], wgu_v[2 + w, r0:r0 + 128, c1:c1 + 128])
            return [(lambda k2=k2: step(k2)) for k2 in (2, 4, 1, 3, 0, 6, 5)]

        def Rr(c):
            def step(rb, b, w):
                rp[c, w, rb, b] = _nn(hr_[128 * rb:128 * rb + 128],
                                      wgu_v[w, 512:640, c * FC + 256 * b:c * FC + 256 * b + 256])
            return [(lambda rb=rb, b=b, w=w: step(rb, b, w)) for rb in range(4) for b in (1, 0) for w in range(2)]

        def M(c, w, k):
            t = comb([gp[c, w, k, k2] for k2 in range(7)])
            return jnp.concatenate([jnp.concatenate(r_, axis=1) for r_ in t], axis=0)

        def quad(c, a, b):
            gu_ = []
            for w in range(2):
                rfull = jnp.concatenate([rp[c, w, rb, b] for rb in range(4)], axis=0)
                t = jnp.concatenate([quarter(rfull, 2 * a), quarter(rfull, 2 * a + 1)], axis=0)
                for sg, k in {(0, 1): ((1, 2), (1, 4)), (1, 0): ((1, 1), (1, 3)),
                              (0, 0): ((1, 3), (-1, 4), (1, 0), (1, 6)),
                              (1, 1): ((1, 2), (-1, 1), (1, 0), (1, 5))}[a, b]:
                    t = t + mm_[c, w, k] if sg > 0 else t - mm_[c, w, k]
                gu_.append(t)
            act[c, a, b] = _gelu_mul(*gu_)

        mm_ = {}

        def fin(c, *ks):
            for k in ks:
                for w in range(2):
                    mm_[c, w, k] = M(c, w, k)

        def dlhs(c, k):
            if (c, k) not in dl:
                a = lambda x, y: act[c, x, y]
                dl[c, k] = [lambda: a(0, 0) + a(1, 1), lambda: a(1, 0) + a(1, 1), lambda: a(0, 0), lambda: a(1, 1),
                            lambda: a(0, 0) + a(0, 1), lambda: a(1, 0) - a(0, 0), lambda: a(0, 1) - a(1, 1),
                            lambda: a(0, 1), lambda: a(1, 0)][k]().astype(bf16)
            return dl[c, k]

        def drhs(c, k):
            if k == 1:
                return wd2.at[0, pl.ds(c * FC, 256), pl.ds(0, 256)]
            if k == 4:
                return wd2.at[0, pl.ds(c * FC + 256, 256), pl.ds(256, 256)]
            r1, c1 = dn_place(c)((0, None, 1, 2, None, 3, 4)[k])
            return wd2.at[1, pl.ds(r1, 256), pl.ds(c1, 256)]

        def Dk(c, k):
            def step(rh, ch):
                t = _nn(dlhs(c, k)[128 * rh:128 * rh + 128], drhs(c, k)[:, 128 * ch:128 * ch + 128])
                dp[k, rh, ch] = t if (k, rh, ch) not in dp else dp[k, rh, ch] + t
            return [(lambda rh=rh, ch=ch: step(rh, ch)) for rh in range(2) for ch in range(2)]

        def a_nat(c):
            qs = [jnp.concatenate([dlhs(c, (2, 8)[q // 2])[128 * (q % 2):128 * (q % 2) + 128],
                                   dlhs(c, (7, 3)[q // 2])[128 * (q % 2):128 * (q % 2) + 128]], axis=1) for q in range(4)]
            return qs

        def Dr(c):
            def step(rb):
                dr[rb] = dr[rb] + _nn(natural(a_nat(c), 2 * rb, 2 * rb + 2), wd2[0, c * FC:(c + 1) * FC, 512:640])
            return [(lambda rb=rb: step(rb)) for rb in range(4)]

        def out_block(r0, n, c0, w, val):
            rr0 = pl.multiple_of(i * T2 + r0, 16)
            out_v[pl.ds(rr0, n), c0:c0 + w] = val.astype(bf16)
            cp(out_v.at[pl.ds(rr0, n), pl.ds(c0, w)], out_hbm.at[0, pl.ds(rr0, n), pl.ds(c0, w)], 0).start()

        def dm(k, rh):
            return jnp.concatenate([dp[k, rh, 0], dp[k, rh, 1]], axis=1)

        run(Rr(0))
        run(G(0, 2))
        held = []
        for c in range(nc):
            fin(c, 2)
            run(G(c, 4), G(c, 1))
            fin(c, 4, 1)
            quad(c, 0, 1)
            run(G(c, 3), G(c, 0))
            fin(c, 3, 0)
            quad(c, 1, 0)
            run(G(c, 6), G(c + 1, 2) if c + 1 < nc else held)
            fin(c, 6)
            quad(c, 0, 0)
            if c + 1 < nc:
                rn_ = Rr(c + 1)
                run(G(c, 5), rn_[:7])
                fin(c, 5)
                quad(c, 1, 1)
                run(rn_[7:] + Dk(c, 2) + Dk(c, 4) + Dk(c, 5))
                late = Dk(c, 0) + Dk(c, 1) + Dk(c, 3) + Dk(c, 6)
                if c + 2 == nc:
                    held, late = late[-7:], late[:-7]
                run(late + Dr(c))
            else:
                d24 = Dk(c, 2) + Dk(c, 4)
                run(G(c, 5), d24)
                fin(c, 5)
                quad(c, 1, 1)
                run(Dk(c, 5) + Dk(c, 0) + Dk(c, 1))
                qs = [dm(2, 0) + dm(4, 0), dm(2, 1) + dm(4, 1),
                      dm(2, 0) - dm(1, 0) + dm(0, 0) + dm(5, 0), dm(2, 1) - dm(1, 1) + dm(0, 1) + dm(5, 1)]
                out_block(0, T2, 256, 256, h[:, 256:512] + natural(qs, 0, NS))
                run(Dr(c))
                out_block(0, T2, 512, 128, jnp.concatenate([dr[rb] for rb in range(4)], axis=0))
                run(Dk(c, 3))
                part = [dm(3, 0) - dm(4, 0) + dm(0, 0) + dm(6, 0), dm(3, 1) - dm(4, 1) + dm(0, 1) + dm(6, 1),
                        dm(1, 0) + dm(3, 0), dm(1, 1) + dm(3, 1)]
                l6 = dlhs(c, 6)
                for s0, s1 in ((0, 4), (4, 6), (6, 7), (7, 8)):
                    n = 16 * (s1 - s0)
                    t = _nn(jnp.concatenate([l6[16 * s0:16 * s1], l6[128 + 16 * s0:128 + 16 * s1]], axis=0), drhs(c, 6)[...])
                    qs = [part[0][16 * s0:16 * s1] + t[0:n], part[1][16 * s0:16 * s1] + t[n:2 * n],
                          part[2][16 * s0:16 * s1], part[3][16 * s0:16 * s1]]
                    out_block(64 * s0, 64 * (s1 - s0), 0, 256, h[64 * s0:64 * s1, 0:256] + natural(qs, 0, s1 - s0))
        return carry

    lax.fori_loop(0, N2, p2, 0)
    cp(out_v, out_hbm.at[0], 0).wait()


def _kernel(*refs):
    @pl.when(pl.program_id(0) == 0)
    def _():
        _body(*refs)


@jax.jit
def pallas_sequential_preLN__linear_kernel_hedgehog__geglu_ffn__prompt_kernel(
    A_x: jax.Array,
    A_wqkv: jax.Array,
    A_w_phi: jax.Array,
    A_wo: jax.Array,
    B_x: jax.Array,
    B_w_gate: jax.Array,
    B_w_up: jax.Array,
    B_w_down: jax.Array,
):
    del B_x
    anyspec = pl.BlockSpec(memory_space=pl.ANY)
    wphi_t = jnp.transpose(A_w_phi, (1, 2, 0))
    return pl.pallas_call(
        _kernel,
        out_shape=jax.ShapeDtypeStruct((1, S, D), bf16),
        grid=(2,),
        in_specs=[anyspec] * 7,
        out_specs=anyspec,
        scratch_shapes=[
            pltpu.VMEM((S, D), bf16),
            pltpu.VMEM((D, D), bf16),
            pltpu.VMEM((D, D), bf16),
            pltpu.VMEM((D, D), bf16),
            pltpu.VMEM((DH, DH, H), bf16),
            pltpu.VMEM((D, D), bf16),
            pltpu.VMEM((4, 1792, F), bf16),
            pltpu.VMEM((2, 2048, D), bf16),
            pltpu.VMEM((928, D), u32),
            pltpu.VMEM((32, D), f32),
            pltpu.VMEM((P1 // 2, D), u32),
            pltpu.VMEM((T1 // 2, D), u32),
            pltpu.VMEM((11, 64, S), u32),
            pltpu.VMEM((11, 64, S), u32),
            pltpu.VMEM((11, 32, S), u32),
            pltpu.VMEM((11, 32, 128), u32),
            pltpu.VMEM((S, D), bf16),
            pltpu.SemaphoreType.DMA((4,)),
        ],
        compiler_params=pltpu.CompilerParams(
            dimension_semantics=("arbitrary",),
            vmem_limit_bytes=100 * 1024 * 1024,
            disable_bounds_checks=True,
            disable_semaphore_checks=True,
        ),
        name="hh",
    )(A_x, A_wqkv, wphi_t, A_wo, B_w_gate, B_w_up, B_w_down)
```

```python
import jax
import jax.numpy as jnp
from jax import lax
from jax.experimental import pallas as pl
from jax.experimental.pallas import tpu as pltpu

S, D, H, DH, F = 2048, 640, 32, 20, 1536
NG = H // 2
LOG2E = 1.4426950408889634
NT_DIMS = (((1,), (1,)), ((), ()))
f32 = jnp.float32
bf16 = jnp.bfloat16
u32 = jnp.uint32

NP = 5
R = 5
T1 = 128 * R
P1 = 128 * NP
N1 = (S - P1 - 128) // T1
T2 = 512
N2 = S // T2
NW = 256
WOB = 64
LNC = 64
TBR = 32
TB2, TBC = 8, 256
TGRP = [[k] for k in range(7)]
HOPS = 1
TAIL = 1
RP = ((0, 256), (256, 128), (384, 64), (448, 32), (480, 32))
FC = 512
PIECES = (128, 128, 128, 64, 32, 32)
POFF = tuple(sum(PIECES[:k]) for k in range(len(PIECES)))
K_OFF, Q_OFF, V_OFF = 0, 304, 608
assert P1 + N1 * T1 + 128 == S and sum(PIECES) == T2


def _ln(x):
    m = jnp.mean(x, axis=-1, keepdims=True)
    xc = x - m
    v = jnp.mean(xc * xc, axis=-1, keepdims=True) + 1e-5
    return xc * jnp.exp2(jnp.log(v) * (-0.5 * LOG2E))


def _rcp(x):
    return pl.reciprocal(x, approx=True)


def _allred(m, op):
    m = op(m, pltpu.roll(m, 2, 0))
    return op(m, pltpu.roll(m, 4, 0))


def _tree(op, xs):
    return op(op(op(xs[0], xs[1]), op(xs[2], xs[3])), xs[4])


def _feat5(ps):
    mx = _allred(_tree(jnp.maximum, ps), jnp.maximum)
    mn = _allred(_tree(jnp.minimum, ps), jnp.minimum)
    ep = [jnp.exp2(q - mx) for q in ps]
    en = [jnp.exp2(mn - q) for q in ps]
    rp = _rcp(_allred(_tree(jnp.add, ep), jnp.add))
    rn = _rcp(_allred(_tree(jnp.add, en), jnp.add))
    return [_pe(a * rp, b * rn) for a, b in zip(ep, en)]


def _gelu_mul(g, u):
    c = 0.7978845608028654
    t = jnp.tanh(g * (c + (c * 0.044715) * (g * g)))
    hgu = (0.5 * g) * u
    return hgu + hgu * t


def _pk(v):
    return pltpu.bitcast(v, u32)


def _pe(a, b):
    return pltpu.pack_elementwise([a, b], packed_dtype=bf16)


def _up(v):
    return pltpu.bitcast(v, bf16)


def _nt(a, b):
    return lax.dot_general(a, b, NT_DIMS, preferred_element_type=f32)


def _nn(a, b):
    return jnp.dot(a, b, preferred_element_type=f32)


def _pair_is(a, w):
    return (lax.broadcasted_iota(jnp.int32, (8, w), 0) >> 1) == a


def _body(x_hbm, wqkv_hbm, wphi_hbm, wo_hbm, wg_hbm, wu_hbm, wd_hbm, out_hbm,
          x_v, wq_v, wk_v, wv_v, wphi_v, wo_v, wgu_v, wd2, wT, bcat,
          xn0, xn_buf, phiq, phik, vaug, kvm, dacc, out_v, sem):
    def cp(src, dst, k):
        return pltpu.make_async_copy(src, dst, sem.at[k])

    def xrows(r0, r1, k):
        return cp(x_hbm.at[0, pl.ds(r0, r1 - r0)], x_v.at[pl.ds(r0, r1 - r0)], k)

    def wk_cols(c0, n, k):
        return cp(wqkv_hbm.at[:, pl.ds(D + c0, n)], wk_v.at[:, pl.ds(c0, n)], k)

    g_phi = [cp(wphi_hbm, wphi_v, 0)]
    g_x0 = [xrows(0, 256, 1)]
    g_ka = [wk_cols(0, 256, 2)]
    g_kb = [wk_cols(256, 256, 3)]
    g_kc = [wk_cols(512, 128, 0), xrows(256, P1, 0)]
    g_qv = [cp(wqkv_hbm.at[:, pl.ds(0, D)], wq_v, 1), cp(wqkv_hbm.at[:, pl.ds(2 * D, D)], wv_v, 1),
            xrows(P1, P1 + 128, 1)]
    g_xr = [xrows(P1 + 128, S, 2), cp(wg_hbm, wgu_v.at[0, pl.ds(0, D)], 2)]
    g_w = [cp(wu_hbm, wgu_v.at[1, pl.ds(0, D)], 3), cp(wd_hbm, wd2.at[0, pl.ds(0, F)], 3), cp(wo_hbm, wo_v, 3)]

    def waits(cs, starts=()):
        for c in cs:
            c.wait()
        for c in starts:
            c.start()

    for c in g_phi + g_x0 + g_ka + g_kb:
        c.start()

    def ln_rows(r0, n, dst, d0):
        for c in range(0, n, LNC):
            xn = _ln(x_v[pl.ds(r0 + c, LNC), :].astype(f32)).astype(bf16)
            dst[(d0 + c) // 2:(d0 + c + LNC) // 2, :] = _pk(xn)

    fill = []
    pending = []

    def drain(keep=0):
        while len(pending) > keep:
            pending.pop(0)()

    def phi_store(dst, g, x, c0):
        T, role = divmod(g, 3)
        cols = pl.ds(c0, 128)
        if role == 0:
            dst[2 * T, 0:40, cols] = jnp.concatenate(x, axis=0)
        elif role == 2:
            dst[2 * T + 1, 24:64, cols] = jnp.concatenate(x, axis=0)
        else:
            even = (lax.broadcasted_iota(jnp.int32, (8, 128), 0) & 1) == 0
            ev = [jnp.where(even, x[a], pltpu.roll(x[a + 1], 1, 0)) for a in (0, 2)]
            od = [jnp.where(even, pltpu.roll(x[a], 7, 0), x[a + 1]) for a in (0, 2)]
            dst[2 * T, 40:64, cols] = jnp.concatenate(ev + [x[4]], axis=0)
            dst[2 * T + 1, 0:24, cols] = jnp.concatenate(od + [x[4]], axis=0)

    def feat_block(p, dst, b, c0, rfirst=True):
        ro, mo = (0, 24) if rfirst else (128, 0)
        rs = [p[ro + 8 * a:ro + 8 + 8 * a] for a in range(3)]
        for a in range(4):
            if a < 3:
                v4 = jnp.where(_pair_is(a, 128), 0.0, rs[a])
            else:
                v4 = jnp.where(_pair_is(0, 128), rs[0],
                               jnp.where(_pair_is(1, 128), rs[1], jnp.where(_pair_is(2, 128), rs[2], 0.0)))
            ps = [p[mo + 32 * a + 8 * v:mo + 8 + 32 * a + 8 * v] for v in range(4)] + [v4]
            phi_store(dst, 4 * b + a, _feat5(ps), c0)

    def xs(xref, xr0):
        return _up(xref[xr0 // 2:xr0 // 2 + 64, :])

    def proj_qk(off, dst, B, xref, xr0, c0):
        p = _nt(_up(wT[off + 152 * B:off + 152 * B + 152, :]), xs(xref, xr0))

        def post():
            feat_block(p[0:152], dst, 2 * B, c0)
            feat_block(p[152:304], dst, 2 * B + 1, c0)
        pending.append(post)

    def proj_k4(wb, b, j, rfirst):
        p = _nt(wb, xs(xn0, 128 * j))
        pending.append(lambda: feat_block(p[0:152], phik, b, 128 * j, rfirst))

    def proj_v(xref, xr0, c0, split_last=False):
        cuts = [0, 80, 160, 240, 280, 320] if split_last else [0, 80, 160, 240, 320]
        p = jnp.concatenate([_nt(_up(wT[V_OFF + a:V_OFF + b, :]), xs(xref, xr0))
                             for a, b in zip(cuts[:-1], cuts[1:])], axis=0)
        low = lax.broadcasted_iota(jnp.int32, (8, 128), 0) < 4
        cols = pl.ds(c0, 128)
        sl = [p[8 * a:8 * a + 8] for a in range(80)]

        def put(t, slabs):
            vaug[t, 0:4 * len(slabs), cols] = jnp.concatenate(
                [_pe(slabs[a], slabs[a + 1]) for a in range(0, len(slabs), 2)], axis=0)
        for T in range(5):
            mid = sl[15 * T + 7]
            put(2 * T, sl[15 * T:15 * T + 7] + [jnp.where(low, mid, 1.0)])
            put(2 * T + 1, [jnp.where(low, 1.0, mid)] + sl[15 * T + 8:15 * T + 15])
            if fill:
                fill.pop(0)()
        put(10, sl[75:80] + [jnp.ones((8, 128), f32)])

    pr = lax.broadcasted_iota(jnp.int32, (D, D), 0)
    pc = lax.broadcasted_iota(jnp.int32, (D, D), 1)
    perm = jnp.where((pr & 31) * DH + (pr >> 5) == pc, 1.0, 0.0).astype(bf16)
    r_i = lax.broadcasted_iota(jnp.int32, (160, 32), 0)
    c_i = lax.broadcasted_iota(jnp.int32, (160, 32), 1)
    gl = r_i // 40
    sl = (r_i - 40 * gl) >> 1
    q_ = sl - 16
    f_ = jnp.where(sl < 16, sl + 1, jnp.where(q_ == gl, 0, jnp.where(q_ < gl, 17 + q_, 16 + q_)))
    e0 = jnp.where(f_ == c_i, 1.0, 0.0)
    es = []
    for t in range(5):
        off = (120 * t) % 160
        es.append((jnp.concatenate([e0[off:], e0[:off]], axis=0) if off else e0).astype(bf16))
    r2 = lax.broadcasted_iota(jnp.int32, (160, 128), 0)
    hr = 2 * (r2 // 40) + (r2 & 1)
    hc = [(lax.broadcasted_iota(jnp.int32, (1, 128), 1) + 128 * t) // DH - 6 * t for t in range(5)]
    bcat[...] = jnp.zeros(bcat.shape, f32)

    waits(g_phi, g_kc)
    for d in range(DH):
        bcat[0:DH, 32 * d:32 * d + 32] = wphi_v[d].astype(f32)
    at = _nn(bcat[...].astype(bf16), perm).astype(bf16)
    pts = [jnp.where(hr == hc[t], _nn(es[t], at[:, 128 * t:128 * t + 128]), 0.0).astype(bf16) for t in range(5)]

    def fold(w_v, off, t, rs, blk):
        rs[t] = _nt(pts[t], w_v[:, 128 * t:128 * t + 128])
        if t == 0:
            return
        b = t - 1
        lo, hi = rs[t - 1], rs[t]
        parts = []
        if b < 3:
            parts.append(lo[40 * b:120])
        parts.append(lo[120:160] + hi[0:40])
        if b > 0:
            parts.append(hi[40:40 + 40 * b])
        w = jnp.concatenate(parts, axis=0)
        mains, v4s = [], []
        for a in range(4):
            v4 = w[40 * a + 32:40 * a + 40]
            base = _allred(jnp.where(_pair_is(a, D), v4, 0.0), jnp.add)
            mains += [(w[40 * a + 8 * v:40 * a + 8 * v + 8] - base) * LOG2E for v in range(4)]
            v4s.append((v4 - base) * LOG2E)
        shared = [jnp.where(_pair_is(a, D), v4s[3], v4s[a]) for a in range(3)]
        blk[b] = (shared, mains)
        if b % 2 == 1:
            B = b // 2
            rows = blk[b - 1][0] + blk[b - 1][1] + blk[b][0] + blk[b][1]
            wT[off + 152 * B:off + 152 * B + 152, :] = _pk(jnp.concatenate(rows, axis=0).astype(bf16))

    def blk16(slabs, rfirst):
        rows = slabs[0] + slabs[1] if rfirst else slabs[1] + slabs[0]
        return jnp.concatenate(rows + [jnp.zeros((8, D), f32)], axis=0).astype(bf16)

    waits(g_x0, g_qv)
    ln_rows(0, 256, xn0, 0)

    rk, rq, bk, bq = {}, {}, {}, {}
    waits(g_ka, g_xr)
    fold(wk_v, K_OFF, 0, rk, bk)
    fold(wk_v, K_OFF, 1, rk, bk)
    w0 = blk16(bk[0], False)
    proj_k4(w0, 0, 0, False)
    proj_k4(w0, 0, 1, False)

    waits(g_kb, g_w)
    fold(wk_v, K_OFF, 2, rk, bk)
    fold(wk_v, K_OFF, 3, rk, bk)
    w1 = blk16(bk[1], False)
    proj_k4(w1, 1, 0, False)
    proj_k4(w1, 1, 1, False)
    w2 = blk16(bk[2], True)
    proj_k4(w2, 2, 0, True)
    drain(1)

    waits(g_kc)
    fold(wk_v, K_OFF, 4, rk, bk)
    proj_k4(w2, 2, 1, True)
    ln_rows(256, P1 - 256, xn0, 256)
    w3 = blk16(bk[3], True)
    proj_k4(w3, 3, 0, True)
    proj_k4(w3, 3, 1, True)
    for j in range(2, NP):
        for B in range(2):
            proj_qk(K_OFF, phik, B, xn0, 128 * j, 128 * j)
    drain(1)

    waits(g_qv)
    for t in range(5):
        fold(wq_v, Q_OFF, t, rq, bq)
    for t in range(5):
        wT[V_OFF + 64 * t:V_OFF + 64 * t + 64, :] = _pk(wv_v[:, 128 * t:128 * t + 128].T)
    ln_rows(P1, 128, xn_buf, 0)
    for j in range(NP):
        for B in range(2):
            proj_qk(Q_OFF, phiq, B, xn0, 128 * j, 128 * j)
    drain()
    for j in range(NP):
        proj_v(xn0, 128 * j, 128 * j, j == NP - 1)

    nc = F // FC

    def tables(ref, src, dst, r0, c0, place):
        for r in range(0, 256, TB2):
            for l in range(0, 256, TBC):
                f11, f12, f21, f22 = [
                    ref[src, r0 + 256 * a + r:r0 + 256 * a + r + TB2, c0 + 256 * b + l:c0 + 256 * b + l + TBC].astype(f32)
                    for a in range(2) for b in range(2)]
                for k, t in enumerate([f11 + f22, f12 - f22, f21 - f11, f11 + f12, f21 + f22]):
                    r1, c1 = place(k)
                    ref[dst, r1 + r:r1 + r + TB2, c1 + l:c1 + l + TBC] = t.astype(bf16)

    def rhs7(b11, b12, b21, b22):
        return [b11 + b22, b11, b12 - b22, b21 - b11, b22, b11 + b12, b21 + b22]

    RH = ((0, 3), (0,), (1, 3), (2, 0), (3,), (0, 1), (2, 3))
    SG = (1, 0, -1, -1, 0, 1, 1)

    def tables2(ref, src, dst, c0):
        for r in range(0, 128, 8):
            for grp in TGRP:
                cache = {}

                def ld(q, a):
                    if (q, a) not in cache:
                        r0 = 256 * (q // 2) + 128 * a + r
                        cache[q, a] = ref[src, r0:r0 + 8, c0 + 256 * (q % 2):c0 + 256 * (q % 2) + 256].astype(f32)
                    return cache[q, a]
                for k1 in grp:
                    for q in RH[k1]:
                        ld(q, 0), ld(q, 1)
                for k1 in grp:
                    rows = []
                    for a in range(2):
                        t = ld(RH[k1][0], a)
                        if SG[k1] > 0:
                            t = t + ld(RH[k1][1], a)
                        elif SG[k1] < 0:
                            t = t - ld(RH[k1][1], a)
                        rows.append(t)
                    ts = rhs7(rows[0][:, 0:128], rows[0][:, 128:256], rows[1][:, 0:128], rows[1][:, 128:256])
                    ref[dst, 256 * k1 + r:256 * k1 + r + 8, c0:c0 + 512] = jnp.concatenate(ts[0:4], axis=1).astype(bf16)
                    ref[dst, 256 * k1 + 128 + r:256 * k1 + 128 + r + 8, c0:c0 + 384] = jnp.concatenate(ts[4:7], axis=1).astype(bf16)
                    for _ in range(HOPS):
                        ref[dst, 256 * k1 + 128 + r:256 * k1 + 128 + r + 8, c0 + 384:c0 + 512] = ref[src, r:r + 8, c0:c0 + 128]

    def gu_place(c):
        return lambda k: (256 * (k // 2), c * FC + 256 * (k % 2))

    def dn_place(c):
        return lambda k: (256 * ((5 * c + k) // 2), 256 * ((5 * c + k) % 2))

    def p1(i, carry):
        @pl.when(i == N1 - 1)
        def _():
            waits(g_w)
        for c in range(nc):
            tables2(wgu_v, i, jnp.minimum(i, 1) + 2, c * FC)
        for j in range(R):
            c0 = pl.multiple_of(P1 + i * T1 + 128 * j, 128)
            rn = pl.multiple_of(P1 + i * T1 + 128 * (j + 1), 128)
            ln_rows(rn, 128, xn_buf, 128 * ((j + 1) % R))
            for off, dst in ((K_OFF, phik), (Q_OFF, phiq)):
                for B in range(2):
                    proj_qk(off, dst, B, xn_buf, 128 * j, c0)
                    drain()
            proj_v(xn_buf, 128 * j, c0)
        while fill:
            fill.pop(0)()
        return carry

    waits(g_xr)
    lax.fori_loop(0, N1, p1, 0)

    pid = pl.program_id(0)
    for c in range(nc):
        tables(wd2, pid, 1, c * FC, 0, dn_place(c))
    proj_v(xn_buf, 0, S - 128)
    for B in range(2):
        proj_qk(K_OFF, phik, B, xn_buf, 0, S - 128)
    for B in range(2):
        proj_qk(Q_OFF, phiq, B, xn_buf, 0, S - 128)
    drain()

    rr = lax.broadcasted_iota(jnp.int32, (64, 128), 0)
    cc = lax.broadcasted_iota(jnp.int32, (64, 128), 1)
    par = (cc >> 1) & 1
    col0 = jnp.where(cc < 80, par, jnp.where(cc < 112, 2, 2 + par))
    col1 = jnp.where(cc < 32, 0, jnp.where(cc < 48, par - 1, 1 + par))
    row0 = jnp.where(rr < 60, rr // DH, jnp.minimum(rr - 60, 2))
    row1 = jnp.where(rr < 4, jnp.minimum(rr, 2), (rr - 4) // DH)
    msks = (col0 == row0, col1 == row1)

    def unzip(y):
        u = _pk(y.astype(bf16))
        lo = lax.bitcast_convert_type(u << 16, f32)
        hi = lax.bitcast_convert_type(u & jnp.uint32(0xFFFF0000), f32)
        return jnp.concatenate([t[a:a + 8] for a in range(0, u.shape[0], 8) for t in (lo, hi)], axis=0)

    for t in range(10):
        for _ in range(2):
            if fill:
                fill.pop(0)()
        kvm[t] = _pk(jnp.where(msks[t % 2], unzip(_nt(_up(vaug[t]), _up(phik[t]))), 0.0).astype(bf16))
    rl = lax.broadcasted_iota(jnp.int32, (48, 80), 0)
    cl = lax.broadcasted_iota(jnp.int32, (48, 80), 1)
    rowl = jnp.where(rl < 40, (rl >= 20).astype(jnp.int32), (rl >= 44).astype(jnp.int32))
    kvl = unzip(_nt(_up(vaug[10, 0:24, :]), _up(phik[10, 0:40, :])))
    kvm[10, 0:24, 0:80] = _pk(jnp.where(((cl >> 1) & 1) == rowl, kvl, 0.0).astype(bf16))
    while fill:
        fill.pop(0)()

    def attn_o(c0):
        low = lax.broadcasted_iota(jnp.int32, (8, NW), 0) < 4
        cols = pl.ds(c0, NW)

        def bc(r, k):
            return jnp.broadcast_to(r[k:k + 1], (8, NW))
        os = []
        for T in range(5):
            n0 = _nn(_up(kvm[2 * T]), _up(phiq[2 * T, :, cols]))
            n1 = _nn(_up(kvm[2 * T + 1]), _up(phiq[2 * T + 1, :, cols]))
            r0 = _rcp(n0[56:64] + 1e-6)
            r1 = _rcp(n1[0:8] + 1e-6)
            a, b, c = bc(r0, 4), bc(r0, 5), bc(r0, 6)
            d, e, f = bc(r1, 0), bc(r1, 1), bc(r1, 2)
            os += [n0[0:8] * a, n0[8:16] * a, n0[16:24] * jnp.where(low, a, b), n0[24:32] * b, n0[32:40] * b,
                   n0[40:48] * c, n0[48:56] * c, jnp.where(low, n0[56:64] * c, n1[0:8] * d),
                   n1[8:16] * d, n1[16:24] * d, n1[24:32] * e, n1[32:40] * e, n1[40:48] * jnp.where(low, e, f),
                   n1[48:56] * f, n1[56:64] * f]
        nd = _nn(_up(kvm[10, 0:24, 0:80]), _up(phiq[10, 0:40, cols]))
        r = _rcp(nd[40:48] + 1e-6)
        rrot = pltpu.roll(r, 4, 0)
        ra = jnp.where(low, r, rrot)
        rb = jnp.where(low, rrot, r)
        os += [nd[0:8] * ra, nd[8:16] * ra, nd[16:24] * r, nd[24:32] * rb, nd[32:40] * rb]
        return jnp.concatenate(os, axis=0).astype(bf16).T

    def lhs7(a11, a12, a21, a22):
        return [(a11 + a22).astype(bf16), (a21 + a22).astype(bf16), a11.astype(bf16), a22.astype(bf16),
                (a11 + a12).astype(bf16), (a21 - a11).astype(bf16), (a12 - a22).astype(bf16)]

    NS = T2 // 64

    def quarter(x, q):
        return jnp.concatenate([x[64 * s_ + 16 * q:64 * s_ + 16 * q + 16] for s_ in range(NS)], axis=0)

    def natural(qs, s0, s1):
        return jnp.concatenate([qs[q][16 * s_:16 * s_ + 16] for s_ in range(s0, s1) for q in range(4)], axis=0)

    def comb(q):
        return [[q[3] - q[4] + q[0] + q[6], q[2] + q[4]], [q[1] + q[3], q[2] - q[1] + q[0] + q[5]]]

    def run(*streams):
        streams = [list(t) for t in streams]
        while any(streams):
            for t in streams:
                if t:
                    t.pop(0)()

    def p2(i, carry):
        o = jnp.concatenate([attn_o(pl.multiple_of(i * T2 + w, NW)) for w in range(0, T2, NW)], axis=0)
        hs, hns = [], []
        for w in range(0, T2, 64):
            r0 = pl.multiple_of(i * T2 + w, 64)
            h = x_v[pl.ds(r0, 64), :].astype(f32) + _nn(o[w:w + 64], wo_v[...])
            hs.append(h)
            hns.append(_ln(h))
        h = jnp.concatenate(hs, axis=0)
        hn = jnp.concatenate(hns, axis=0)
        hq = [quarter(hn[:, 0:512], q) for q in range(4)]
        top = jnp.concatenate(hq[0:2], axis=0)
        bot = jnp.concatenate(hq[2:4], axis=0)
        a11_, a12_, a21_, a22_ = top[:, 0:256], top[:, 256:512], bot[:, 0:256], bot[:, 256:512]
        L1 = [a11_ + a22_, a21_ + a22_, a11_, a22_, a11_ + a12_, a21_ - a11_, a12_ - a22_]
        L = [lhs7(t[:128, :128], t[:128, 128:], t[128:, :128], t[128:, 128:]) for t in L1]
        hr_ = [hn[128 * rb:128 * rb + 128, 512:640].astype(bf16) for rb in range(4)]

        gp = {}
        rp = {}
        dp = {}
        dr = {rb: h[128 * rb:128 * rb + 128, 512:640] for rb in range(4)}
        act = {}
        dl = {}

        def G(c, k):
            def step(k2):
                r0, c1 = 256 * k + 128 * (k2 // 4), c * FC + 128 * (k2 % 4)
                for w in range(2):
                    gp[c, w, k, k2] = _nn(L[k][k2], wgu_v[2 + w, r0:r0 + 128, c1:c1 + 128])
            return [(lambda k2=k2: step(k2)) for k2 in (2, 4, 1, 3, 0, 6, 5)]

        def Rr(c):
            def step(rb, b, w):
                rp[c, w, rb, b] = _nn(hr_[rb],
                                      wgu_v[w, 512:640, c * FC + 256 * b:c * FC + 256 * b + 256])
            return [(lambda rb=rb, b=b, w=w: step(rb, b, w)) for rb in range(4) for b in (1, 0) for w in range(2)]

        def M(c, w, k):
            t = comb([gp[c, w, k, k2] for k2 in range(7)])
            return jnp.concatenate([jnp.concatenate(r_, axis=1) for r_ in t], axis=0)

        def quad(c, a, b):
            gu_ = []
            for w in range(2):
                rfull = jnp.concatenate([rp[c, w, rb, b] for rb in range(4)], axis=0)
                t = jnp.concatenate([quarter(rfull, 2 * a), quarter(rfull, 2 * a + 1)], axis=0)
                for sg, k in {(0, 1): ((1, 2), (1, 4)), (1, 0): ((1, 1), (1, 3)),
                              (0, 0): ((1, 3), (-1, 4), (1, 0), (1, 6)),
                              (1, 1): ((1, 2), (-1, 1), (1, 0), (1, 5))}[a, b]:
                    t = t + mm_[c, w, k] if sg > 0 else t - mm_[c, w, k]
                gu_.append(t)
            act[c, a, b] = _gelu_mul(*gu_)

        mm_ = {}

        def fin(c, *ks):
            for k in ks:
                for w in range(2):
                    mm_[c, w, k] = M(c, w, k)

        def dlhs(c, k, rh):
            if (c, k, rh) not in dl:
                a = lambda x, y: act[c, x, y][128 * rh:128 * rh + 128]
                dl[c, k, rh] = [lambda: a(0, 0) + a(1, 1), lambda: a(1, 0) + a(1, 1), lambda: a(0, 0), lambda: a(1, 1),
                                lambda: a(0, 0) + a(0, 1), lambda: a(1, 0) - a(0, 0),
                                lambda: a(0, 1) - a(1, 1)][k]().astype(bf16)
            return dl[c, k, rh]

        def drhs(c, k):
            if k == 1:
                return wd2.at[0, pl.ds(c * FC, 256), pl.ds(0, 256)]
            if k == 4:
                return wd2.at[0, pl.ds(c * FC + 256, 256), pl.ds(256, 256)]
            r1, c1 = dn_place(c)((0, None, 1, 2, None, 3, 4)[k])
            return wd2.at[1, pl.ds(r1, 256), pl.ds(c1, 256)]

        def Dk(c, k):
            def step(rh, ch):
                t = _nn(dlhs(c, k, rh), drhs(c, k)[:, 128 * ch:128 * ch + 128])
                ix = 4 * k + 2 * rh + ch
                if c == 0:
                    dacc[ix] = t
                elif c < nc - 1:
                    dacc[ix] = dacc[ix] + t
                else:
                    dp[k, rh, ch] = dacc[ix] + t
            return [(lambda rh=rh, ch=ch: step(rh, ch)) for rh in range(2) for ch in range(2)]

        def a_nat(c):
            return [jnp.concatenate([act[c, q // 2, b][128 * (q % 2):128 * (q % 2) + 128] for b in range(2)], axis=1)
                    for q in range(4)]

        def Dr(c):
            def step(rb):
                dr[rb] = dr[rb] + _nn(natural(a_nat(c), 2 * rb, 2 * rb + 2).astype(bf16),
                                      wd2[0, c * FC:(c + 1) * FC, 512:640])
            return [(lambda rb=rb: step(rb)) for rb in range(4)]

        def out_block(r0, n, c0, w, val):
            rr0 = pl.multiple_of(i * T2 + r0, 16)
            out_v[pl.ds(rr0, n), c0:c0 + w] = val.astype(bf16)
            cp(out_v.at[pl.ds(rr0, n), pl.ds(c0, w)], out_hbm.at[0, pl.ds(rr0, n), pl.ds(c0, w)], 0).start()

        def dm(k, rh):
            return jnp.concatenate([dp[k, rh, 0], dp[k, rh, 1]], axis=1)

        run(Rr(0))
        run(G(0, 2))
        for c in range(nc):
            fin(c, 2)
            if c == 0:
                run(G(c, 4), G(c, 1))
                fin(c, 4, 1)
                quad(c, 0, 1)
                run(G(c, 3), G(c, 0))
                fin(c, 3, 0)
                quad(c, 1, 0)
                run(G(c, 6), G(c + 1, 2))
                fin(c, 6)
                quad(c, 0, 0)
                rn_ = Rr(c + 1)
                run(G(c, 5), rn_[:7])
                fin(c, 5)
                quad(c, 1, 1)
                run(rn_[7:])
                continue
            dd = sum([Dk(c - 1, k) for k in (2, 4, 5, 0, 1, 3, 6)], [])
            run(G(c, 4), dd[0:7])
            fin(c, 4)
            quad(c, 0, 1)
            run(G(c, 1))
            run(Dr(c - 1)[:2])
            run(G(c, 3), dd[7:14])
            fin(c, 1, 3)
            quad(c, 1, 0)
            run(G(c, 0))
            run(Dr(c - 1)[2:])
            run(G(c, 6), dd[14:21])
            fin(c, 0, 6)
            quad(c, 0, 0)
            if c + 1 < nc:
                run(G(c + 1, 2))
                run(G(c, 5), dd[21:28])
                fin(c, 5)
                quad(c, 1, 1)
                run(Rr(c + 1))
            else:
                run(G(c, 5), dd[21:28])
                fin(c, 5)
                quad(c, 1, 1)
                run(Dk(c, 2) + Dk(c, 4) + Dk(c, 5) + Dk(c, 0) + Dk(c, 1))
                qs = [dm(2, 0) + dm(4, 0), dm(2, 1) + dm(4, 1),
                      dm(2, 0) - dm(1, 0) + dm(0, 0) + dm(5, 0), dm(2, 1) - dm(1, 1) + dm(0, 1) + dm(5, 1)]
                out_block(0, T2, 256, 256, h[:, 256:512] + natural(qs, 0, NS))
                if TAIL == 0:
                    run(Dk(c, 3) + Dk(c, 6))
                    part = [dm(3, 0) - dm(4, 0) + dm(0, 0) + dm(6, 0), dm(3, 1) - dm(4, 1) + dm(0, 1) + dm(6, 1),
                            dm(1, 0) + dm(3, 0), dm(1, 1) + dm(3, 1)]
                    out_block(0, T2, 0, 256, h[:, 0:256] + natural(part, 0, NS))
                    drf = jnp.concatenate([dr[rb] for rb in range(4)], axis=0)
                    an = natural(a_nat(c), 0, NS)
                    for lo, n in RP:
                        out_block(lo, n, 512, 128, drf[lo:lo + n] + _nn(an[lo:lo + n].astype(bf16), wd2[0, c * FC:(c + 1) * FC, 512:640]))
                else:
                    d3, d6 = Dk(c, 3), Dk(c, 6)
                    for ch in range(2):
                        run([d3[ch], d3[2 + ch], d6[ch], d6[2 + ch]])
                        g_ = lambda k, rh: dp[k, rh, ch]
                        part = [g_(3, 0) - g_(4, 0) + g_(0, 0) + g_(6, 0), g_(3, 1) - g_(4, 1) + g_(0, 1) + g_(6, 1),
                                g_(1, 0) + g_(3, 0), g_(1, 1) + g_(3, 1)]
                        out_block(0, T2, 128 * ch, 128, h[:, 128 * ch:128 * ch + 128] + natural(part, 0, NS))
                    drf = jnp.concatenate([dr[rb] for rb in range(4)], axis=0)
                    an = natural(a_nat(c), 0, NS)
                    for lo, n in RP:
                        out_block(lo, n, 512, 128, drf[lo:lo + n] + _nn(an[lo:lo + n].astype(bf16), wd2[0, c * FC:(c + 1) * FC, 512:640]))
        return carry

    lax.fori_loop(0, N2, p2, 0)
    cp(out_v, out_hbm.at[0], 0).wait()


def _kernel(*refs):
    @pl.when(pl.program_id(0) == 0)
    def _():
        _body(*refs)


@jax.jit
def pallas_sequential_preLN__linear_kernel_hedgehog__geglu_ffn__prompt_kernel(
    A_x: jax.Array,
    A_wqkv: jax.Array,
    A_w_phi: jax.Array,
    A_wo: jax.Array,
    B_x: jax.Array,
    B_w_gate: jax.Array,
    B_w_up: jax.Array,
    B_w_down: jax.Array,
):
    del B_x
    anyspec = pl.BlockSpec(memory_space=pl.ANY)
    wphi_t = jnp.transpose(A_w_phi, (1, 2, 0))
    return pl.pallas_call(
        _kernel,
        out_shape=jax.ShapeDtypeStruct((1, S, D), bf16),
        grid=(2,),
        in_specs=[anyspec] * 7,
        out_specs=anyspec,
        scratch_shapes=[
            pltpu.VMEM((S, D), bf16),
            pltpu.VMEM((D, D), bf16),
            pltpu.VMEM((D, D), bf16),
            pltpu.VMEM((D, D), bf16),
            pltpu.VMEM((DH, DH, H), bf16),
            pltpu.VMEM((D, D), bf16),
            pltpu.VMEM((4, 1792, F), bf16),
            pltpu.VMEM((2, 2048, D), bf16),
            pltpu.VMEM((928, D), u32),
            pltpu.VMEM((32, D), f32),
            pltpu.VMEM((P1 // 2, D), u32),
            pltpu.VMEM((T1 // 2, D), u32),
            pltpu.VMEM((11, 64, S), u32),
            pltpu.VMEM((11, 64, S), u32),
            pltpu.VMEM((11, 32, S), u32),
            pltpu.VMEM((11, 32, 128), u32),
            pltpu.VMEM((28, 128, 128), f32),
            pltpu.VMEM((S, D), bf16),
            pltpu.SemaphoreType.DMA((4,)),
        ],
        compiler_params=pltpu.CompilerParams(
            dimension_semantics=("arbitrary",),
            vmem_limit_bytes=100 * 1024 * 1024,
            disable_bounds_checks=True,
            disable_semaphore_checks=True,
        ),
        name="hh",
    )(A_x, A_wqkv, wphi_t, A_wo, B_w_gate, B_w_up, B_w_down)
```

```python
import jax
import jax.numpy as jnp
from jax import lax
from jax.experimental import pallas as pl
from jax.experimental.pallas import tpu as pltpu

S, D, H, DH, F = 2048, 640, 32, 20, 1536
LOG2E = 1.4426950408889634
NT_DIMS = (((1,), (1,)), ((), ()))
f32 = jnp.float32
bf16 = jnp.bfloat16
u32 = jnp.uint32

NP = 5
R = 5
T1 = 128 * R
P1 = 128 * NP
N1 = (S - P1 - 128) // T1
T2 = 512
N2 = S // T2
NS = T2 // 64
NW = 256
LNC = 64
FC = 512
NC = F // FC
K_OFF, Q_OFF, V_OFF = 0, 304, 608
LAST_PIECES = ((0, 128), (128, 128), (256, 128), (384, 64), (448, 32), (480, 32))
assert P1 + N1 * T1 + 128 == S and N1 == 2 and NC == 3


def _ln(x):
    m = jnp.mean(x, axis=-1, keepdims=True)
    xc = x - m
    v = jnp.mean(xc * xc, axis=-1, keepdims=True) + 1e-5
    return xc * jnp.exp2(jnp.log(v) * (-0.5 * LOG2E))


def _rcp(x):
    return pl.reciprocal(x, approx=True)


def _allred(m, op):
    m = op(m, pltpu.roll(m, 2, 0))
    return op(m, pltpu.roll(m, 4, 0))


def _tree(op, xs):
    return op(op(op(xs[0], xs[1]), op(xs[2], xs[3])), xs[4])


def _pk(v):
    return pltpu.bitcast(v, u32)


def _pe(a, b):
    return pltpu.pack_elementwise([a, b], packed_dtype=bf16)


def _up(v):
    return pltpu.bitcast(v, bf16)


def _feat5(ps):
    mx = _allred(_tree(jnp.maximum, ps), jnp.maximum)
    mn = _allred(_tree(jnp.minimum, ps), jnp.minimum)
    ep = [jnp.exp2(q - mx) for q in ps]
    en = [jnp.exp2(mn - q) for q in ps]
    rp = _rcp(_allred(_tree(jnp.add, ep), jnp.add))
    rn = _rcp(_allred(_tree(jnp.add, en), jnp.add))
    return [_pe(a * rp, b * rn) for a, b in zip(ep, en)]


def _gelu_mul(g, u):
    c = 0.7978845608028654
    t = jnp.tanh(g * (c + (c * 0.044715) * (g * g)))
    hgu = (0.5 * g) * u
    return hgu + hgu * t


def _nt(a, b):
    return lax.dot_general(a, b, NT_DIMS, preferred_element_type=f32)


def _nn(a, b):
    return jnp.dot(a, b, preferred_element_type=f32)


def _pair_is(a, w):
    return (lax.broadcasted_iota(jnp.int32, (8, w), 0) >> 1) == a


def _lhs7(a11, a12, a21, a22):
    return [a11 + a22, a21 + a22, a11, a22, a11 + a12, a21 - a11, a12 - a22]


def _rhs7(b11, b12, b21, b22):
    return [b11 + b22, b11, b12 - b22, b21 - b11, b22, b11 + b12, b21 + b22]


def _comb(q):
    return [[q[3] - q[4] + q[0] + q[6], q[2] + q[4]], [q[1] + q[3], q[2] - q[1] + q[0] + q[5]]]


_RHS_BLOCKS = ((0, 3), (0,), (1, 3), (2, 0), (3,), (0, 1), (2, 3))
_RHS_SIGN = (1, 0, -1, -1, 0, 1, 1)
_QUAD_TERMS = {(0, 1): ((1, 2), (1, 4)), (1, 0): ((1, 1), (1, 3)),
               (0, 0): ((1, 3), (-1, 4), (1, 0), (1, 6)), (1, 1): ((1, 2), (-1, 1), (1, 0), (1, 5))}


def _quarter(x, q):
    return jnp.concatenate([x[64 * s + 16 * q:64 * s + 16 * q + 16] for s in range(NS)], axis=0)


def _natural(qs, s0, s1):
    return jnp.concatenate([qs[q][16 * s:16 * s + 16] for s in range(s0, s1) for q in range(4)], axis=0)


def _run(*streams):
    streams = [list(t) for t in streams]
    while any(streams):
        for t in streams:
            if t:
                t.pop(0)()


def _body(x_hbm, wqkv_hbm, wphi_hbm, wo_hbm, wg_hbm, wu_hbm, wd_hbm, out_hbm,
          x_v, wq_v, wk_v, wv_v, wphi_v, wo_v, wgu, wd2, wT, bcat,
          xn0, xn_buf, phiq, phik, vaug, kvm, dacc, out_v, sem):
    def cp(src, dst, k):
        return pltpu.make_async_copy(src, dst, sem.at[k])

    def xrows(r0, r1, k):
        return cp(x_hbm.at[0, pl.ds(r0, r1 - r0)], x_v.at[pl.ds(r0, r1 - r0)], k)

    def wk_cols(c0, n, k):
        return cp(wqkv_hbm.at[:, pl.ds(D + c0, n)], wk_v.at[:, pl.ds(c0, n)], k)

    g_phi = [cp(wphi_hbm, wphi_v, 0)]
    g_x0 = [xrows(0, 256, 1)]
    g_ka = [wk_cols(0, 256, 2)]
    g_kb = [wk_cols(256, 256, 3)]
    g_kc = [wk_cols(512, 128, 0), xrows(256, P1, 0)]
    g_qv = [cp(wqkv_hbm.at[:, pl.ds(0, D)], wq_v, 1), cp(wqkv_hbm.at[:, pl.ds(2 * D, D)], wv_v, 1),
            xrows(P1, P1 + 128, 1)]
    g_xr = [xrows(P1 + 128, S, 2), cp(wg_hbm, wgu.at[0, pl.ds(0, D)], 2)]
    g_w = [cp(wu_hbm, wgu.at[1, pl.ds(0, D)], 3), cp(wd_hbm, wd2.at[0, pl.ds(0, F)], 3), cp(wo_hbm, wo_v, 3)]

    def waits(cs, starts=()):
        for c in cs:
            c.wait()
        for c in starts:
            c.start()

    for c in g_phi + g_x0 + g_ka + g_kb:
        c.start()

    def ln_rows(r0, n, dst, d0):
        for c in range(0, n, LNC):
            xn = _ln(x_v[pl.ds(r0 + c, LNC), :].astype(f32)).astype(bf16)
            dst[(d0 + c) // 2:(d0 + c + LNC) // 2, :] = _pk(xn)

    pending = []

    def drain(keep=0):
        while len(pending) > keep:
            pending.pop(0)()

    def phi_store(dst, g, x, c0):
        T, role = divmod(g, 3)
        cols = pl.ds(c0, 128)
        if role == 0:
            dst[2 * T, 0:40, cols] = jnp.concatenate(x, axis=0)
        elif role == 2:
            dst[2 * T + 1, 24:64, cols] = jnp.concatenate(x, axis=0)
        else:
            even = (lax.broadcasted_iota(jnp.int32, (8, 128), 0) & 1) == 0
            ev = [jnp.where(even, x[a], pltpu.roll(x[a + 1], 1, 0)) for a in (0, 2)]
            od = [jnp.where(even, pltpu.roll(x[a], 7, 0), x[a + 1]) for a in (0, 2)]
            dst[2 * T, 40:64, cols] = jnp.concatenate(ev + [x[4]], axis=0)
            dst[2 * T + 1, 0:24, cols] = jnp.concatenate(od + [x[4]], axis=0)

    def feat_block(p, dst, b, c0, rfirst=True):
        ro, mo = (0, 24) if rfirst else (128, 0)
        rs = [p[ro + 8 * a:ro + 8 + 8 * a] for a in range(3)]
        for a in range(4):
            if a < 3:
                v4 = jnp.where(_pair_is(a, 128), 0.0, rs[a])
            else:
                v4 = jnp.where(_pair_is(0, 128), rs[0],
                               jnp.where(_pair_is(1, 128), rs[1], jnp.where(_pair_is(2, 128), rs[2], 0.0)))
            ps = [p[mo + 32 * a + 8 * v:mo + 8 + 32 * a + 8 * v] for v in range(4)] + [v4]
            phi_store(dst, 4 * b + a, _feat5(ps), c0)

    def xs(xref, xr0):
        return _up(xref[xr0 // 2:xr0 // 2 + 64, :])

    def proj_qk(off, dst, B, xref, xr0, c0):
        p = _nt(_up(wT[off + 152 * B:off + 152 * B + 152, :]), xs(xref, xr0))

        def post():
            feat_block(p[0:152], dst, 2 * B, c0)
            feat_block(p[152:304], dst, 2 * B + 1, c0)
        pending.append(post)

    def proj_k4(wb, b, j, rfirst):
        p = _nt(wb, xs(xn0, 128 * j))
        pending.append(lambda: feat_block(p[0:152], phik, b, 128 * j, rfirst))

    def proj_v(xref, xr0, c0, split_last=False):
        cuts = [0, 80, 160, 240, 280, 320] if split_last else [0, 80, 160, 240, 320]
        p = jnp.concatenate([_nt(_up(wT[V_OFF + a:V_OFF + b, :]), xs(xref, xr0))
                             for a, b in zip(cuts[:-1], cuts[1:])], axis=0)
        low = lax.broadcasted_iota(jnp.int32, (8, 128), 0) < 4
        cols = pl.ds(c0, 128)
        sl = [p[8 * a:8 * a + 8] for a in range(80)]

        def put(t, slabs):
            vaug[t, 0:4 * len(slabs), cols] = jnp.concatenate(
                [_pe(slabs[a], slabs[a + 1]) for a in range(0, len(slabs), 2)], axis=0)
        for T in range(5):
            mid = sl[15 * T + 7]
            put(2 * T, sl[15 * T:15 * T + 7] + [jnp.where(low, mid, 1.0)])
            put(2 * T + 1, [jnp.where(low, 1.0, mid)] + sl[15 * T + 8:15 * T + 15])
        put(10, sl[75:80] + [jnp.ones((8, 128), f32)])

    pr = lax.broadcasted_iota(jnp.int32, (D, D), 0)
    pc = lax.broadcasted_iota(jnp.int32, (D, D), 1)
    perm = jnp.where((pr & 31) * DH + (pr >> 5) == pc, 1.0, 0.0).astype(bf16)
    r_i = lax.broadcasted_iota(jnp.int32, (160, 32), 0)
    c_i = lax.broadcasted_iota(jnp.int32, (160, 32), 1)
    gl = r_i // 40
    sl_ = (r_i - 40 * gl) >> 1
    q_ = sl_ - 16
    f_ = jnp.where(sl_ < 16, sl_ + 1, jnp.where(q_ == gl, 0, jnp.where(q_ < gl, 17 + q_, 16 + q_)))
    e0 = jnp.where(f_ == c_i, 1.0, 0.0)
    es = []
    for t in range(5):
        off = (120 * t) % 160
        es.append((jnp.concatenate([e0[off:], e0[:off]], axis=0) if off else e0).astype(bf16))
    r2 = lax.broadcasted_iota(jnp.int32, (160, 128), 0)
    hr = 2 * (r2 // 40) + (r2 & 1)
    hc = [(lax.broadcasted_iota(jnp.int32, (1, 128), 1) + 128 * t) // DH - 6 * t for t in range(5)]
    bcat[...] = jnp.zeros(bcat.shape, f32)

    waits(g_phi, g_kc)
    for d in range(DH):
        bcat[0:DH, 32 * d:32 * d + 32] = wphi_v[d].astype(f32)
    at = _nn(bcat[...].astype(bf16), perm).astype(bf16)
    pts = [jnp.where(hr == hc[t], _nn(es[t], at[:, 128 * t:128 * t + 128]), 0.0).astype(bf16) for t in range(5)]

    def fold(w_v, off, t, rs, blk):
        rs[t] = _nt(pts[t], w_v[:, 128 * t:128 * t + 128])
        if t == 0:
            return
        b = t - 1
        lo, hi = rs[t - 1], rs[t]
        parts = []
        if b < 3:
            parts.append(lo[40 * b:120])
        parts.append(lo[120:160] + hi[0:40])
        if b > 0:
            parts.append(hi[40:40 + 40 * b])
        w = jnp.concatenate(parts, axis=0)
        mains, v4s = [], []
        for a in range(4):
            v4 = w[40 * a + 32:40 * a + 40]
            base = _allred(jnp.where(_pair_is(a, D), v4, 0.0), jnp.add)
            mains += [(w[40 * a + 8 * v:40 * a + 8 * v + 8] - base) * LOG2E for v in range(4)]
            v4s.append((v4 - base) * LOG2E)
        shared = [jnp.where(_pair_is(a, D), v4s[3], v4s[a]) for a in range(3)]
        blk[b] = (shared, mains)
        if b % 2 == 1:
            B = b // 2
            rows = blk[b - 1][0] + blk[b - 1][1] + blk[b][0] + blk[b][1]
            wT[off + 152 * B:off + 152 * B + 152, :] = _pk(jnp.concatenate(rows, axis=0).astype(bf16))

    def blk16(slabs, rfirst):
        rows = slabs[0] + slabs[1] if rfirst else slabs[1] + slabs[0]
        return jnp.concatenate(rows + [jnp.zeros((8, D), f32)], axis=0).astype(bf16)

    waits(g_x0, g_qv)
    ln_rows(0, 256, xn0, 0)

    rk, rq, bk, bq = {}, {}, {}, {}
    waits(g_ka, g_xr)
    fold(wk_v, K_OFF, 0, rk, bk)
    fold(wk_v, K_OFF, 1, rk, bk)
    w0 = blk16(bk[0], False)
    proj_k4(w0, 0, 0, False)
    proj_k4(w0, 0, 1, False)

    waits(g_kb, g_w)
    fold(wk_v, K_OFF, 2, rk, bk)
    fold(wk_v, K_OFF, 3, rk, bk)
    w1 = blk16(bk[1], False)
    proj_k4(w1, 1, 0, False)
    proj_k4(w1, 1, 1, False)
    w2 = blk16(bk[2], True)
    proj_k4(w2, 2, 0, True)
    drain(1)

    waits(g_kc)
    fold(wk_v, K_OFF, 4, rk, bk)
    proj_k4(w2, 2, 1, True)
    ln_rows(256, P1 - 256, xn0, 256)
    w3 = blk16(bk[3], True)
    proj_k4(w3, 3, 0, True)
    proj_k4(w3, 3, 1, True)
    for j in range(2, NP):
        for B in range(2):
            proj_qk(K_OFF, phik, B, xn0, 128 * j, 128 * j)
    drain(1)

    waits(g_qv)
    for t in range(5):
        fold(wq_v, Q_OFF, t, rq, bq)
    for t in range(5):
        wT[V_OFF + 64 * t:V_OFF + 64 * t + 64, :] = _pk(wv_v[:, 128 * t:128 * t + 128].T)
    ln_rows(P1, 128, xn_buf, 0)
    for j in range(NP):
        for B in range(2):
            proj_qk(Q_OFF, phiq, B, xn0, 128 * j, 128 * j)
    drain()
    for j in range(NP):
        proj_v(xn0, 128 * j, 128 * j, j == NP - 1)

    def dn_place(c, k):
        return 256 * ((5 * c + k) // 2), 256 * ((5 * c + k) % 2)

    def down_tables(src, c):
        for r in range(0, 256, 8):
            b11, b12, b21, b22 = [
                wd2[src, c * FC + 256 * a + r:c * FC + 256 * a + r + 8, 256 * b:256 * b + 256].astype(f32)
                for a in range(2) for b in range(2)]
            for k, t in enumerate([b11 + b22, b12 - b22, b21 - b11, b11 + b12, b21 + b22]):
                r1, c1 = dn_place(c, k)
                wd2[1, r1 + r:r1 + r + 8, c1:c1 + 256] = t.astype(bf16)

    def gu_tables(src, dst, c0):
        for r in range(0, 128, 8):
            for k1 in range(7):
                def ld(q, a):
                    r0 = 256 * (q // 2) + 128 * a + r
                    return wgu[src, r0:r0 + 8, c0 + 256 * (q % 2):c0 + 256 * (q % 2) + 256].astype(f32)
                blocks = [[ld(q, a) for a in range(2)] for q in _RHS_BLOCKS[k1]]
                if _RHS_SIGN[k1] > 0:
                    rows = [blocks[0][a] + blocks[1][a] for a in range(2)]
                elif _RHS_SIGN[k1] < 0:
                    rows = [blocks[0][a] - blocks[1][a] for a in range(2)]
                else:
                    rows = blocks[0]
                ts = _rhs7(rows[0][:, 0:128], rows[0][:, 128:256], rows[1][:, 0:128], rows[1][:, 128:256])
                rd = 256 * k1 + r
                wgu[dst, rd:rd + 8, c0:c0 + 512] = jnp.concatenate(ts[0:4], axis=1).astype(bf16)
                wgu[dst, rd + 128:rd + 136, c0:c0 + 384] = jnp.concatenate(ts[4:7], axis=1).astype(bf16)
                wgu[dst, rd + 128:rd + 136, c0 + 384:c0 + 512] = wgu[src, r:r + 8, c0:c0 + 128]

    def p1(i, carry):
        @pl.when(i == N1 - 1)
        def _():
            waits(g_w)
        for c in range(NC):
            gu_tables(i, jnp.minimum(i, 1) + 2, c * FC)
        for j in range(R):
            c0 = pl.multiple_of(P1 + i * T1 + 128 * j, 128)
            rn = pl.multiple_of(P1 + i * T1 + 128 * (j + 1), 128)
            ln_rows(rn, 128, xn_buf, 128 * ((j + 1) % R))
            for off, dst in ((K_OFF, phik), (Q_OFF, phiq)):
                for B in range(2):
                    proj_qk(off, dst, B, xn_buf, 128 * j, c0)
                    drain()
            proj_v(xn_buf, 128 * j, c0)
        return carry

    waits(g_xr)
    lax.fori_loop(0, N1, p1, 0)

    for c in range(NC):
        down_tables(pl.program_id(0), c)
    proj_v(xn_buf, 0, S - 128)
    for off, dst in ((K_OFF, phik), (Q_OFF, phiq)):
        for B in range(2):
            proj_qk(off, dst, B, xn_buf, 0, S - 128)
    drain()

    rr = lax.broadcasted_iota(jnp.int32, (64, 128), 0)
    cc = lax.broadcasted_iota(jnp.int32, (64, 128), 1)
    par = (cc >> 1) & 1
    col0 = jnp.where(cc < 80, par, jnp.where(cc < 112, 2, 2 + par))
    col1 = jnp.where(cc < 32, 0, jnp.where(cc < 48, par - 1, 1 + par))
    row0 = jnp.where(rr < 60, rr // DH, jnp.minimum(rr - 60, 2))
    row1 = jnp.where(rr < 4, jnp.minimum(rr, 2), (rr - 4) // DH)
    msks = (col0 == row0, col1 == row1)

    def unzip(y):
        u = _pk(y.astype(bf16))
        lo = lax.bitcast_convert_type(u << 16, f32)
        hi = lax.bitcast_convert_type(u & jnp.uint32(0xFFFF0000), f32)
        return jnp.concatenate([t[a:a + 8] for a in range(0, u.shape[0], 8) for t in (lo, hi)], axis=0)

    for t in range(10):
        kvm[t] = _pk(jnp.where(msks[t % 2], unzip(_nt(_up(vaug[t]), _up(phik[t]))), 0.0).astype(bf16))
    rl = lax.broadcasted_iota(jnp.int32, (48, 80), 0)
    cl = lax.broadcasted_iota(jnp.int32, (48, 80), 1)
    rowl = jnp.where(rl < 40, (rl >= 20).astype(jnp.int32), (rl >= 44).astype(jnp.int32))
    kvl = unzip(_nt(_up(vaug[10, 0:24, :]), _up(phik[10, 0:40, :])))
    kvm[10, 0:24, 0:80] = _pk(jnp.where(((cl >> 1) & 1) == rowl, kvl, 0.0).astype(bf16))

    def attn_o(c0):
        low = lax.broadcasted_iota(jnp.int32, (8, NW), 0) < 4
        cols = pl.ds(c0, NW)

        def bc(r, k):
            return jnp.broadcast_to(r[k:k + 1], (8, NW))
        os = []
        for T in range(5):
            n0 = _nn(_up(kvm[2 * T]), _up(phiq[2 * T, :, cols]))
            n1 = _nn(_up(kvm[2 * T + 1]), _up(phiq[2 * T + 1, :, cols]))
            r0 = _rcp(n0[56:64] + 1e-6)
            r1 = _rcp(n1[0:8] + 1e-6)
            a, b, c = bc(r0, 4), bc(r0, 5), bc(r0, 6)
            d, e, f = bc(r1, 0), bc(r1, 1), bc(r1, 2)
            os += [n0[0:8] * a, n0[8:16] * a, n0[16:24] * jnp.where(low, a, b), n0[24:32] * b, n0[32:40] * b,
                   n0[40:48] * c, n0[48:56] * c, jnp.where(low, n0[56:64] * c, n1[0:8] * d),
                   n1[8:16] * d, n1[16:24] * d, n1[24:32] * e, n1[32:40] * e, n1[40:48] * jnp.where(low, e, f),
                   n1[48:56] * f, n1[56:64] * f]
        nd = _nn(_up(kvm[10, 0:24, 0:80]), _up(phiq[10, 0:40, cols]))
        r = _rcp(nd[40:48] + 1e-6)
        rrot = pltpu.roll(r, 4, 0)
        ra = jnp.where(low, r, rrot)
        rb = jnp.where(low, rrot, r)
        os += [nd[0:8] * ra, nd[8:16] * ra, nd[16:24] * r, nd[24:32] * rb, nd[32:40] * rb]
        return jnp.concatenate(os, axis=0).astype(bf16).T

    def p2(i, carry):
        o = jnp.concatenate([attn_o(pl.multiple_of(i * T2 + w, NW)) for w in range(0, T2, NW)], axis=0)
        hs, hns = [], []
        for w in range(0, T2, 64):
            r0 = pl.multiple_of(i * T2 + w, 64)
            hw = x_v[pl.ds(r0, 64), :].astype(f32) + _nn(o[w:w + 64], wo_v[...])
            hs.append(hw)
            hns.append(_ln(hw))
        h = jnp.concatenate(hs, axis=0)
        hn = jnp.concatenate(hns, axis=0)
        hq = [_quarter(hn[:, 0:512], q) for q in range(4)]
        top = jnp.concatenate(hq[0:2], axis=0)
        bot = jnp.concatenate(hq[2:4], axis=0)
        L = [[t.astype(bf16) for t in _lhs7(t1[:128, :128], t1[:128, 128:], t1[128:, :128], t1[128:, 128:])]
             for t1 in _lhs7(top[:, 0:256], top[:, 256:512], bot[:, 0:256], bot[:, 256:512])]
        hrest = [hn[128 * rb:128 * rb + 128, 512:640].astype(bf16) for rb in range(4)]

        gp = {}
        gm = {}
        rp = {}
        act = {}
        dl = {}
        dp = {}
        dr = {rb: h[128 * rb:128 * rb + 128, 512:640] for rb in range(4)}

        def G(c, k):
            def step(k2):
                r0, c1 = 256 * k + 128 * (k2 // 4), c * FC + 128 * (k2 % 4)
                for w in range(2):
                    gp[c, w, k, k2] = _nn(L[k][k2], wgu[2 + w, r0:r0 + 128, c1:c1 + 128])
            return [(lambda k2=k2: step(k2)) for k2 in (2, 4, 1, 3, 0, 6, 5)]

        def Rr(c):
            def step(rb, b, w):
                rp[c, w, rb, b] = _nn(hrest[rb], wgu[w, 512:640, c * FC + 256 * b:c * FC + 256 * b + 256])
            return [(lambda rb=rb, b=b, w=w: step(rb, b, w)) for rb in range(4) for b in (1, 0) for w in range(2)]

        def fin(c, *ks):
            for k in ks:
                for w in range(2):
                    t = _comb([gp[c, w, k, k2] for k2 in range(7)])
                    gm[c, w, k] = jnp.concatenate([jnp.concatenate(r_, axis=1) for r_ in t], axis=0)

        def quad(c, a, b):
            gu = []
            for w in range(2):
                full = jnp.concatenate([rp[c, w, rb, b] for rb in range(4)], axis=0)
                t = jnp.concatenate([_quarter(full, 2 * a), _quarter(full, 2 * a + 1)], axis=0)
                for sg, k in _QUAD_TERMS[a, b]:
                    t = t + gm[c, w, k] if sg > 0 else t - gm[c, w, k]
                gu.append(t)
            act[c, a, b] = _gelu_mul(*gu)

        def dlhs(c, k, rh):
            if (c, k, rh) not in dl:
                def a(x, y):
                    return act[c, x, y][128 * rh:128 * rh + 128]
                dl[c, k, rh] = [lambda: a(0, 0) + a(1, 1), lambda: a(1, 0) + a(1, 1), lambda: a(0, 0),
                                lambda: a(1, 1), lambda: a(0, 0) + a(0, 1), lambda: a(1, 0) - a(0, 0),
                                lambda: a(0, 1) - a(1, 1)][k]().astype(bf16)
            return dl[c, k, rh]

        def drhs(c, k, ch):
            if k == 1:
                n, r1, c1 = 0, c * FC, 0
            elif k == 4:
                n, r1, c1 = 0, c * FC + 256, 256
            else:
                n, (r1, c1) = 1, dn_place(c, (0, None, 1, 2, None, 3, 4)[k])
            return wd2[n, r1:r1 + 256, c1 + 128 * ch:c1 + 128 * ch + 128]

        def Dk(c, k):
            def step(rh, ch):
                t = _nn(dlhs(c, k, rh), drhs(c, k, ch))
                ix = 4 * k + 2 * rh + ch
                if c == 0:
                    dacc[ix] = t
                elif c < NC - 1:
                    dacc[ix] = dacc[ix] + t
                else:
                    dp[k, rh, ch] = dacc[ix] + t
            return [(lambda rh=rh, ch=ch: step(rh, ch)) for rh in range(2) for ch in range(2)]

        def act_rows(c):
            return [jnp.concatenate([act[c, q // 2, b][128 * (q % 2):128 * (q % 2) + 128] for b in range(2)], axis=1)
                    for q in range(4)]

        def Dr(c):
            def step(rb):
                dr[rb] = dr[rb] + _nn(_natural(act_rows(c), 2 * rb, 2 * rb + 2).astype(bf16),
                                      wd2[0, c * FC:(c + 1) * FC, 512:640])
            return [(lambda rb=rb: step(rb)) for rb in range(4)]

        def out_block(r0, n, c0, val):
            rr0 = pl.multiple_of(i * T2 + r0, 16)
            out_v[pl.ds(rr0, n), c0:c0 + 128] = val.astype(bf16)
            cp(out_v.at[pl.ds(rr0, n), pl.ds(c0, 128)], out_hbm.at[0, pl.ds(rr0, n), pl.ds(c0, 128)], 0).start()

        def all_d(c):
            return sum([Dk(c, k) for k in (2, 4, 5, 0, 1, 3, 6)], [])

        r1s, r2s = Rr(1), Rr(2)
        _run(Rr(0))
        _run(G(0, 2))
        for c in range(NC):
            if c == 0:
                mates = [r1s[:7], r1s[7:14], G(1, 2), None]
                gaps = [[], [], r1s[14:]]
            elif c == 1:
                dd = all_d(0)[7:] + r2s[:7]
                mates = [dd[0:7], dd[7:14], dd[14:21], dd[21:28]]
                gaps = [Dr(0)[:2], Dr(0)[2:], G(2, 2)]
            else:
                dd = all_d(1)
                mates = [dd[0:7], dd[7:14], dd[14:21], dd[21:28]]
                gaps = [Dr(1)[:2], Dr(1)[2:], []]
            fin(c, 2)
            _run(G(c, 4), mates[0])
            fin(c, 4)
            quad(c, 0, 1)
            _run(G(c, 1))
            _run(gaps[0])
            _run(G(c, 3), mates[1])
            fin(c, 1, 3)
            quad(c, 1, 0)
            _run(G(c, 0))
            _run(gaps[1])
            _run(G(c, 6), mates[2])
            fin(c, 0, 6)
            quad(c, 0, 0)
            _run(gaps[2])
            _run(G(c, 5), mates[3] if c else all_d(0)[:7])
            fin(c, 5)
            quad(c, 1, 1)
            if c == 1:
                _run(r2s[7:])

        c = NC - 1
        _run(Dk(c, 2) + Dk(c, 4) + Dk(c, 5))
        da, db = {1: Dk(c, 0), 0: Dk(c, 3)}, {1: Dk(c, 1), 0: Dk(c, 6)}
        for blk in (1, 0):
            for ch in range(2):
                _run([da[blk][ch], da[blk][2 + ch], db[blk][ch], db[blk][2 + ch]])

                def g_(k, rh):
                    return dp[k, rh, ch]
                if blk == 1:
                    part = [g_(2, 0) + g_(4, 0), g_(2, 1) + g_(4, 1),
                            g_(2, 0) + g_(5, 0) + g_(0, 0) - g_(1, 0), g_(2, 1) + g_(5, 1) + g_(0, 1) - g_(1, 1)]
                else:
                    part = [g_(0, 0) - g_(4, 0) + g_(3, 0) + g_(6, 0), g_(0, 1) - g_(4, 1) + g_(3, 1) + g_(6, 1),
                            g_(1, 0) + g_(3, 0), g_(1, 1) + g_(3, 1)]
                c0 = 256 * blk + 128 * ch
                out_block(0, T2, c0, h[:, c0:c0 + 128] + _natural(part, 0, NS))
        drf = jnp.concatenate([dr[rb] for rb in range(4)], axis=0)
        an = _natural(act_rows(c), 0, NS)
        for lo, n in LAST_PIECES:
            out_block(lo, n, 512,
                      drf[lo:lo + n] + _nn(an[lo:lo + n].astype(bf16), wd2[0, c * FC:(c + 1) * FC, 512:640]))
        return carry

    lax.fori_loop(0, N2, p2, 0)
    cp(out_v, out_hbm.at[0], 0).wait()


def _kernel(*refs):
    @pl.when(pl.program_id(0) == 0)
    def _():
        _body(*refs)


@jax.jit
def pallas_sequential_preLN__linear_kernel_hedgehog__geglu_ffn__prompt_kernel(
    A_x: jax.Array,
    A_wqkv: jax.Array,
    A_w_phi: jax.Array,
    A_wo: jax.Array,
    B_x: jax.Array,
    B_w_gate: jax.Array,
    B_w_up: jax.Array,
    B_w_down: jax.Array,
):
    del B_x
    anyspec = pl.BlockSpec(memory_space=pl.ANY)
    wphi_t = jnp.transpose(A_w_phi, (1, 2, 0))
    return pl.pallas_call(
        _kernel,
        out_shape=jax.ShapeDtypeStruct((1, S, D), bf16),
        grid=(2,),
        in_specs=[anyspec] * 7,
        out_specs=anyspec,
        scratch_shapes=[
            pltpu.VMEM((S, D), bf16),
            pltpu.VMEM((D, D), bf16),
            pltpu.VMEM((D, D), bf16),
            pltpu.VMEM((D, D), bf16),
            pltpu.VMEM((DH, DH, H), bf16),
            pltpu.VMEM((D, D), bf16),
            pltpu.VMEM((4, 1792, F), bf16),
            pltpu.VMEM((2, 2048, D), bf16),
            pltpu.VMEM((928, D), u32),
            pltpu.VMEM((32, D), f32),
            pltpu.VMEM((P1 // 2, D), u32),
            pltpu.VMEM((T1 // 2, D), u32),
            pltpu.VMEM((11, 64, S), u32),
            pltpu.VMEM((11, 64, S), u32),
            pltpu.VMEM((11, 32, S), u32),
            pltpu.VMEM((11, 32, 128), u32),
            pltpu.VMEM((28, 128, 128), f32),
            pltpu.VMEM((S, D), bf16),
            pltpu.SemaphoreType.DMA((4,)),
        ],
        compiler_params=pltpu.CompilerParams(
            dimension_semantics=("arbitrary",),
            vmem_limit_bytes=100 * 1024 * 1024,
            disable_bounds_checks=True,
            disable_semaphore_checks=True,
        ),
        name="hh",
    )(A_x, A_wqkv, wphi_t, A_wo, B_w_gate, B_w_up, B_w_down)
```

```python
import jax
import jax.numpy as jnp
from jax import lax
from jax.experimental import pallas as pl
from jax.experimental.pallas import tpu as pltpu

S, D, H, DH, F = 2048, 640, 32, 20, 1536
LOG2E = 1.4426950408889634
NT_DIMS = (((1,), (1,)), ((), ()))
f32 = jnp.float32
bf16 = jnp.bfloat16
u32 = jnp.uint32

NP = 6
R = 5
T1 = 128 * R
P1 = 128 * NP
N1 = (S - P1) // T1
T2 = 512
N2 = S // T2
NS = T2 // 64
NW = 256
LNC = 64
FC = 512
NC = F // FC
K_OFF, Q_OFF, V_OFF = 0, 304, 608
LAST_PIECES = ((0, 128), (128, 128), (256, 128), (384, 64), (448, 32), (480, 32))
assert P1 + N1 * T1 == S and N1 == 2 and NC == 3


def _ln(x):
    m = jnp.mean(x, axis=-1, keepdims=True)
    xc = x - m
    v = jnp.mean(xc * xc, axis=-1, keepdims=True) + 1e-5
    return xc * jnp.exp2(jnp.log(v) * (-0.5 * LOG2E))


def _rcp(x):
    return pl.reciprocal(x, approx=True)


def _allred(m, op):
    m = op(m, pltpu.roll(m, 2, 0))
    return op(m, pltpu.roll(m, 4, 0))


def _tree(op, xs):
    return op(op(op(xs[0], xs[1]), op(xs[2], xs[3])), xs[4])


def _pk(v):
    return pltpu.bitcast(v, u32)


def _pe(a, b):
    return pltpu.pack_elementwise([a, b], packed_dtype=bf16)


def _up(v):
    return pltpu.bitcast(v, bf16)


def _feat5(ps):
    mx = _allred(_tree(jnp.maximum, ps), jnp.maximum)
    mn = _allred(_tree(jnp.minimum, ps), jnp.minimum)
    ep = [jnp.exp2(q - mx) for q in ps]
    en = [jnp.exp2(mn - q) for q in ps]
    rp = _rcp(_allred(_tree(jnp.add, ep), jnp.add))
    rn = _rcp(_allred(_tree(jnp.add, en), jnp.add))
    return [_pe(a * rp, b * rn) for a, b in zip(ep, en)]


def _gelu_mul(g, u):
    c = 0.7978845608028654
    t = jnp.tanh(g * (c + (c * 0.044715) * (g * g)))
    hgu = (0.5 * g) * u
    return hgu + hgu * t


def _nt(a, b):
    return lax.dot_general(a, b, NT_DIMS, preferred_element_type=f32)


def _nn(a, b):
    return jnp.dot(a, b, preferred_element_type=f32)


def _pair_is(a, w):
    return (lax.broadcasted_iota(jnp.int32, (8, w), 0) >> 1) == a


def _lhs7(a11, a12, a21, a22):
    return [a11 + a22, a21 + a22, a11, a22, a11 + a12, a21 - a11, a12 - a22]


def _rhs7(b11, b12, b21, b22):
    return [b11 + b22, b11, b12 - b22, b21 - b11, b22, b11 + b12, b21 + b22]


def _comb(q):
    return [[q[3] - q[4] + q[0] + q[6], q[2] + q[4]], [q[1] + q[3], q[2] - q[1] + q[0] + q[5]]]


_RHS_BLOCKS = ((0, 3), (0,), (1, 3), (2, 0), (3,), (0, 1), (2, 3))
_RHS_SIGN = (1, 0, -1, -1, 0, 1, 1)
_QUAD_TERMS = {(0, 1): ((1, 2), (1, 4)), (1, 0): ((1, 1), (1, 3)),
               (0, 0): ((1, 3), (-1, 4), (1, 0), (1, 6)), (1, 1): ((1, 2), (-1, 1), (1, 0), (1, 5))}


def _quarter(x, q):
    return jnp.concatenate([x[64 * s + 16 * q:64 * s + 16 * q + 16] for s in range(NS)], axis=0)


def _natural(qs, s0, s1):
    return jnp.concatenate([qs[q][16 * s:16 * s + 16] for s in range(s0, s1) for q in range(4)], axis=0)


def _run(*streams):
    streams = [list(t) for t in streams]
    while any(streams):
        for t in streams:
            if t:
                t.pop(0)()


def _body(x_hbm, wqkv_hbm, wphi_hbm, wo_hbm, wg_hbm, wu_hbm, wd_hbm, out_hbm,
          x_v, wq_v, wk_v, wv_v, wphi_v, wo_v, wgu, wd2, wT, bcat,
          xn0, xn_buf, phiq, phik, vaug, kvm, dacc, out_v, sem):
    def cp(src, dst, k):
        return pltpu.make_async_copy(src, dst, sem.at[k])

    def xrows(r0, r1, k):
        return cp(x_hbm.at[0, pl.ds(r0, r1 - r0)], x_v.at[pl.ds(r0, r1 - r0)], k)

    def wk_cols(c0, n, k):
        return cp(wqkv_hbm.at[:, pl.ds(D + c0, n)], wk_v.at[:, pl.ds(c0, n)], k)

    g_phi = [cp(wphi_hbm, wphi_v, 0)]
    g_x0 = [xrows(0, 256, 1)]
    g_ka = [wk_cols(0, 256, 2)]
    g_kb = [wk_cols(256, 256, 3)]
    g_kc = [wk_cols(512, 128, 0), xrows(256, P1, 0)]
    g_qv = [cp(wqkv_hbm.at[:, pl.ds(0, D)], wq_v, 1), cp(wqkv_hbm.at[:, pl.ds(2 * D, D)], wv_v, 1),
            xrows(P1, P1 + 128, 1)]
    g_xr = [xrows(P1 + 128, S, 2), cp(wg_hbm, wgu.at[0, pl.ds(0, D)], 2)]
    g_w = [cp(wu_hbm, wgu.at[1, pl.ds(0, D)], 3), cp(wd_hbm, wd2.at[0, pl.ds(0, F)], 3), cp(wo_hbm, wo_v, 3)]

    def waits(cs, starts=()):
        for c in cs:
            c.wait()
        for c in starts:
            c.start()

    for c in g_phi + g_x0 + g_ka + g_kb:
        c.start()

    def ln_rows(r0, n, dst, d0):
        for c in range(0, n, LNC):
            xn = _ln(x_v[pl.ds(r0 + c, LNC), :].astype(f32)).astype(bf16)
            dst[(d0 + c) // 2:(d0 + c + LNC) // 2, :] = _pk(xn)

    pending = []

    def drain(keep=0):
        while len(pending) > keep:
            pending.pop(0)()

    def phi_store(dst, g, x, c0):
        T, role = divmod(g, 3)
        cols = pl.ds(c0, 128)
        if role == 0:
            dst[2 * T, 0:40, cols] = jnp.concatenate(x, axis=0)
        elif role == 2:
            dst[2 * T + 1, 24:64, cols] = jnp.concatenate(x, axis=0)
        else:
            even = (lax.broadcasted_iota(jnp.int32, (8, 128), 0) & 1) == 0
            ev = [jnp.where(even, x[a], pltpu.roll(x[a + 1], 1, 0)) for a in (0, 2)]
            od = [jnp.where(even, pltpu.roll(x[a], 7, 0), x[a + 1]) for a in (0, 2)]
            dst[2 * T, 40:64, cols] = jnp.concatenate(ev + [x[4]], axis=0)
            dst[2 * T + 1, 0:24, cols] = jnp.concatenate(od + [x[4]], axis=0)

    def feat_block(p, dst, b, c0, rfirst=True):
        ro, mo = (0, 24) if rfirst else (128, 0)
        rs = [p[ro + 8 * a:ro + 8 + 8 * a] for a in range(3)]
        for a in range(4):
            if a < 3:
                v4 = jnp.where(_pair_is(a, 128), 0.0, rs[a])
            else:
                v4 = jnp.where(_pair_is(0, 128), rs[0],
                               jnp.where(_pair_is(1, 128), rs[1], jnp.where(_pair_is(2, 128), rs[2], 0.0)))
            ps = [p[mo + 32 * a + 8 * v:mo + 8 + 32 * a + 8 * v] for v in range(4)] + [v4]
            phi_store(dst, 4 * b + a, _feat5(ps), c0)

    def xs(xref, xr0):
        return _up(xref[xr0 // 2:xr0 // 2 + 64, :])

    def proj_qk(off, dst, B, xref, xr0, c0):
        p = _nt(_up(wT[off + 152 * B:off + 152 * B + 152, :]), xs(xref, xr0))

        def post():
            feat_block(p[0:152], dst, 2 * B, c0)
            feat_block(p[152:304], dst, 2 * B + 1, c0)
        pending.append(post)

    def nt2(a, b, split):
        if split:
            return jnp.concatenate([_nt(a[0:80], b), _nt(a[80:160], b)], axis=0)
        return _nt(a, b)

    def proj_k4(wb, b, j, rfirst, split=False):
        p = nt2(wb, xs(xn0, 128 * j), split)
        pending.append(lambda: feat_block(p[0:152], phik, b, 128 * j, rfirst))

    def proj_v(xref, xr0, c0):
        p = jnp.concatenate([_nt(_up(wT[V_OFF + a:V_OFF + a + 80, :]), xs(xref, xr0))
                             for a in range(0, 320, 80)], axis=0)
        low = lax.broadcasted_iota(jnp.int32, (8, 128), 0) < 4
        cols = pl.ds(c0, 128)
        sl = [p[8 * a:8 * a + 8] for a in range(80)]

        def put(t, slabs):
            vaug[t, 0:4 * len(slabs), cols] = jnp.concatenate(
                [_pe(slabs[a], slabs[a + 1]) for a in range(0, len(slabs), 2)], axis=0)
        for T in range(5):
            mid = sl[15 * T + 7]
            put(2 * T, sl[15 * T:15 * T + 7] + [jnp.where(low, mid, 1.0)])
            put(2 * T + 1, [jnp.where(low, 1.0, mid)] + sl[15 * T + 8:15 * T + 15])
        put(10, sl[75:80] + [jnp.ones((8, 128), f32)])

    pr = lax.broadcasted_iota(jnp.int32, (D, D), 0)
    pc = lax.broadcasted_iota(jnp.int32, (D, D), 1)
    perm = jnp.where((pr & 31) * DH + (pr >> 5) == pc, 1.0, 0.0).astype(bf16)
    r_i = lax.broadcasted_iota(jnp.int32, (160, 32), 0)
    c_i = lax.broadcasted_iota(jnp.int32, (160, 32), 1)
    gl = r_i // 40
    sl_ = (r_i - 40 * gl) >> 1
    q_ = sl_ - 16
    f_ = jnp.where(sl_ < 16, sl_ + 1, jnp.where(q_ == gl, 0, jnp.where(q_ < gl, 17 + q_, 16 + q_)))
    e0 = jnp.where(f_ == c_i, 1.0, 0.0)
    es = []
    for t in range(5):
        off = (120 * t) % 160
        es.append((jnp.concatenate([e0[off:], e0[:off]], axis=0) if off else e0).astype(bf16))
    r2 = lax.broadcasted_iota(jnp.int32, (160, 128), 0)
    hr = 2 * (r2 // 40) + (r2 & 1)
    hc = [(lax.broadcasted_iota(jnp.int32, (1, 128), 1) + 128 * t) // DH - 6 * t for t in range(5)]
    bcat[...] = jnp.zeros(bcat.shape, f32)

    waits(g_phi, g_kc)
    for d in range(DH):
        bcat[0:DH, 32 * d:32 * d + 32] = wphi_v[d].astype(f32)
    at = _nn(bcat[...].astype(bf16), perm).astype(bf16)

    def edot(t):
        return jnp.concatenate([_nn(es[t][a:b], at[:, 128 * t:128 * t + 128])
                                for a, b in ((0, 48), (48, 80), (80, 128), (128, 160))], axis=0)
    pts = [jnp.where(hr == hc[t], edot(t), 0.0).astype(bf16) for t in range(5)]

    def fold(w_v, off, t, rs, blk, split=False):
        rs[t] = nt2(pts[t], w_v[:, 128 * t:128 * t + 128], split)
        if t == 0:
            return
        b = t - 1
        lo, hi = rs[t - 1], rs[t]
        parts = []
        if b < 3:
            parts.append(lo[40 * b:120])
        parts.append(lo[120:160] + hi[0:40])
        if b > 0:
            parts.append(hi[40:40 + 40 * b])
        w = jnp.concatenate(parts, axis=0)
        mains, v4s = [], []
        for a in range(4):
            v4 = w[40 * a + 32:40 * a + 40]
            base = _allred(jnp.where(_pair_is(a, D), v4, 0.0), jnp.add)
            mains += [(w[40 * a + 8 * v:40 * a + 8 * v + 8] - base) * LOG2E for v in range(4)]
            v4s.append((v4 - base) * LOG2E)
        shared = [jnp.where(_pair_is(a, D), v4s[3], v4s[a]) for a in range(3)]
        blk[b] = (shared, mains)
        if b % 2 == 1:
            B = b // 2
            rows = blk[b - 1][0] + blk[b - 1][1] + blk[b][0] + blk[b][1]
            wT[off + 152 * B:off + 152 * B + 152, :] = _pk(jnp.concatenate(rows, axis=0).astype(bf16))

    def blk16(slabs, rfirst):
        rows = slabs[0] + slabs[1] if rfirst else slabs[1] + slabs[0]
        return jnp.concatenate(rows + [jnp.zeros((8, D), f32)], axis=0).astype(bf16)

    waits(g_x0, g_qv)
    ln_rows(0, 256, xn0, 0)

    rk, rq, bk, bq = {}, {}, {}, {}
    waits(g_ka, g_xr)
    fold(wk_v, K_OFF, 0, rk, bk)
    fold(wk_v, K_OFF, 1, rk, bk)
    w0 = blk16(bk[0], False)
    proj_k4(w0, 0, 0, False)
    proj_k4(w0, 0, 1, False)

    waits(g_kb, g_w)
    fold(wk_v, K_OFF, 2, rk, bk)
    fold(wk_v, K_OFF, 3, rk, bk)
    w1 = blk16(bk[1], False)
    proj_k4(w1, 1, 0, False)
    proj_k4(w1, 1, 1, False)
    w2 = blk16(bk[2], True)
    proj_k4(w2, 2, 0, True, True)
    proj_k4(w2, 2, 1, True, True)
    drain(1)

    waits(g_kc)
    fold(wk_v, K_OFF, 4, rk, bk, True)
    ln_rows(256, P1 - 256, xn0, 256)
    w3 = blk16(bk[3], False)
    proj_k4(w3, 3, 0, False, True)
    for j in range(2, NP):
        for B in range(2):
            proj_qk(K_OFF, phik, B, xn0, 128 * j, 128 * j)
    drain(1)

    waits(g_qv)
    for t in range(5):
        fold(wq_v, Q_OFF, t, rq, bq, t == 4)
    proj_k4(w3, 3, 1, False, True)
    for t in range(5):
        wT[V_OFF + 64 * t:V_OFF + 64 * t + 64, :] = _pk(wv_v[:, 128 * t:128 * t + 128].T)
    ln_rows(P1, 128, xn_buf, 0)
    for j in range(NP):
        for B in range(2):
            proj_qk(Q_OFF, phiq, B, xn0, 128 * j, 128 * j)
    drain()
    for j in range(NP):
        proj_v(xn0, 128 * j, 128 * j)

    def dn_place(c, k):
        return 256 * ((5 * c + k) // 2), 256 * ((5 * c + k) % 2)

    def down_tables(src, c):
        for r in range(0, 256, 8):
            b11, b12, b21, b22 = [
                wd2[src, c * FC + 256 * a + r:c * FC + 256 * a + r + 8, 256 * b:256 * b + 256].astype(f32)
                for a in range(2) for b in range(2)]
            for k, t in enumerate([b11 + b22, b12 - b22, b21 - b11, b11 + b12, b21 + b22]):
                r1, c1 = dn_place(c, k)
                wd2[1, r1 + r:r1 + r + 8, c1:c1 + 256] = t.astype(bf16)

    def gu_tables(src, dst, c0):
        for r in range(0, 128, 8):
            for k1 in range(7):
                def ld(q, a):
                    r0 = 256 * (q // 2) + 128 * a + r
                    return wgu[src, r0:r0 + 8, c0 + 256 * (q % 2):c0 + 256 * (q % 2) + 256].astype(f32)
                blocks = [[ld(q, a) for a in range(2)] for q in _RHS_BLOCKS[k1]]
                if _RHS_SIGN[k1] > 0:
                    rows = [blocks[0][a] + blocks[1][a] for a in range(2)]
                elif _RHS_SIGN[k1] < 0:
                    rows = [blocks[0][a] - blocks[1][a] for a in range(2)]
                else:
                    rows = blocks[0]
                ts = _rhs7(rows[0][:, 0:128], rows[0][:, 128:256], rows[1][:, 0:128], rows[1][:, 128:256])
                rd = 256 * k1 + r
                wgu[dst, rd:rd + 8, c0:c0 + 512] = jnp.concatenate(ts[0:4], axis=1).astype(bf16)
                wgu[dst, rd + 128:rd + 136, c0:c0 + 384] = jnp.concatenate(ts[4:7], axis=1).astype(bf16)
                wgu[dst, rd + 128:rd + 136, c0 + 384:c0 + 512] = wgu[src, r:r + 8, c0:c0 + 128]

    def p1(i, carry):
        @pl.when(i == N1 - 1)
        def _():
            waits(g_w)
        for c in range(NC):
            gu_tables(i, jnp.minimum(i, 1) + 2, c * FC)
        for j in range(R):
            c0 = pl.multiple_of(P1 + i * T1 + 128 * j, 128)
            rn = pl.multiple_of(jnp.minimum(P1 + i * T1 + 128 * (j + 1), S - 128), 128)
            ln_rows(rn, 128, xn_buf, 128 * ((j + 1) % R))
            for off, dst in ((K_OFF, phik), (Q_OFF, phiq)):
                for B in range(2):
                    proj_qk(off, dst, B, xn_buf, 128 * j, c0)
                    drain()
            proj_v(xn_buf, 128 * j, c0)
        return carry

    waits(g_xr)
    lax.fori_loop(0, N1, p1, 0)

    for c in range(NC):
        down_tables(pl.program_id(0), c)

    rr = lax.broadcasted_iota(jnp.int32, (64, 128), 0)
    cc = lax.broadcasted_iota(jnp.int32, (64, 128), 1)
    par = (cc >> 1) & 1
    col0 = jnp.where(cc < 80, par, jnp.where(cc < 112, 2, 2 + par))
    col1 = jnp.where(cc < 32, 0, jnp.where(cc < 48, par - 1, 1 + par))
    row0 = jnp.where(rr < 60, rr // DH, jnp.minimum(rr - 60, 2))
    row1 = jnp.where(rr < 4, jnp.minimum(rr, 2), (rr - 4) // DH)
    msks = (col0 == row0, col1 == row1)

    def unzip(y):
        u = _pk(y.astype(bf16))
        lo = lax.bitcast_convert_type(u << 16, f32)
        hi = lax.bitcast_convert_type(u & jnp.uint32(0xFFFF0000), f32)
        return jnp.concatenate([t[a:a + 8] for a in range(0, u.shape[0], 8) for t in (lo, hi)], axis=0)

    for t in range(10):
        kvm[t] = _pk(jnp.where(msks[t % 2], unzip(_nt(_up(vaug[t]), _up(phik[t]))), 0.0).astype(bf16))
    rl = lax.broadcasted_iota(jnp.int32, (48, 80), 0)
    cl = lax.broadcasted_iota(jnp.int32, (48, 80), 1)
    rowl = jnp.where(rl < 40, (rl >= 20).astype(jnp.int32), (rl >= 44).astype(jnp.int32))
    kvl = unzip(_nt(_up(vaug[10, 0:24, :]), _up(phik[10, 0:40, :])))
    kvm[10, 0:24, 0:80] = _pk(jnp.where(((cl >> 1) & 1) == rowl, kvl, 0.0).astype(bf16))

    def attn_o(c0):
        low = lax.broadcasted_iota(jnp.int32, (8, NW), 0) < 4
        cols = pl.ds(c0, NW)

        def bc(r, k):
            return jnp.broadcast_to(r[k:k + 1], (8, NW))
        os = []
        for T in range(5):
            n0 = _nn(_up(kvm[2 * T]), _up(phiq[2 * T, :, cols]))
            n1 = _nn(_up(kvm[2 * T + 1]), _up(phiq[2 * T + 1, :, cols]))
            r0 = _rcp(n0[56:64] + 1e-6)
            r1 = _rcp(n1[0:8] + 1e-6)
            a, b, c = bc(r0, 4), bc(r0, 5), bc(r0, 6)
            d, e, f = bc(r1, 0), bc(r1, 1), bc(r1, 2)
            os += [n0[0:8] * a, n0[8:16] * a, n0[16:24] * jnp.where(low, a, b), n0[24:32] * b, n0[32:40] * b,
                   n0[40:48] * c, n0[48:56] * c, jnp.where(low, n0[56:64] * c, n1[0:8] * d),
                   n1[8:16] * d, n1[16:24] * d, n1[24:32] * e, n1[32:40] * e, n1[40:48] * jnp.where(low, e, f),
                   n1[48:56] * f, n1[56:64] * f]
        nd = _nn(_up(kvm[10, 0:24, 0:80]), _up(phiq[10, 0:40, cols]))
        r = _rcp(nd[40:48] + 1e-6)
        rrot = pltpu.roll(r, 4, 0)
        ra = jnp.where(low, r, rrot)
        rb = jnp.where(low, rrot, r)
        os += [nd[0:8] * ra, nd[8:16] * ra, nd[16:24] * r, nd[24:32] * rb, nd[32:40] * rb]
        return jnp.concatenate(os, axis=0).astype(bf16).T

    def p2(i, carry):
        o = jnp.concatenate([attn_o(pl.multiple_of(i * T2 + w, NW)) for w in range(0, T2, NW)], axis=0)
        hs, hns = [], []
        for w in range(0, T2, 64):
            r0 = pl.multiple_of(i * T2 + w, 64)
            hw = x_v[pl.ds(r0, 64), :].astype(f32) + _nn(o[w:w + 64], wo_v[...])
            hs.append(hw)
            hns.append(_ln(hw))
        h = jnp.concatenate(hs, axis=0)
        hn = jnp.concatenate(hns, axis=0)
        hq = [_quarter(hn[:, 0:512], q) for q in range(4)]
        top = jnp.concatenate(hq[0:2], axis=0)
        bot = jnp.concatenate(hq[2:4], axis=0)
        L = [[t.astype(bf16) for t in _lhs7(t1[:128, :128], t1[:128, 128:], t1[128:, :128], t1[128:, 128:])]
             for t1 in _lhs7(top[:, 0:256], top[:, 256:512], bot[:, 0:256], bot[:, 256:512])]
        hrest = [hn[128 * rb:128 * rb + 128, 512:640].astype(bf16) for rb in range(4)]

        gp = {}
        gm = {}
        rp = {}
        act = {}
        dl = {}
        dp = {}
        dr = {rb: h[128 * rb:128 * rb + 128, 512:640] for rb in range(4)}

        def G(c, k):
            def step(k2):
                r0, c1 = 256 * k + 128 * (k2 // 4), c * FC + 128 * (k2 % 4)
                for w in range(2):
                    gp[c, w, k, k2] = _nn(L[k][k2], wgu[2 + w, r0:r0 + 128, c1:c1 + 128])
            return [(lambda k2=k2: step(k2)) for k2 in (2, 4, 1, 3, 0, 6, 5)]

        def Rr(c):
            def step(rb, b, w):
                rp[c, w, rb, b] = _nn(hrest[rb], wgu[w, 512:640, c * FC + 256 * b:c * FC + 256 * b + 256])
            return [(lambda rb=rb, b=b, w=w: step(rb, b, w)) for rb in range(4) for b in (1, 0) for w in range(2)]

        def fin(c, *ks):
            for k in ks:
                for w in range(2):
                    t = _comb([gp[c, w, k, k2] for k2 in range(7)])
                    gm[c, w, k] = jnp.concatenate([jnp.concatenate(r_, axis=1) for r_ in t], axis=0)

        def quad(c, a, b):
            gu = []
            for w in range(2):
                full = jnp.concatenate([rp[c, w, rb, b] for rb in range(4)], axis=0)
                t = jnp.concatenate([_quarter(full, 2 * a), _quarter(full, 2 * a + 1)], axis=0)
                for sg, k in _QUAD_TERMS[a, b]:
                    t = t + gm[c, w, k] if sg > 0 else t - gm[c, w, k]
                gu.append(t)
            act[c, a, b] = _gelu_mul(*gu)

        def dlhs(c, k, rh):
            if (c, k, rh) not in dl:
                def a(x, y):
                    return act[c, x, y][128 * rh:128 * rh + 128]
                dl[c, k, rh] = [lambda: a(0, 0) + a(1, 1), lambda: a(1, 0) + a(1, 1), lambda: a(0, 0),
                                lambda: a(1, 1), lambda: a(0, 0) + a(0, 1), lambda: a(1, 0) - a(0, 0),
                                lambda: a(0, 1) - a(1, 1)][k]().astype(bf16)
            return dl[c, k, rh]

        def drhs(c, k, ch):
            if k == 1:
                n, r1, c1 = 0, c * FC, 0
            elif k == 4:
                n, r1, c1 = 0, c * FC + 256, 256
            else:
                n, (r1, c1) = 1, dn_place(c, (0, None, 1, 2, None, 3, 4)[k])
            return wd2[n, r1:r1 + 256, c1 + 128 * ch:c1 + 128 * ch + 128]

        def Dk(c, k):
            def step(rh, ch):
                t = _nn(dlhs(c, k, rh), drhs(c, k, ch))
                ix = 4 * k + 2 * rh + ch
                if c == 0:
                    dacc[ix] = t
                elif c < NC - 1:
                    dacc[ix] = dacc[ix] + t
                else:
                    dp[k, rh, ch] = dacc[ix] + t
            return [(lambda rh=rh, ch=ch: step(rh, ch)) for rh in range(2) for ch in range(2)]

        def act_rows(c):
            return [jnp.concatenate([act[c, q // 2, b][128 * (q % 2):128 * (q % 2) + 128] for b in range(2)], axis=1)
                    for q in range(4)]

        def Dr(c):
            def step(rb):
                dr[rb] = dr[rb] + _nn(_natural(act_rows(c), 2 * rb, 2 * rb + 2).astype(bf16),
                                      wd2[0, c * FC:(c + 1) * FC, 512:640])
            return [(lambda rb=rb: step(rb)) for rb in range(4)]

        def out_block(r0, n, c0, val):
            rr0 = pl.multiple_of(i * T2 + r0, 16)
            out_v[pl.ds(rr0, n), c0:c0 + 128] = val.astype(bf16)
            cp(out_v.at[pl.ds(rr0, n), pl.ds(c0, 128)], out_hbm.at[0, pl.ds(rr0, n), pl.ds(c0, 128)], 0).start()

        def all_d(c):
            return sum([Dk(c, k) for k in (2, 4, 5, 0, 1, 3, 6)], [])

        r1s, r2s = Rr(1), Rr(2)
        _run(Rr(0))
        _run(G(0, 2))
        for c in range(NC):
            if c == 0:
                mates = [r1s[:7], r1s[7:14], G(1, 2), None]
                gaps = [[], [], r1s[14:]]
            elif c == 1:
                dd = all_d(0)[7:] + r2s[:7]
                mates = [dd[0:7], dd[7:14], dd[14:21], dd[21:28]]
                gaps = [Dr(0)[:2], Dr(0)[2:], G(2, 2)]
            else:
                dd = all_d(1)
                mates = [dd[0:7], dd[7:14], dd[14:21], dd[21:28]]
                gaps = [Dr(1)[:2], Dr(1)[2:], []]
            fin(c, 2)
            _run(G(c, 4), mates[0])
            fin(c, 4)
            quad(c, 0, 1)
            _run(G(c, 1))
            _run(gaps[0])
            _run(G(c, 3), mates[1])
            fin(c, 1, 3)
            quad(c, 1, 0)
            _run(G(c, 0))
            _run(gaps[1])
            _run(G(c, 6), mates[2])
            fin(c, 0, 6)
            quad(c, 0, 0)
            _run(gaps[2])
            _run(G(c, 5), mates[3] if c else all_d(0)[:7])
            fin(c, 5)
            quad(c, 1, 1)
            if c == 1:
                _run(r2s[7:])

        c = NC - 1
        _run(Dk(c, 2) + Dk(c, 4) + Dk(c, 5))
        da, db = {1: Dk(c, 0), 0: Dk(c, 3)}, {1: Dk(c, 1), 0: Dk(c, 6)}
        for blk in (1, 0):
            for ch in range(2):
                _run([da[blk][ch], da[blk][2 + ch], db[blk][ch], db[blk][2 + ch]])

                def g_(k, rh):
                    return dp[k, rh, ch]
                if blk == 1:
                    part = [g_(2, 0) + g_(4, 0), g_(2, 1) + g_(4, 1),
                            g_(2, 0) + g_(5, 0) + g_(0, 0) - g_(1, 0), g_(2, 1) + g_(5, 1) + g_(0, 1) - g_(1, 1)]
                else:
                    part = [g_(0, 0) - g_(4, 0) + g_(3, 0) + g_(6, 0), g_(0, 1) - g_(4, 1) + g_(3, 1) + g_(6, 1),
                            g_(1, 0) + g_(3, 0), g_(1, 1) + g_(3, 1)]
                c0 = 256 * blk + 128 * ch
                out_block(0, T2, c0, h[:, c0:c0 + 128] + _natural(part, 0, NS))
        drf = jnp.concatenate([dr[rb] for rb in range(4)], axis=0)
        an = _natural(act_rows(c), 0, NS)
        for lo, n in LAST_PIECES:
            out_block(lo, n, 512,
                      drf[lo:lo + n] + _nn(an[lo:lo + n].astype(bf16), wd2[0, c * FC:(c + 1) * FC, 512:640]))
        return carry

    lax.fori_loop(0, N2, p2, 0)
    cp(out_v, out_hbm.at[0], 0).wait()


def _kernel(*refs):
    @pl.when(pl.program_id(0) == 0)
    def _():
        _body(*refs)


@jax.jit
def pallas_sequential_preLN__linear_kernel_hedgehog__geglu_ffn__prompt_kernel(
    A_x: jax.Array,
    A_wqkv: jax.Array,
    A_w_phi: jax.Array,
    A_wo: jax.Array,
    B_x: jax.Array,
    B_w_gate: jax.Array,
    B_w_up: jax.Array,
    B_w_down: jax.Array,
):
    del B_x
    anyspec = pl.BlockSpec(memory_space=pl.ANY)
    wphi_t = jnp.transpose(A_w_phi, (1, 2, 0))
    return pl.pallas_call(
        _kernel,
        out_shape=jax.ShapeDtypeStruct((1, S, D), bf16),
        grid=(2,),
        in_specs=[anyspec] * 7,
        out_specs=anyspec,
        scratch_shapes=[
            pltpu.VMEM((S, D), bf16),
            pltpu.VMEM((D, D), bf16),
            pltpu.VMEM((D, D), bf16),
            pltpu.VMEM((D, D), bf16),
            pltpu.VMEM((DH, DH, H), bf16),
            pltpu.VMEM((D, D), bf16),
            pltpu.VMEM((4, 1792, F), bf16),
            pltpu.VMEM((2, 2048, D), bf16),
            pltpu.VMEM((928, D), u32),
            pltpu.VMEM((32, D), f32),
            pltpu.VMEM((P1 // 2, D), u32),
            pltpu.VMEM((T1 // 2, D), u32),
            pltpu.VMEM((11, 64, S), u32),
            pltpu.VMEM((11, 64, S), u32),
            pltpu.VMEM((11, 32, S), u32),
            pltpu.VMEM((11, 32, 128), u32),
            pltpu.VMEM((28, 128, 128), f32),
            pltpu.VMEM((S, D), bf16),
            pltpu.SemaphoreType.DMA((4,)),
        ],
        compiler_params=pltpu.CompilerParams(
            dimension_semantics=("arbitrary",),
            vmem_limit_bytes=100 * 1024 * 1024,
            disable_bounds_checks=True,
            disable_semaphore_checks=True,
        ),
        name="hh",
    )(A_x, A_wqkv, wphi_t, A_wo, B_w_gate, B_w_up, B_w_down)
```

```python
import jax
import jax.numpy as jnp
from jax import lax
from jax.experimental import pallas as pl
from jax.experimental.pallas import tpu as pltpu

S, D, H, DH, F = 2048, 640, 32, 20, 1536
LOG2E = 1.4426950408889634
NT_DIMS = (((1,), (1,)), ((), ()))
f32 = jnp.float32
bf16 = jnp.bfloat16
u32 = jnp.uint32

NP = 6
R = 5
T1 = 128 * R
P1 = 128 * NP
N1 = (S - P1) // T1
T2 = 512
N2 = S // T2
NS = T2 // 64
NW = 256
LNC = 64
FC = 512
NC = F // FC
K_OFF, Q_OFF, V_OFF = 0, 304, 608
LAST_PIECES = ((0, 128), (128, 128), (256, 128), (384, 64), (448, 32), (480, 32))
assert P1 + N1 * T1 == S and N1 == 2 and NC == 3


def _ln(x):
    m = jnp.mean(x, axis=-1, keepdims=True)
    xc = x - m
    v = jnp.mean(xc * xc, axis=-1, keepdims=True) + 1e-5
    return xc * jnp.exp2(jnp.log(v) * (-0.5 * LOG2E))


def _rcp(x):
    return pl.reciprocal(x, approx=True)


def _allred(m, op):
    m = op(m, pltpu.roll(m, 2, 0))
    return op(m, pltpu.roll(m, 4, 0))


def _tree(op, xs):
    return op(op(op(xs[0], xs[1]), op(xs[2], xs[3])), xs[4])


def _pk(v):
    return pltpu.bitcast(v, u32)


def _up(v):
    return pltpu.bitcast(v, bf16)


def _feat5(ps):
    mx = _allred(_tree(jnp.maximum, ps), jnp.maximum)
    mn = _allred(_tree(jnp.minimum, ps), jnp.minimum)
    ep = [jnp.exp2(q - mx) for q in ps]
    en = [jnp.exp2(mn - q) for q in ps]
    rp = _rcp(_allred(_tree(jnp.add, ep), jnp.add))
    rn = _rcp(_allred(_tree(jnp.add, en), jnp.add))
    return [e * rp for e in ep] + [e * rn for e in en]


def _gelu_mul(g, u):
    c = 0.7978845608028654
    t = jnp.tanh(g * (c + (c * 0.044715) * (g * g)))
    hgu = (0.5 * g) * u
    return hgu + hgu * t


def _nt(a, b):
    return lax.dot_general(a, b, NT_DIMS, preferred_element_type=f32)


def _nn(a, b):
    return jnp.dot(a, b, preferred_element_type=f32)


def _pair_is(a, w):
    return (lax.broadcasted_iota(jnp.int32, (8, w), 0) >> 1) == a


def _lhs7(a11, a12, a21, a22):
    return [a11 + a22, a21 + a22, a11, a22, a11 + a12, a21 - a11, a12 - a22]


def _rhs7(b11, b12, b21, b22):
    return [b11 + b22, b11, b12 - b22, b21 - b11, b22, b11 + b12, b21 + b22]


def _comb(q):
    return [[q[3] - q[4] + q[0] + q[6], q[2] + q[4]], [q[1] + q[3], q[2] - q[1] + q[0] + q[5]]]


_RHS_BLOCKS = ((0, 3), (0,), (1, 3), (2, 0), (3,), (0, 1), (2, 3))
_RHS_SIGN = (1, 0, -1, -1, 0, 1, 1)
_QUAD_TERMS = {(0, 1): ((1, 2), (1, 4)), (1, 0): ((1, 1), (1, 3)),
               (0, 0): ((1, 3), (-1, 4), (1, 0), (1, 6)), (1, 1): ((1, 2), (-1, 1), (1, 0), (1, 5))}


def _quarter(x, q):
    return jnp.concatenate([x[64 * s + 16 * q:64 * s + 16 * q + 16] for s in range(NS)], axis=0)


def _natural(qs, s0, s1):
    return jnp.concatenate([qs[q][16 * s:16 * s + 16] for s in range(s0, s1) for q in range(4)], axis=0)


def _run(*streams):
    streams = [list(t) for t in streams]
    while any(streams):
        for t in streams:
            if t:
                t.pop(0)()


def _body(x_hbm, wqkv_hbm, wphi_hbm, wo_hbm, wg_hbm, wu_hbm, wd_hbm, out_hbm,
          x_v, wq_v, wk_v, wv_v, wphi_v, wo_v, wgu, wd2, wT, bcat,
          xn0, xn_buf, phiq, phik, vaug, kvm, dacc, out_v, sem):
    def cp(src, dst, k):
        return pltpu.make_async_copy(src, dst, sem.at[k])

    def xrows(r0, r1, k):
        return cp(x_hbm.at[0, pl.ds(r0, r1 - r0)], x_v.at[pl.ds(r0, r1 - r0)], k)

    def wk_cols(c0, n, k):
        return cp(wqkv_hbm.at[:, pl.ds(D + c0, n)], wk_v.at[:, pl.ds(c0, n)], k)

    g_phi = [cp(wphi_hbm, wphi_v, 0)]
    g_x0 = [xrows(0, 256, 1)]
    g_ka = [wk_cols(0, 256, 2)]
    g_kb = [wk_cols(256, 256, 3)]
    g_kc = [wk_cols(512, 128, 0), xrows(256, P1, 0)]
    g_qv = [cp(wqkv_hbm.at[:, pl.ds(0, D)], wq_v, 1), cp(wqkv_hbm.at[:, pl.ds(2 * D, D)], wv_v, 1),
            xrows(P1, P1 + 128, 1)]
    g_xr = [xrows(P1 + 128, S, 2), cp(wg_hbm, wgu.at[0, pl.ds(0, D)], 2)]
    g_w = [cp(wu_hbm, wgu.at[1, pl.ds(0, D)], 3), cp(wd_hbm, wd2.at[0, pl.ds(0, F)], 3), cp(wo_hbm, wo_v, 3)]

    def waits(cs, starts=()):
        for c in cs:
            c.wait()
        for c in starts:
            c.start()

    for c in g_phi + g_x0 + g_ka + g_kb:
        c.start()

    def ln_rows(r0, n, dst, d0):
        for c in range(0, n, LNC):
            xn = _ln(x_v[pl.ds(r0 + c, LNC), :].astype(f32)).astype(bf16)
            dst[(d0 + c) // 2:(d0 + c + LNC) // 2, :] = _pk(xn)

    pending = []

    def drain(keep=0):
        while len(pending) > keep:
            pending.pop(0)()

    def phi_store(dst, g, x, j):
        T, role = divmod(g, 3)
        if role == 0:
            dst[2 * T, j, 0:80, :] = jnp.concatenate(x, axis=0).astype(bf16)
        elif role == 2:
            dst[2 * T + 1, j, 48:128, :] = jnp.concatenate(x, axis=0).astype(bf16)
        else:
            even = (lax.broadcasted_iota(jnp.int32, (8, 128), 0) & 1) == 0
            ev = [jnp.where(even, x[a], pltpu.roll(x[a + 1], 1, 0)) for a in (0, 2, 4, 6)]
            od = [jnp.where(even, pltpu.roll(x[a], 7, 0), x[a + 1]) for a in (0, 2, 4, 6)]
            dst[2 * T, j, 80:128, :] = jnp.concatenate(ev + x[8:10], axis=0).astype(bf16)
            dst[2 * T + 1, j, 0:48, :] = jnp.concatenate(od + x[8:10], axis=0).astype(bf16)

    def feat_block(p, dst, b, j, rfirst=True):
        ro, mo = (0, 24) if rfirst else (128, 0)
        rs = [p[ro + 8 * a:ro + 8 + 8 * a] for a in range(3)]
        for a in range(4):
            if a < 3:
                v4 = jnp.where(_pair_is(a, 128), 0.0, rs[a])
            else:
                v4 = jnp.where(_pair_is(0, 128), rs[0],
                               jnp.where(_pair_is(1, 128), rs[1], jnp.where(_pair_is(2, 128), rs[2], 0.0)))
            ps = [p[mo + 32 * a + 8 * v:mo + 8 + 32 * a + 8 * v] for v in range(4)] + [v4]
            phi_store(dst, 4 * b + a, _feat5(ps), j)

    def xs(xref, xr0):
        return _up(xref[xr0 // 2:xr0 // 2 + 64, :])

    def proj_qk(off, dst, B, xref, xr0, j):
        p = _nt(_up(wT[off + 152 * B:off + 152 * B + 152, :]), xs(xref, xr0))

        def post():
            feat_block(p[0:152], dst, 2 * B, j)
            feat_block(p[152:304], dst, 2 * B + 1, j)
        pending.append(post)

    def nt2(a, b, split):
        if split:
            return jnp.concatenate([_nt(a[0:80], b), _nt(a[80:160], b)], axis=0)
        return _nt(a, b)

    def proj_k4(wb, b, j, rfirst, split=False):
        p = nt2(wb, xs(xn0, 128 * j), split)
        pending.append(lambda: feat_block(p[0:152], phik, b, j, rfirst))

    def proj_v(xref, xr0, j):
        p = jnp.concatenate([_nt(_up(wT[V_OFF + a:V_OFF + a + 80, :]), xs(xref, xr0))
                             for a in range(0, 320, 80)], axis=0)
        low = lax.broadcasted_iota(jnp.int32, (8, 128), 0) < 4
        for T in range(5):
            mid = p[120 * T + 56:120 * T + 64]
            t0 = jnp.concatenate([p[120 * T:120 * T + 56], jnp.where(low, mid, 1.0)], axis=0)
            t1 = jnp.concatenate([jnp.where(low, 1.0, mid), p[120 * T + 64:120 * T + 120]], axis=0)
            vaug[2 * T, j] = t0.astype(bf16)
            vaug[2 * T + 1, j] = t1.astype(bf16)
        vaug[10, j, 0:48, :] = jnp.concatenate([p[600:640], jnp.ones((8, 128), f32)], axis=0).astype(bf16)

    pr = lax.broadcasted_iota(jnp.int32, (D, D), 0)
    pc = lax.broadcasted_iota(jnp.int32, (D, D), 1)
    perm = jnp.where((pr & 31) * DH + (pr >> 5) == pc, 1.0, 0.0).astype(bf16)
    r_i = lax.broadcasted_iota(jnp.int32, (160, 32), 0)
    c_i = lax.broadcasted_iota(jnp.int32, (160, 32), 1)
    gl = r_i // 40
    sl_ = (r_i - 40 * gl) >> 1
    q_ = sl_ - 16
    f_ = jnp.where(sl_ < 16, sl_ + 1, jnp.where(q_ == gl, 0, jnp.where(q_ < gl, 17 + q_, 16 + q_)))
    e0 = jnp.where(f_ == c_i, 1.0, 0.0)
    es = []
    for t in range(5):
        off = (120 * t) % 160
        es.append((jnp.concatenate([e0[off:], e0[:off]], axis=0) if off else e0).astype(bf16))
    r2 = lax.broadcasted_iota(jnp.int32, (160, 128), 0)
    hr = 2 * (r2 // 40) + (r2 & 1)
    hc = [(lax.broadcasted_iota(jnp.int32, (1, 128), 1) + 128 * t) // DH - 6 * t for t in range(5)]
    bcat[...] = jnp.zeros(bcat.shape, f32)

    waits(g_phi, g_kc)
    for d in range(DH):
        bcat[0:DH, 32 * d:32 * d + 32] = wphi_v[d].astype(f32)
    at = _nn(bcat[...].astype(bf16), perm).astype(bf16)

    def edot(t):
        return jnp.concatenate([_nn(es[t][a:b], at[:, 128 * t:128 * t + 128])
                                for a, b in ((0, 48), (48, 80), (80, 128), (128, 160))], axis=0)
    pts = [jnp.where(hr == hc[t], edot(t), 0.0).astype(bf16) for t in range(5)]

    def fold(w_v, off, t, rs, blk, split=False):
        rs[t] = nt2(pts[t], w_v[:, 128 * t:128 * t + 128], split)
        if t == 0:
            return
        b = t - 1
        lo, hi = rs[t - 1], rs[t]
        parts = []
        if b < 3:
            parts.append(lo[40 * b:120])
        parts.append(lo[120:160] + hi[0:40])
        if b > 0:
            parts.append(hi[40:40 + 40 * b])
        w = jnp.concatenate(parts, axis=0)
        mains, v4s = [], []
        for a in range(4):
            v4 = w[40 * a + 32:40 * a + 40]
            base = _allred(jnp.where(_pair_is(a, D), v4, 0.0), jnp.add)
            mains += [(w[40 * a + 8 * v:40 * a + 8 * v + 8] - base) * LOG2E for v in range(4)]
            v4s.append((v4 - base) * LOG2E)
        shared = [jnp.where(_pair_is(a, D), v4s[3], v4s[a]) for a in range(3)]
        blk[b] = (shared, mains)
        if b % 2 == 1:
            B = b // 2
            rows = blk[b - 1][0] + blk[b - 1][1] + blk[b][0] + blk[b][1]
            wT[off + 152 * B:off + 152 * B + 152, :] = _pk(jnp.concatenate(rows, axis=0).astype(bf16))

    def blk16(slabs, rfirst):
        rows = slabs[0] + slabs[1] if rfirst else slabs[1] + slabs[0]
        return jnp.concatenate(rows + [jnp.zeros((8, D), f32)], axis=0).astype(bf16)

    waits(g_x0, g_qv)
    ln_rows(0, 256, xn0, 0)

    rk, rq, bk, bq = {}, {}, {}, {}
    waits(g_ka, g_xr)
    fold(wk_v, K_OFF, 0, rk, bk)
    fold(wk_v, K_OFF, 1, rk, bk)
    w0 = blk16(bk[0], False)
    proj_k4(w0, 0, 0, False)
    proj_k4(w0, 0, 1, False)

    waits(g_kb, g_w)
    fold(wk_v, K_OFF, 2, rk, bk)
    fold(wk_v, K_OFF, 3, rk, bk)
    w1 = blk16(bk[1], False)
    proj_k4(w1, 1, 0, False)
    proj_k4(w1, 1, 1, False)
    w2 = blk16(bk[2], True)
    proj_k4(w2, 2, 0, True, True)
    proj_k4(w2, 2, 1, True, True)
    drain(1)

    waits(g_kc)
    fold(wk_v, K_OFF, 4, rk, bk, True)
    ln_rows(256, P1 - 256, xn0, 256)
    w3 = blk16(bk[3], False)
    proj_k4(w3, 3, 0, False, True)
    for j in range(2, NP):
        for B in range(2):
            proj_qk(K_OFF, phik, B, xn0, 128 * j, j)
    drain(1)

    waits(g_qv)
    for t in range(5):
        fold(wq_v, Q_OFF, t, rq, bq, t == 4)
    proj_k4(w3, 3, 1, False, True)
    for t in range(5):
        wT[V_OFF + 64 * t:V_OFF + 64 * t + 64, :] = _pk(wv_v[:, 128 * t:128 * t + 128].T)
    ln_rows(P1, 128, xn_buf, 0)
    for j in range(NP):
        for B in range(2):
            proj_qk(Q_OFF, phiq, B, xn0, 128 * j, j)
    drain()
    for j in range(NP):
        proj_v(xn0, 128 * j, j)

    def dn_place(c, k):
        return 256 * ((5 * c + k) // 2), 256 * ((5 * c + k) % 2)

    def down_tables(src, c):
        for r in range(0, 256, 8):
            b11, b12, b21, b22 = [
                wd2[src, c * FC + 256 * a + r:c * FC + 256 * a + r + 8, 256 * b:256 * b + 256].astype(f32)
                for a in range(2) for b in range(2)]
            for k, t in enumerate([b11 + b22, b12 - b22, b21 - b11, b11 + b12, b21 + b22]):
                r1, c1 = dn_place(c, k)
                wd2[1, r1 + r:r1 + r + 8, c1:c1 + 256] = t.astype(bf16)

    def gu_tables(src, dst, c0):
        for r in range(0, 128, 8):
            for k1 in range(7):
                def ld(q, a):
                    r0 = 256 * (q // 2) + 128 * a + r
                    return wgu[src, r0:r0 + 8, c0 + 256 * (q % 2):c0 + 256 * (q % 2) + 256].astype(f32)
                blocks = [[ld(q, a) for a in range(2)] for q in _RHS_BLOCKS[k1]]
                if _RHS_SIGN[k1] > 0:
                    rows = [blocks[0][a] + blocks[1][a] for a in range(2)]
                elif _RHS_SIGN[k1] < 0:
                    rows = [blocks[0][a] - blocks[1][a] for a in range(2)]
                else:
                    rows = blocks[0]
                ts = _rhs7(rows[0][:, 0:128], rows[0][:, 128:256], rows[1][:, 0:128], rows[1][:, 128:256])
                rd = 256 * k1 + r
                wgu[dst, rd:rd + 8, c0:c0 + 512] = jnp.concatenate(ts[0:4], axis=1).astype(bf16)
                wgu[dst, rd + 128:rd + 136, c0:c0 + 384] = jnp.concatenate(ts[4:7], axis=1).astype(bf16)
                wgu[dst, rd + 128:rd + 136, c0 + 384:c0 + 512] = wgu[src, r:r + 8, c0:c0 + 128]

    def p1(i, carry):
        @pl.when(i == N1 - 1)
        def _():
            waits(g_w)
        for c in range(NC):
            gu_tables(i, jnp.minimum(i, 1) + 2, c * FC)
        for j in range(R):
            jt = NP + i * R + j
            rn = pl.multiple_of(jnp.minimum(P1 + i * T1 + 128 * (j + 1), S - 128), 128)
            ln_rows(rn, 128, xn_buf, 128 * ((j + 1) % R))
            for off, dst in ((K_OFF, phik), (Q_OFF, phiq)):
                for B in range(2):
                    proj_qk(off, dst, B, xn_buf, 128 * j, jt)
                    drain()
            proj_v(xn_buf, 128 * j, jt)
        return carry

    waits(g_xr)
    lax.fori_loop(0, N1, p1, 0)

    for c in range(NC):
        down_tables(pl.program_id(0), c)

    rr = lax.broadcasted_iota(jnp.int32, (64, 128), 0)
    cc = lax.broadcasted_iota(jnp.int32, (64, 128), 1)
    par = cc & 1
    col0 = jnp.where(cc < 80, par, jnp.where(cc < 112, 2, 2 + par))
    col1 = jnp.where(cc < 32, 0, jnp.where(cc < 48, par - 1, 1 + par))
    row0 = jnp.where(rr < 60, rr // DH, jnp.minimum(rr - 60, 2))
    row1 = jnp.where(rr < 4, jnp.minimum(rr, 2), (rr - 4) // DH)
    msks = (col0 == row0, col1 == row1)

    def allcols(ref, t, n):
        return jnp.concatenate([ref[t, j, 0:n, :] for j in range(S // 128)], axis=1)

    for t in range(10):
        kvm[t] = _pk(jnp.where(msks[t % 2], _nt(allcols(vaug, t, 64), allcols(phik, t, 128)), 0.0).astype(bf16))
    rl = lax.broadcasted_iota(jnp.int32, (48, 80), 0)
    cl = lax.broadcasted_iota(jnp.int32, (48, 80), 1)
    rowl = jnp.where(rl < 40, (rl >= 20).astype(jnp.int32), (rl >= 44).astype(jnp.int32))
    kvl = _nt(allcols(vaug, 10, 48), allcols(phik, 10, 80))
    kvm[10, 0:24, 0:80] = _pk(jnp.where((cl & 1) == rowl, kvl, 0.0).astype(bf16))

    def attn_o(j0):
        low = lax.broadcasted_iota(jnp.int32, (8, NW), 0) < 4

        def pq(t, n):
            return jnp.concatenate([phiq[t, j0 + j, 0:n, :] for j in range(NW // 128)], axis=1)

        def bc(r, k):
            return jnp.broadcast_to(r[k:k + 1], (8, NW))
        os = []
        for T in range(5):
            n0 = _nn(_up(kvm[2 * T]), pq(2 * T, 128))
            n1 = _nn(_up(kvm[2 * T + 1]), pq(2 * T + 1, 128))
            r0 = _rcp(n0[56:64] + 1e-6)
            r1 = _rcp(n1[0:8] + 1e-6)
            a, b, c = bc(r0, 4), bc(r0, 5), bc(r0, 6)
            d, e, f = bc(r1, 0), bc(r1, 1), bc(r1, 2)
            os += [n0[0:8] * a, n0[8:16] * a, n0[16:24] * jnp.where(low, a, b), n0[24:32] * b, n0[32:40] * b,
                   n0[40:48] * c, n0[48:56] * c, jnp.where(low, n0[56:64] * c, n1[0:8] * d),
                   n1[8:16] * d, n1[16:24] * d, n1[24:32] * e, n1[32:40] * e, n1[40:48] * jnp.where(low, e, f),
                   n1[48:56] * f, n1[56:64] * f]
        nd = _nn(_up(kvm[10, 0:24, 0:80]), pq(10, 80))
        r = _rcp(nd[40:48] + 1e-6)
        rrot = pltpu.roll(r, 4, 0)
        ra = jnp.where(low, r, rrot)
        rb = jnp.where(low, rrot, r)
        os += [nd[0:8] * ra, nd[8:16] * ra, nd[16:24] * r, nd[24:32] * rb, nd[32:40] * rb]
        return jnp.concatenate(os, axis=0).astype(bf16).T

    def p2(i, carry):
        o = jnp.concatenate([attn_o(i * (T2 // 128) + w // 128) for w in range(0, T2, NW)], axis=0)
        hs, hns = [], []
        for w in range(0, T2, 64):
            r0 = pl.multiple_of(i * T2 + w, 64)
            hw = x_v[pl.ds(r0, 64), :].astype(f32) + _nn(o[w:w + 64], wo_v[...])
            hs.append(hw)
            hns.append(_ln(hw))
        h = jnp.concatenate(hs, axis=0)
        hn = jnp.concatenate(hns, axis=0)
        hq = [_quarter(hn[:, 0:512], q) for q in range(4)]
        top = jnp.concatenate(hq[0:2], axis=0)
        bot = jnp.concatenate(hq[2:4], axis=0)
        L = [[t.astype(bf16) for t in _lhs7(t1[:128, :128], t1[:128, 128:], t1[128:, :128], t1[128:, 128:])]
             for t1 in _lhs7(top[:, 0:256], top[:, 256:512], bot[:, 0:256], bot[:, 256:512])]
        hrest = [hn[128 * rb:128 * rb + 128, 512:640].astype(bf16) for rb in range(4)]

        gp = {}
        gm = {}
        rp = {}
        act = {}
        dl = {}
        dp = {}
        dr = {rb: h[128 * rb:128 * rb + 128, 512:640] for rb in range(4)}

        def G(c, k):
            def step(k2):
                r0, c1 = 256 * k + 128 * (k2 // 4), c * FC + 128 * (k2 % 4)
                for w in range(2):
                    gp[c, w, k, k2] = _nn(L[k][k2], wgu[2 + w, r0:r0 + 128, c1:c1 + 128])
            return [(lambda k2=k2: step(k2)) for k2 in (2, 4, 3, 1, 0, 5, 6)]

        def Rr(c):
            def step(rb, b, w):
                rp[c, w, rb, b] = _nn(hrest[rb], wgu[w, 512:640, c * FC + 256 * b:c * FC + 256 * b + 256])
            return [(lambda rb=rb, b=b, w=w: step(rb, b, w)) for rb in range(4) for b in (1, 0) for w in range(2)]

        def fin(c, *ks):
            for k in ks:
                for w in range(2):
                    t = _comb([gp[c, w, k, k2] for k2 in range(7)])
                    gm[c, w, k] = jnp.concatenate([jnp.concatenate(r_, axis=1) for r_ in t], axis=0)

        def quad(c, a, b):
            gu = []
            for w in range(2):
                full = jnp.concatenate([rp[c, w, rb, b] for rb in range(4)], axis=0)
                t = jnp.concatenate([_quarter(full, 2 * a), _quarter(full, 2 * a + 1)], axis=0)
                for sg, k in _QUAD_TERMS[a, b]:
                    t = t + gm[c, w, k] if sg > 0 else t - gm[c, w, k]
                gu.append(t)
            act[c, a, b] = _gelu_mul(*gu)

        def dlhs(c, k, rh):
            if (c, k, rh) not in dl:
                def a(x, y):
                    return act[c, x, y][128 * rh:128 * rh + 128]
                dl[c, k, rh] = [lambda: a(0, 0) + a(1, 1), lambda: a(1, 0) + a(1, 1), lambda: a(0, 0),
                                lambda: a(1, 1), lambda: a(0, 0) + a(0, 1), lambda: a(1, 0) - a(0, 0),
                                lambda: a(0, 1) - a(1, 1)][k]().astype(bf16)
            return dl[c, k, rh]

        def drhs(c, k, ch):
            if k == 1:
                n, r1, c1 = 0, c * FC, 0
            elif k == 4:
                n, r1, c1 = 0, c * FC + 256, 256
            else:
                n, (r1, c1) = 1, dn_place(c, (0, None, 1, 2, None, 3, 4)[k])
            return wd2[n, r1:r1 + 256, c1 + 128 * ch:c1 + 128 * ch + 128]

        def Dk(c, k):
            def step(rh, ch):
                t = _nn(dlhs(c, k, rh), drhs(c, k, ch))
                ix = 4 * k + 2 * rh + ch
                if c == 0:
                    dacc[ix] = t
                elif c < NC - 1:
                    dacc[ix] = dacc[ix] + t
                else:
                    dp[k, rh, ch] = dacc[ix] + t
            return [(lambda rh=rh, ch=ch: step(rh, ch)) for rh in range(2) for ch in range(2)]

        def act_rows(c):
            return [jnp.concatenate([act[c, q // 2, b][128 * (q % 2):128 * (q % 2) + 128] for b in range(2)], axis=1)
                    for q in range(4)]

        def Dr(c):
            def step(rb):
                dr[rb] = dr[rb] + _nn(_natural(act_rows(c), 2 * rb, 2 * rb + 2).astype(bf16),
                                      wd2[0, c * FC:(c + 1) * FC, 512:640])
            return [(lambda rb=rb: step(rb)) for rb in range(4)]

        def out_block(r0, n, c0, val):
            rr0 = pl.multiple_of(i * T2 + r0, 16)
            out_v[pl.ds(rr0, n), c0:c0 + 128] = val.astype(bf16)
            cp(out_v.at[pl.ds(rr0, n), pl.ds(c0, 128)], out_hbm.at[0, pl.ds(rr0, n), pl.ds(c0, 128)], 0).start()

        def all_d(c):
            return sum([Dk(c, k) for k in (2, 4, 5, 0, 1, 3, 6)], [])

        r1s, r2s = Rr(1), Rr(2)
        _run(Rr(0))
        _run(G(0, 2))
        for c in range(NC):
            if c == 0:
                mates = [r1s[:7], r1s[7:14], G(1, 2), None]
                gaps = [[], [], r1s[14:]]
            elif c == 1:
                dd = all_d(0)[7:] + r2s[:7]
                mates = [dd[0:7], dd[7:14], dd[14:21], dd[21:28]]
                gaps = [Dr(0)[:2], Dr(0)[2:], G(2, 2)]
            else:
                dd = all_d(1)
                mates = [dd[0:7], dd[7:14], dd[14:21], dd[21:28]]
                gaps = [Dr(1)[:2], Dr(1)[2:], []]
            fin(c, 2)
            _run(G(c, 4), mates[0])
            fin(c, 4)
            quad(c, 0, 1)
            _run(G(c, 1))
            _run(gaps[0])
            _run(G(c, 3), mates[1])
            fin(c, 1, 3)
            quad(c, 1, 0)
            _run(G(c, 0))
            _run(gaps[1])
            _run(G(c, 6), mates[2])
            fin(c, 0, 6)
            quad(c, 0, 0)
            _run(gaps[2])
            _run(G(c, 5), mates[3] if c else all_d(0)[:7])
            fin(c, 5)
            quad(c, 1, 1)
            if c == 1:
                _run(r2s[7:])

        c = NC - 1
        _run(Dk(c, 2) + Dk(c, 4) + Dk(c, 5))
        da, db = {1: Dk(c, 0), 0: Dk(c, 3)}, {1: Dk(c, 1), 0: Dk(c, 6)}
        for blk in (1, 0):
            for ch in range(2):
                _run([da[blk][ch], da[blk][2 + ch], db[blk][ch], db[blk][2 + ch]])

                def g_(k, rh):
                    return dp[k, rh, ch]
                if blk == 1:
                    part = [g_(2, 0) + g_(4, 0), g_(2, 1) + g_(4, 1),
                            g_(2, 0) + g_(5, 0) + g_(0, 0) - g_(1, 0), g_(2, 1) + g_(5, 1) + g_(0, 1) - g_(1, 1)]
                else:
                    part = [g_(0, 0) - g_(4, 0) + g_(3, 0) + g_(6, 0), g_(0, 1) - g_(4, 1) + g_(3, 1) + g_(6, 1),
                            g_(1, 0) + g_(3, 0), g_(1, 1) + g_(3, 1)]
                c0 = 256 * blk + 128 * ch
                out_block(0, T2, c0, h[:, c0:c0 + 128] + _natural(part, 0, NS))
        drf = jnp.concatenate([dr[rb] for rb in range(4)], axis=0)
        an = _natural(act_rows(c), 0, NS)
        for lo, n in LAST_PIECES:
            out_block(lo, n, 512,
                      drf[lo:lo + n] + _nn(an[lo:lo + n].astype(bf16), wd2[0, c * FC:(c + 1) * FC, 512:640]))
        return carry

    lax.fori_loop(0, N2, p2, 0)
    cp(out_v, out_hbm.at[0], 0).wait()


def _kernel(*refs):
    @pl.when(pl.program_id(0) == 0)
    def _():
        _body(*refs)


@jax.jit
def pallas_sequential_preLN__linear_kernel_hedgehog__geglu_ffn__prompt_kernel(
    A_x: jax.Array,
    A_wqkv: jax.Array,
    A_w_phi: jax.Array,
    A_wo: jax.Array,
    B_x: jax.Array,
    B_w_gate: jax.Array,
    B_w_up: jax.Array,
    B_w_down: jax.Array,
):
    del B_x
    anyspec = pl.BlockSpec(memory_space=pl.ANY)
    wphi_t = jnp.transpose(A_w_phi, (1, 2, 0))
    return pl.pallas_call(
        _kernel,
        out_shape=jax.ShapeDtypeStruct((1, S, D), bf16),
        grid=(2,),
        in_specs=[anyspec] * 7,
        out_specs=anyspec,
        scratch_shapes=[
            pltpu.VMEM((S, D), bf16),
            pltpu.VMEM((D, D), bf16),
            pltpu.VMEM((D, D), bf16),
            pltpu.VMEM((D, D), bf16),
            pltpu.VMEM((DH, DH, H), bf16),
            pltpu.VMEM((D, D), bf16),
            pltpu.VMEM((4, 1792, F), bf16),
            pltpu.VMEM((2, 2048, D), bf16),
            pltpu.VMEM((928, D), u32),
            pltpu.VMEM((32, D), f32),
            pltpu.VMEM((P1 // 2, D), u32),
            pltpu.VMEM((T1 // 2, D), u32),
            pltpu.VMEM((11, S // 128, 128, 128), bf16),
            pltpu.VMEM((11, S // 128, 128, 128), bf16),
            pltpu.VMEM((11, S // 128, 64, 128), bf16),
            pltpu.VMEM((11, 32, 128), u32),
            pltpu.VMEM((28, 128, 128), f32),
            pltpu.VMEM((S, D), bf16),
            pltpu.SemaphoreType.DMA((4,)),
        ],
        compiler_params=pltpu.CompilerParams(
            dimension_semantics=("arbitrary",),
            vmem_limit_bytes=100 * 1024 * 1024,
            disable_bounds_checks=True,
            disable_semaphore_checks=True,
        ),
        name="hh",
    )(A_x, A_wqkv, wphi_t, A_wo, B_w_gate, B_w_up, B_w_down)
```
